```python
import jax
import jax.numpy as jnp

def _softmax(x, axis=-1):
    return jax.nn.softmax(x, axis=axis)
def _gelu(x):
    return jax.nn.gelu(x, approximate=True)
def _silu(x):
    return jax.nn.silu(x)
def _sigmoid(x):
    return jax.nn.sigmoid(x)
def _layernorm(x, axis=-1, eps=1e-5):
    m = jnp.mean(x, axis=axis, keepdims=True)
    v = jnp.var(x, axis=axis, keepdims=True)
    return (x - m) / jnp.sqrt(v + eps)
def _scatter_add(tgt, idx, src, axis=0):
    return tgt.at[idx].add(src)
def _segment_sum(src, seg, n):
    return jax.ops.segment_sum(src, seg, n)
class _Rng:
    def __init__(self, key):
        self._k = key
    def _next(self):
        self._k, sub = jax.random.split(self._k)
        return sub
    def normal(self, shape):
        return jax.random.normal(self._next(), shape, dtype=jnp.bfloat16)
    def randint(self, lo, hi, shape):
        return jax.random.randint(self._next(), shape, lo, hi, dtype=jnp.int32)
    def uniform(self, shape, lo=0.0, hi=1.0):
        return jax.random.uniform(self._next(), shape, jnp.bfloat16, lo, hi)
    def permutation(self, n):
        return jax.random.permutation(self._next(), n)


kernel_name = 'standalone__batchnorm__prompt'

def setup_inputs():
    _rng = _Rng(jax.random.key(int.from_bytes(__import__("os").urandom(4), "little")))
    _w = (lambda a: (lambda t: t.astype(jnp.bfloat16) if jnp.issubdtype(t.dtype, jnp.floating) else t)(jnp.asarray(a)))
    B, S, C = 2, 2048, 1024
    K = 3
    return {
        "x": _w((lambda *s: _rng.normal(s) * 0.05)(B, S, C)),
        "w": _w((lambda *s: _rng.normal(s) * 0.05)(K, C, C) * (1.0 / (K * C) ** 0.5)),
        "mean": _w((lambda *s: _rng.normal(s) * 0.05)(C) * 0.1),
        "var": _w(jnp.abs((lambda *s: _rng.normal(s) * 0.05)(C)) + 0.5),
        "g": _w((lambda *s: _rng.normal(s) * 0.05)(C) + 1.0),
        "b": _w((lambda *s: _rng.normal(s) * 0.05)(C) * 0.1),
    }

def reference(x, w, mean, var, g, b):
    K = 3
    P = K // 2
    S = x.shape[1]
    xp = jnp.pad(x, ((0, 0), (P, P), (0, 0)))
    y = sum(jnp.einsum('bsc,cd->bsd', xp[:, k:k + S, :], w[k]) for k in range(K))
    inv_std = 1.0 / jnp.sqrt(var + 1e-5)
    y = (y - mean) * (g * inv_std) + b
    return _silu(y)
```

```python
import jax
import jax.numpy as jnp
import jax.experimental.pallas as pl
import jax.experimental.pallas.tpu as pltpu

_A = 1.6
_B = 1.0 / _A
_A2 = _A * _A
_B2 = _B * _B
_LA = 1.0 / (2.0 * _A2 * (_A2 - _B2))
_LB = 1.0 / (2.0 * _B2 * (_A2 - _B2))
_EPS = 1e-5
_L = 128
_HALO = 8

_F32 = jnp.float32
_BF16 = jnp.bfloat16


def _kernel(x_hbm, w_hbm, mean_hbm, var_hbm, g_hbm, b_hbm, o_hbm,
            xbuf, wraw, pbuf, xt, wt, xf, acc, yst, ob, scsh,
            sem_x, sem_w, sem_p, sem_o, *, nb, seq, ch):
    T = seq // 4
    nct = ch // _L
    XR = 512
    nxc = seq // XR
    WC = 256
    nwc = ch // WC
    NACC = acc.shape[0]

    def x_copy(b, i):
        return pltpu.make_async_copy(
            x_hbm.at[b, pl.ds(i * XR, XR), :], xbuf.at[b, pl.ds(i * XR, XR), :],
            sem_x.at[b * nxc + i])

    def w_copy(j):
        return pltpu.make_async_copy(
            w_hbm.at[:, :, pl.ds(j * WC, WC)], wraw.at[:, :, pl.ds(j * WC, WC)],
            sem_w.at[j])

    def p_copy(i):
        src = (mean_hbm, var_hbm, g_hbm, b_hbm)[i]
        return pltpu.make_async_copy(src, pbuf.at[i], sem_p.at[i])

    def o_copy(b, j):
        return pltpu.make_async_copy(
            ob.at[b * nct + j], o_hbm.at[b, :, pl.ds(j * _L, _L)],
            sem_o.at[b * nct + j])

    def x_transform(b, r0, nrows, slot):
        G = 32
        for ct in range(nct):
            cs = pl.ds(ct * _L, _L)
            st = xf.at[slot, ct]
            st[0:nrows, :] = xbuf[b, r0:r0 + nrows, cs].astype(_F32)
            for t in range(0, nrows // 4, G):
                x0, x1, x2, x3 = (
                    st[pl.ds(4 * t + j, G, stride=4), :] for j in range(4))
                ea = x0 + _A2 * x2
                oa = _A * x1 + (_A * _A2) * x3
                eb = x0 + _B2 * x2
                obb = _B * x1 + (_B * _B2) * x3
                rows = pl.ds(r0 // 4 + t, G)
                for p, v in enumerate((x0, ea + oa, ea - oa, eb + obb, eb - obb, x3)):
                    xt[p, b, rows, cs] = v.astype(_BF16)

    def w_transform(j):
        G = 64
        cs = pl.ds(j * _L, _L)
        for k in range(0, ch, G):
            g0 = wraw[0, k:k + G, cs].astype(_F32)
            g1 = wraw[1, k:k + G, cs].astype(_F32)
            g2 = wraw[2, k:k + G, cs].astype(_F32)
            ea = _LA * g2 + (_LA * _A2) * g0
            oa = (_LA * _A) * g1
            eb = _LB * g2 + (_LB * _B2) * g0
            obb = (_LB * _B) * g1
            for p, v in enumerate((ea + oa, ea - oa, eb + obb, eb - obb)):
                wt[p, k:k + G, cs] = v.astype(_BF16)

    def rhs(p, j):
        cs = pl.ds(j * _L, _L)
        if p == 0:
            return wraw[2, :, cs]
        if p == 5:
            return wraw[0, :, cs]
        return wt[p - 1, :, cs]

    def matmuls(b, j, t0, n, slot):
        for p in (0, 5, 1, 2, 3, 4):
            acc[slot, p, _HALO + t0:_HALO + t0 + n, :] = jnp.dot(
                xt[p, b, t0:t0 + n, :], rhs(p, j), preferred_element_type=_F32)

    def epilogue(b, j, slot, yslot):
        cs = pl.ds(j * _L, _L)
        sc = scsh[0:1, cs]
        sh = scsh[1:2, cs]
        a_ = acc.at[slot]
        ys = yst.at[yslot]
        G = 32
        for r in range(0, T, G):
            q = _HALO + r
            z0 = a_[0, q:q + G, :]
            z5 = a_[5, q:q + G, :]
            z0n = a_[0, q + 1:q + 1 + G, :]
            z5p = a_[5, q - 1:q - 1 + G, :]
            ma, mna, mb, mnb = (a_[p, q:q + G, :] for p in (1, 2, 3, 4))
            sa = ma + mna
            da = ma - mna
            sb = mb + mnb
            db = mb - mnb
            u = sa + z0
            v = sb - z0
            y0 = (_A * db - _B * da) + (z5 + z5p)
            y1 = _A2 * v - _B2 * u
            y2 = (_A * da - _B * db) - (_A2 + _B2) * z5
            y3 = (u - sb) + z0n
            for i, y in enumerate((y0, y1, y2, y3)):
                h = y * sc + sh
                ys[pl.ds(4 * r + i, G, stride=4), :] = h * jnp.tanh(h) + h
            ob[b * nct + j, 4 * r:4 * (r + G), :] = (
                ys[4 * r:4 * (r + G), :].astype(_BF16))

    x_copy(0, 0).start()
    w_copy(0).start()
    for i in range(1, nxc):
        x_copy(0, i).start()
    for i in range(4):
        p_copy(i).start()
    for j in range(1, nwc):
        w_copy(j).start()
    for b in range(1, nb):
        for i in range(nxc):
            x_copy(b, i).start()

    zero = jnp.zeros((_HALO, _L), _F32)
    for s in range(NACC):
        acc[s, 0, _HALO + T:2 * _HALO + T, :] = zero
        acc[s, 5, 0:_HALO, :] = zero

    tpc = XR // 4
    x_copy(0, 0).wait()
    x_transform(0, 0, XR, 0)
    w_copy(0).wait()
    w_transform(0)
    w_transform(1)
    for i in range(nxc):
        if i > 0:
            x_copy(0, i).wait()
            x_transform(0, i * XR, XR, i % 2)
        matmuls(0, 0, i * tpc, tpc, 0)
        matmuls(0, 1, i * tpc, tpc, 1)

    for i in range(4):
        p_copy(i).wait()
    mean, var, gam, bet = (pbuf[i].astype(_F32) for i in range(4))
    s = gam * jax.lax.rsqrt(var + _EPS)
    scsh[0:1, :] = 0.5 * s
    scsh[1:2, :] = 0.5 * (bet - mean * s)

    steps = [(b, j) for b in range(nb) for j in range(nct)]
    for n, (b, j) in enumerate(steps):
        if b == 0 and j >= 2:
            if j % 2 == 0:
                w_copy(j // 2).wait()
            w_transform(j)
        if b > 0 and j == 0:
            for i in range(nxc):
                x_copy(b, i).wait()
            for i in range(nxc):
                x_transform(b, i * XR, XR, i % 2)
        if n >= 2:
            matmuls(b, j, 0, T, n % NACC)
        epilogue(b, j, n % NACC, n % 2)
        o_copy(b, j).start()
    for b, j in steps:
        o_copy(b, j).wait()


@jax.jit
def pallas_standalone__batchnorm__prompt_kernel(
    x: jax.Array,
    w: jax.Array,
    mean: jax.Array,
    var: jax.Array,
    g: jax.Array,
    b: jax.Array,
):
    nb, seq, ch = x.shape
    T = seq // 4
    nct = ch // _L
    vec = lambda v: v.reshape(1, ch)

    def kernel(*refs):
        _kernel(*refs, nb=nb, seq=seq, ch=ch)

    any_spec = pl.BlockSpec(memory_space=pl.ANY)
    return pl.pallas_call(
        kernel,
        out_shape=jax.ShapeDtypeStruct(x.shape, x.dtype),
        in_specs=[any_spec] * 6,
        out_specs=any_spec,
        scratch_shapes=[
            pltpu.VMEM((nb, seq, ch), _BF16),
            pltpu.VMEM((3, ch, ch), _BF16),
            pltpu.VMEM((4, 1, ch), _BF16),
            pltpu.VMEM((6, nb, T, ch), _BF16),
            pltpu.VMEM((4, ch, ch), _BF16),
            pltpu.VMEM((2, nct, 512, _L), _F32),
            pltpu.VMEM((4, 6, T + 2 * _HALO, _L), _F32),
            pltpu.VMEM((2, seq, _L), _F32),
            pltpu.VMEM((nb * nct, seq, _L), _BF16),
            pltpu.VMEM((2, ch), _F32),
            pltpu.SemaphoreType.DMA((nb * (seq // 512),)),
            pltpu.SemaphoreType.DMA((ch // 256,)),
            pltpu.SemaphoreType.DMA((4,)),
            pltpu.SemaphoreType.DMA((nb * nct,)),
        ],
        compiler_params=pltpu.CompilerParams(vmem_limit_bytes=100 * 1024 * 1024),
    )(x, w, vec(mean), vec(var), vec(g), vec(b))
```

```python
import jax
import jax.numpy as jnp
import jax.experimental.pallas as pl
import jax.experimental.pallas.tpu as pltpu

_A = 1.6
_B = 1.0 / _A
_A2 = _A * _A
_B2 = _B * _B
_C = _A2 + _B2
_LA = 1.0 / (2.0 * _A2 * (_A2 - _B2))
_LB = 1.0 / (2.0 * _B2 * (_A2 - _B2))
_EPS = 1e-5
_L = 128
_HALO = 8
_TS = 64
_NACC = 4

_F32 = jnp.float32
_BF16 = jnp.bfloat16
_U32 = jnp.uint32


def _kernel(x_hbm, w_hbm, mean_hbm, var_hbm, g_hbm, b_hbm, o_hbm,
            xb, wr, pb0, pb1, pb2, pb3, xt, wt, acc, ob, scsh, zsrc, zer,
            sem_i, sem_o, *, nb, seq, ch):
    pbuf = (pb0, pb1, pb2, pb3)
    T = seq // 4
    nct = ch // _L
    ng = T // _TS
    XR = 512
    nxc = seq // XR

    sem_x = sem_i.at[pl.ds(0, nxc + nb - 1)]
    sem_w = sem_i.at[pl.ds(nxc + nb - 1, nct)]
    sem_p = sem_i.at[pl.ds(nxc + nb - 1 + nct, 2)]
    def x_copies(b, r0, nr, sem):
        return [pltpu.make_async_copy(
            x_hbm.at[b, pl.ds(r0, nr), pl.ds(ct * _L, _L)],
            xb.at[b, ct, pl.ds(r0, nr), :], sem) for ct in range(nct)]

    def x0_copies(i):
        return x_copies(0, i * XR, XR, sem_x.at[i])

    def xb_copies(b):
        return x_copies(b, 0, seq, sem_x.at[nxc + b - 1])

    def w_copies(j):
        return [pltpu.make_async_copy(
            w_hbm.at[k, :, pl.ds(j * _L, _L)], wr.at[j, k], sem_w.at[j])
            for k in (2, 0, 1)]

    def p_copies():
        return [pltpu.make_async_copy(src, pbuf[i], sem_p.at[0])
                for i, src in enumerate((mean_hbm, var_hbm, g_hbm, b_hbm))]

    def o_copy(b, j):
        return pltpu.make_async_copy(
            ob.at[b * nct + j].bitcast(_BF16), o_hbm.at[b, :, pl.ds(j * _L, _L)],
            sem_o.at[b * nct + j])

    def start(cs):
        for c in cs:
            c.start()

    def wait(cs):
        for c in cs:
            c.wait()

    def unpackers(tok):
        sh = jnp.full((8, _L), 16, _U32)
        mk = jnp.full((8, _L), 0xFFFF0000, _U32)
        if tok is not None:
            z = pltpu.bitcast(tok, _U32) & zer[...]
            sh, mk = sh | z, mk | z
        return (lambda u: pltpu.bitcast(u << sh, _F32),
                lambda u: pltpu.bitcast(u & mk, _F32))

    def pack(lo, hi):
        return pltpu.pack_elementwise([lo, hi], packed_dtype=_BF16)

    def x_slice(b, g, ct, tok=None):
        lo, hi = unpackers(tok)
        xu = xb.at[b, ct].bitcast(_U32)
        for t in range(g * _TS, (g + 1) * _TS, 16):
            vals = []
            for par in range(2):
                we = xu[pl.ds(2 * (t + par), 8, stride=4), :]
                wo = xu[pl.ds(2 * (t + par) + 1, 8, stride=4), :]
                x0, x1, x2, x3 = lo(we), hi(we), lo(wo), hi(wo)
                ea = x0 + _A2 * x2
                oa = _A * x1 + (_A * _A2) * x3
                eb = x0 + _B2 * x2
                obb = _B * x1 + (_B * _B2) * x3
                vals.append((x0, ea + oa, ea - oa, eb + obb, eb - obb, x3))
            for p in range(6):
                xt[p, b, t // 2:t // 2 + 8, ct * _L:(ct + 1) * _L] = pack(
                    vals[0][p], vals[1][p])

    def w_slice(j, kc, tok=None):
        lo, hi = unpackers(tok)
        for k in range(kc * _L // 2, (kc + 1) * _L // 2, 8):
            u = [wr.at[j, i].bitcast(_U32)[k:k + 8, :] for i in range(3)]
            vals = []
            for f in (lo, hi):
                g0, g1, g2 = f(u[0]), f(u[1]), f(u[2])
                ea = _LA * g2 + (_LA * _A2) * g0
                oa = (_LA * _A) * g1
                eb = _LB * g2 + (_LB * _B2) * g0
                obb = (_LB * _B) * g1
                vals.append((ea + oa, ea - oa, eb + obb, eb - obb))
            for p in range(4):
                wt[j, p, k:k + 8, :] = pack(vals[0][p], vals[1][p])

    def rhs(p, j):
        if p == 0:
            r = wr.at[j, 2].bitcast(_U32)[...]
        elif p == 5:
            r = wr.at[j, 0].bitcast(_U32)[...]
        else:
            r = wt[j, p - 1]
        return pltpu.bitcast(r, _BF16)

    def epilogue(b, j, slot, r0, r1):
        cs = slice(j * _L, (j + 1) * _L)
        sc = scsh[0:1, cs]
        scc = scsh[1:2, cs]
        sh = scsh[2:3, cs]
        o_ = ob.at[b * nct + j]
        G = 8
        for r in range(r0, r1, G):
            q = _HALO + r

            def ld(p, o=0):
                return acc[slot, p, q + o:q + o + G, :]

            m, mb = ld(4), ld(3)
            db = mb - m
            sb = mb + m
            ma, mna, z0, z5 = ld(1), ld(2), ld(0), ld(5)
            y0 = (_B * (((_A / _B) * db - ma) + mna) + z5) + ld(5, -1)
            t2 = (_A / _C) * ((ma - (_B / _A) * db) - mna) - z5
            z4 = ((ma - sb) + mna) + z0
            y3 = z4 + ld(0, 1)
            y1 = _A2 * (sb - z0) - _B2 * (z4 + sb)
            hs = (y0 * sc + sh, y1 * sc + sh, t2 * scc + sh, y3 * sc + sh)
            o0, o1, o2, o3 = (h * jnp.tanh(h) + h for h in hs)
            o_[pl.ds(2 * r, G, stride=2), :] = pltpu.pack_elementwise(
                [o0, o1], packed_dtype=_BF16)
            o_[pl.ds(2 * r + 1, G, stride=2), :] = pltpu.pack_elementwise(
                [o2, o3], packed_dtype=_BF16)

    def tile(b, g, j, jobs=()):
        slot = (b * nct + j) % _NACC
        t0 = g * _TS
        jobs = list(jobs)
        for p in (0, 5, 1, 2, 3, 4):
            lhs = pltpu.bitcast(xt[p, b, t0 // 2:(t0 + _TS) // 2, :], _BF16)
            res = jnp.dot(lhs, rhs(p, j), preferred_element_type=_F32)
            acc[slot, p, _HALO + t0:_HALO + t0 + _TS, :] = res
            if jobs and p != 4:
                jobs.pop(0)(res[0:8, :])
        assert not jobs
        r0 = max(t0 - 8, 0)
        r1 = t0 + _TS - 8 if g < ng - 1 else T
        epilogue(b, j, slot, r0, r1)
        if g == ng - 1:
            o_copy(b, j).start()

    start(x0_copies(0))
    start(w_copies(0))
    start(p_copies())
    start(w_copies(1))
    for i in range(1, nxc):
        start(x0_copies(i))

    zsrc[...] = jnp.zeros((8, _L), _U32)
    z_copy = pltpu.make_async_copy(zsrc, zer, sem_p.at[1])
    z_copy.start()
    zero = jnp.zeros((_HALO, _L), _F32)
    for s in range(_NACC):
        acc[s, 0, _HALO + T:2 * _HALO + T, :] = zero
        acc[s, 5, 0:_HALO, :] = zero

    gpc = XR // (4 * _TS)
    wait(x0_copies(0))
    for j in range(2, nct):
        start(w_copies(j))
    for b in range(1, nb):
        start(xb_copies(b))
    for g in range(gpc):
        for ct in range(nct):
            x_slice(0, g, ct)
    wait(w_copies(0))
    wait(p_copies())
    z_copy.wait()
    mean, var, gam, bet = (pbuf[i][...].astype(_F32).reshape(1, ch) for i in range(4))
    s = gam * jax.lax.rsqrt(var + _EPS)
    scsh[0:1, :] = 0.5 * s
    scsh[1:2, :] = (0.5 * _C) * s
    scsh[2:3, :] = 0.5 * (bet - mean * s)
    for kc in range(nct):
        w_slice(0, kc)
    for g in range(gpc):
        tile(0, g, 0)
    wait(w_copies(1))
    for kc in range(nct):
        w_slice(1, kc)
    for g in range(gpc):
        tile(0, g, 1)

    def wjob(j, kc):
        return lambda tok: w_slice(j, kc, tok)

    def xjob(b, g, ct):
        return lambda tok: x_slice(b, g, ct, tok)

    for i in range(1, nxc):
        wait(x0_copies(i))
        last = i == nxc - 1
        if last:
            wait(w_copies(2))
        for g in range(i * gpc, (i + 1) * gpc):
            for ct in range(nct):
                x_slice(0, g, ct)
        n = 0
        for g in range(i * gpc, (i + 1) * gpc):
            for j in range(2):
                jobs = [wjob(2, 2 * n), wjob(2, 2 * n + 1)] if last else []
                tile(0, g, j, jobs)
                n += 1

    xjobs = [xjob(b, g, ct) for b in range(1, nb) for g in range(ng)
             for ct in range(nct)]
    for j in range(2, nct):
        if j == 2:
            wait(w_copies(3))
        if j == 3:
            for jj in range(4, nct):
                wait(w_copies(jj))
        if j == 5:
            for b in range(1, nb):
                wait(xb_copies(b))
        for g in range(ng):
            jobs = [wjob(j + 1, g)] if j + 1 < nct else []
            if j >= 5:
                jobs += [xjobs.pop(0) for _ in range(min(3, len(xjobs)))]
            tile(0, g, j, jobs)
    assert not xjobs
    for b in range(1, nb):
        for j in range(nct):
            for g in range(ng):
                tile(b, g, j)
    for b in range(nb):
        for j in range(nct):
            o_copy(b, j).wait()


@jax.jit
def pallas_standalone__batchnorm__prompt_kernel(
    x: jax.Array,
    w: jax.Array,
    mean: jax.Array,
    var: jax.Array,
    g: jax.Array,
    b: jax.Array,
):
    nb, seq, ch = x.shape
    T = seq // 4
    nct = ch // _L

    def kernel(*refs):
        _kernel(*refs, nb=nb, seq=seq, ch=ch)

    any_spec = pl.BlockSpec(memory_space=pl.ANY)
    return pl.pallas_call(
        kernel,
        out_shape=jax.ShapeDtypeStruct(x.shape, x.dtype),
        in_specs=[any_spec] * 6,
        out_specs=any_spec,
        scratch_shapes=[
            pltpu.VMEM((nb, nct, seq, _L), _BF16),
            pltpu.VMEM((nct, 3, ch, _L), _BF16),
            pltpu.VMEM((ch,), _BF16),
            pltpu.VMEM((ch,), _BF16),
            pltpu.VMEM((ch,), _BF16),
            pltpu.VMEM((ch,), _BF16),
            pltpu.VMEM((6, nb, T // 2, ch), _U32),
            pltpu.VMEM((nct, 4, ch // 2, _L), _U32),
            pltpu.VMEM((_NACC, 6, T + 2 * _HALO, _L), _F32),
            pltpu.VMEM((nb * nct, seq // 2, _L), _U32),
            pltpu.VMEM((3, ch), _F32),
            pltpu.VMEM((8, _L), _U32),
            pltpu.VMEM((8, _L), _U32),
            pltpu.SemaphoreType.DMA((seq // 512 + nb - 1 + nct + 2,)),
            pltpu.SemaphoreType.DMA((nb * nct,)),
        ],
        compiler_params=pltpu.CompilerParams(vmem_limit_bytes=100 * 1024 * 1024),
    )(x, w, mean, var, g, b)
```

```python
import jax
import jax.numpy as jnp
import jax.experimental.pallas as pl
import jax.experimental.pallas.tpu as pltpu

_A = 1.5
_B = 1.0 / _A
_A2 = _A * _A
_B2 = _B * _B
_C = _A2 + _B2
_LA = 1.0 / (2.0 * _A2 * (_A2 - _B2))
_LB = 1.0 / (2.0 * _B2 * (_A2 - _B2))
_GAM = 1.35
_EPS = 1e-5
_L = 128
_HALO = 8
_RG = 64
_POINTS = (0, 5, 1, 2, 3, 4)

_F32 = jnp.float32
_BF16 = jnp.bfloat16
_U32 = jnp.uint32

CFG = dict(r1=3.2, r2=2.8,
           r3=2.8, r4=2.5,
           r5=1.8, n1=16, n2=16, n3=16,
           trunc=0)


def _kernel(x_hbm, w_hbm, mean_hbm, var_hbm, g_hbm, b_hbm, o_hbm,
            xb, wr, pb0, pb1, pb2, pb3, xs, ws, acc, ob, scsh, zsrc, zer,
            sem_i, sem_o, *, nb, seq, ch):
    pbuf = (pb0, pb1, pb2, pb3)
    T = seq // 4
    nct = ch // _L
    ncp = nct // 2
    nq = nct // 2
    ng = T // _RG
    nblk = T // 8
    nslot = acc.shape[0]
    c1 = [4 * (q // 2) + q % 2 for q in range(nq)]
    c2 = [c + 2 for c in c1]

    nsem = [0]

    def new_sem():
        nsem[0] += 1
        return sem_i.at[nsem[0] - 1]

    def x_copies(b, r0, nr, cts=None):
        sem = new_sem()
        return [pltpu.make_async_copy(
            x_hbm.at[b, pl.ds(r0, nr), pl.ds(ct * _L, _L)],
            xb.at[b, ct, pl.ds(r0, nr), :], sem) for ct in (cts or range(nct))]

    def w_copies(cp, taps=(2, 0, 1), k0=0, nk=None):
        sem = new_sem()
        nk = nk or ch
        return [pltpu.make_async_copy(
            w_hbm.at[k, pl.ds(k0, nk), pl.ds(j * _L, _L)],
            wr.at[j, k, pl.ds(k0, nk), :], sem)
            for k in taps for j in (2 * cp, 2 * cp + 1)]

    o_copies = []

    def start_out(b, j, r0, nr):
        c = pltpu.make_async_copy(
            ob.at[b * nct + j].bitcast(_BF16).at[pl.ds(r0, nr), :],
            o_hbm.at[b, pl.ds(r0, nr), pl.ds(j * _L, _L)], sem_o.at[0])
        c.start()
        o_copies.append(c)

    def start(cs):
        for c in cs:
            c.start()

    def wait(cs):
        bg['tok'] = None
        for c in cs:
            c.wait()

    tok_cache = {}

    def tok0(tok, rows):
        if id(tok) not in tok_cache:
            tok_cache[id(tok)] = (tok, pltpu.bitcast(tok, _U32) & zer[...])
        z = tok_cache[id(tok)][1]
        return jnp.tile(z, (rows // 8, 1)) if rows > 8 else z

    def unpackers(tok, rows):
        if tok is None:
            sh = jnp.full((rows, _L), 16, _U32)
            mk = jnp.full((rows, _L), 0xFFFF0000, _U32)
        else:
            z = tok0(tok, 8)
            sh = jnp.tile(z | jnp.uint32(16), (rows // 8, 1))
            mk = jnp.tile(z | jnp.uint32(0xFFFF0000), (rows // 8, 1))
        return (lambda u: pltpu.bitcast(u << sh, _F32),
                lambda u: pltpu.bitcast(u & mk, _F32))

    def pack(lo, hi):
        return pltpu.pack_elementwise([lo, hi], packed_dtype=_BF16)

    def cat(vs, axis=0):
        return vs[0] if len(vs) == 1 else jnp.concatenate(vs, axis=axis)

    have = set()

    def x_job(b, g, q, h, phases):
        def words(half, ct, o):
            xu = xb.at[b, ct].bitcast(_U32)
            t = g * _RG + 32 * half + 16 * h
            return cat([xu[pl.ds(2 * (t + par) + o, 8, stride=4), :]
                        for par in range(2)])

        blocks = [(half, ct) for half in range(2) for ct in (c1[q], c2[q])]
        for phase in phases:
            if phase < 2:
                lo, hi = unpackers((yield 27), 16)
                if phase == 0:
                    outs = {0: [lo(words(*bl, 0)) for bl in blocks]}
                else:
                    outs = {5: [hi(words(*bl, 1)) for bl in blocks]}
            else:
                c = _A if phase == 2 else _B
                p = 2 * phase - 3
                outs = {p: [], p + 1: []}
                for bl in blocks:
                    lo, hi = unpackers((yield 42 if bl == blocks[-1] else 25), 16)
                    we, wo = words(*bl, 0), words(*bl, 1)
                    e = lo(we) + (c * c) * lo(wo)
                    o = c * hi(we) + (c * c * c) * hi(wo)
                    outs[p].append(e + o)
                    outs[p + 1].append(e - o)
            for p, (a11, a12, a21, a22) in outs.items():
                if phase >= 2 and p % 2 == 0:
                    tok = yield 22
                    a11, a22 = tie(a11, tok), tie(a22, tok)
                ss = (a11 + a22, a21 + a22, a11, a22, a11 + a12, a21 - a11,
                      a12 - a22)
                for i, s in enumerate(ss):
                    r = 16 * g + 8 * h
                    xs[p, i, b, r:r + 8, q * _L:(q + 1) * _L] = pack(
                        s[0:8], s[8:16])
                have.add(('x', p, b, g, q, h))

    def w_job(cp, q, kk, phases):
        def vals(tap, j, lo, hi):
            wu = wr.at[j, tap].bitcast(_U32)
            u = cat([wu[ct * 64 + 8 * kk:ct * 64 + 8 * kk + 8, :]
                     for ct in (c1[q], c2[q])])
            return cat([lo(u), hi(u)])

        j1, j2 = 2 * cp, 2 * cp + 1
        gh = 0.5 * _GAM
        for phase in phases:
            if phase < 2:
                lo, hi = unpackers((yield 34), 16)
                tap = 2 if phase == 0 else 0
                p = 0 if phase == 0 else 5
                outs = {p: (gh * vals(tap, j1, lo, hi), vals(tap, j2, lo, hi))}
            else:
                c, lam = (_A, _LA) if phase == 2 else (_B, _LB)
                p = 2 * phase - 3
                uv = []
                for j, s in ((j1, gh * lam), (j2, lam)):
                    lo, hi = unpackers((yield 39), 16)
                    e = s * vals(2, j, lo, hi) + (s * c * c) * vals(0, j, lo, hi)
                    o = (s * c) * vals(1, j, lo, hi)
                    uv.append((e + o, e - o))
                outs = {p: (uv[0][0], uv[1][0]), p + 1: (uv[0][1], uv[1][1])}
            for p, (u, v) in outs.items():
                half = jnp.full((16, _L), 0.5, _F32)
                if phase >= 2:
                    half = tie(half, (yield 23))
                sel = lambda a, n: cat(
                    [a[8 * n:8 * n + 8], a[16 + 8 * n:24 + 8 * n]])
                u1, u2, v1, v2 = sel(u, 0), sel(u, 1), sel(v, 0), sel(v, 1)
                t2 = half * v1 + u1
                t5 = half * v2 - u2
                t1 = t2 + t5
                ts = [t1, t2, v1 - t1, v2 - t1, t5]
                if phase >= 2:
                    ts += [v1, v2]
                for i, t in enumerate(ts):
                    r = 64 * q + 8 * kk
                    ws[cp, p, i, r:r + 8, :] = pack(t[0:8], t[8:16])
                have.add(('w', p, cp, q, kk))

    def lhs(p, i, b, gs, qs):
        return pltpu.bitcast(
            xs[p, i, b, 16 * gs[0]:16 * (gs[-1] + 1),
               qs[0] * _L:(qs[-1] + 1) * _L], _BF16)

    def rhs(p, i, cp, qs):
        if p in (0, 5) and i >= 5:
            wu = wr.at[2 * cp + 1, 2 if p == 0 else 0].bitcast(_U32)
            cts = [(c1 if i == 5 else c2)[q] for q in qs]
            r = cat([wu[64 * ct:64 * ct + 64, :] for ct in cts])
        else:
            r = ws[cp, p, i, 64 * qs[0]:64 * (qs[-1] + 1), :]
        return pltpu.bitcast(r, _BF16)

    def tie(v, tok):
        if tok is None:
            return v
        return pltpu.bitcast(pltpu.bitcast(v, _U32) | tok0(tok, v.shape[0]), _F32)

    def ep_job(b, cp, slot, r0, n, outs):
        q = _HALO + r0
        ys = []
        for c in range(2):
            def ld(p, o=0, c=c):
                return acc[slot, c, p, q + o:q + o + n, :]

            m, mb = tie(ld(4), (yield 24)), ld(3)
            db = mb - m
            sb = mb + m
            ma, mna, z0, z5 = ld(1), ld(2), ld(0), ld(5)
            y0 = (_B * (((_A / _B) * db - ma) + mna) + z5) + ld(5, -1)
            t2 = (_A / _C) * ((ma - (_B / _A) * db) - mna) - z5
            z4 = ((ma - sb) + mna) + z0
            y3 = z4 + ld(0, 1)
            y1 = _A2 * (sb - z0) - _B2 * (z4 + sb)
            ys.append((y0, y1, t2, y3))
        for c in range(2):
            j = 2 * cp + c
            tok = yield 25
            sc, scc, sh = tie(scsh[0, j], tok), tie(scsh[1, j], tok), scsh[2, j]
            if n > 8:
                sc, scc, sh = (jnp.tile(v, (n // 8, 1)) for v in (sc, scc, sh))
            os_ = []
            for k in range(4):
                y = ys[0][k] - ys[1][k] if c == 0 else ys[0][k] + ys[1][k]
                h = y * (scc if k == 2 else sc) + sh
                os_.append(h * jnp.tanh(h) + h)
            o_ = ob.at[b * nct + j]
            o_[pl.ds(2 * r0, n, stride=2), :] = pack(os_[0], os_[1])
            o_[pl.ds(2 * r0 + 1, n, stride=2), :] = pack(os_[2], os_[3])
        st(b, cp)['emitted'].add(r0 // 8)
        for o in outs:
            start_out(*o)

    epq = []
    bg = dict(jobs=[], every=0, rate=2.0, budget=0.0, since=0, active=None,
              cost=0, tok=None)

    def fetch(force=False):
        if bg['active'] is None:
            if bg['jobs'] and (force or bg['since'] >= bg['every']):
                bg['since'] = min(bg['since'] - bg['every'], 4 * bg['every'])
                bg['active'] = bg['jobs'].pop(0)
            elif epq:
                bg['active'] = epq.pop(0)
            else:
                return False
            bg['cost'] = next(bg['active'])
        return True

    def advance(tok, force=False):
        if fetch(force):
            try:
                bg['cost'] = bg['active'].send(tok)
            except StopIteration:
                bg['active'] = None

    def clock(tok, cycles):
        bg['since'] += cycles
        bg['tok'] = tok
        bg['budget'] += bg['rate'] * cycles
        if not fetch():
            bg['budget'] = 0.0
        elif bg['budget'] >= bg['cost']:
            bg['budget'] = min(bg['budget'] - bg['cost'], 16.0)
            advance(tok)

    def require(keys):
        while not all(k in have for k in keys):
            assert bg['active'] is not None or bg['jobs'], keys
            bg['late'] = bg.get('late', 0) + 1
            advance(bg['tok'], force=True)

    def drain():
        bg['every'] = 0
        while bg['active'] is not None or epq or bg['jobs']:
            advance(None)

    state = {}
    owner = {}

    def st(b, cp):
        return state.setdefault((b, cp), dict(
            full={p: set() for p in range(6)}, done=set(), emitted=set(),
            sent=0))

    def flush(b, cp, slot, out_rows):
        s = st(b, cp)
        f = s['full']
        ready = [r for r in range(nblk) if r not in s['done']
                 and all(r in f[p] for p in range(6))
                 and (r + 1 == nblk or r + 1 in f[0])
                 and (r == 0 or r - 1 in f[5])]
        for r in ready:
            s['done'].add(r)
            e = s['sent']
            while e in s['done']:
                e += 1
            outs = []
            if r == ready[-1] and e > s['sent'] and (
                    32 * (e - s['sent']) >= out_rows or e == nblk):
                outs = [(b, j, 32 * s['sent'], 32 * (e - s['sent']))
                        for j in (2 * cp, 2 * cp + 1)]
                s['sent'] = e
            epq.append(ep_job(b, cp, slot, 8 * r, 8, outs))

    def tiles(subs, qs=None, first=True, last=True, out_rows=None,
              two_phase=True):
        qs = tuple(qs or range(nq))
        out_rows = out_rows or seq

        def prod(t, p, i):
            b, gs, cp = t
            require([('x', p, b, g, q, h) for g in gs for q in qs for h in range(2)]
                    + [('w', p, cp, q, kk) for q in qs for kk in range(8)])
            r = jnp.dot(lhs(p, i, b, gs, qs), rhs(p, i, cp, qs),
                        preferred_element_type=_F32)
            for k in range(0, r.shape[0], 8):
                clock(r[k:k + 8], 2 * len(qs))
            return r

        def put(t, p, half, c, v, init, final):
            b, gs, cp = t
            slot = (b * ncp + cp) % nslot
            owner.setdefault(slot, (b, cp))
            if owner[slot] != (b, cp):
                assert len(st(*owner[slot])['emitted']) == nblk
                owner[slot] = (b, cp)
            for n, g in enumerate(gs):
                q = _HALO + g * _RG + 32 * half
                part = v[32 * n:32 * n + 32]
                if not init:
                    part = part + acc[slot, c, p, q:q + 32, :]
                acc[slot, c, p, q:q + 32, :] = part
                if final and last and c == 1:
                    st(b, cp)['full'][p].update(
                        range(8 * g + 4 * half, 8 * g + 4 * half + 4))

        def upper(t, p):
            p1 = prod(t, p, 0)
            c11 = p1 + prod(t, p, 6)
            p4 = prod(t, p, 3)
            c11 = c11 + p4
            p3 = prod(t, p, 2)
            c22 = p1 + p3
            p5 = prod(t, p, 4)
            put(t, p, 0, 0, c11 - p5, first, True)
            put(t, p, 0, 1, p3 + p5, first, True)
            if not two_phase:
                return p4, c22
            put(t, p, 1, 0, p4, first, False)
            put(t, p, 1, 1, c22, first, False)

        def lower(t, p, part=None):
            p6 = prod(t, p, 5)
            if part:
                p6 = p6 + part[1]
            p2 = prod(t, p, 1)
            put(t, p, 1, 0, p2 + part[0] if part else p2, first and part, True)
            put(t, p, 1, 1, p6 - p2, first and part, True)

        def flush_all():
            for b, _, cp in subs:
                flush(b, cp, (b * ncp + cp) % nslot, out_rows)

        if two_phase:
            for p in _POINTS:
                for t in subs:
                    upper(t, p)
            flush_all()
            for p in _POINTS:
                for t in subs:
                    lower(t, p)
        else:
            for p in _POINTS:
                for t in subs:
                    lower(t, p, upper(t, p))
        flush_all()

    def xjobs(b, g, qs=None, phases=(0, 1, 2, 3)):
        return [x_job(b, g, q, h, phases)
                for q in (qs or range(nq)) for h in range(2)]

    def wjobs(cp, qs=None, phases=(0, 1, 2, 3)):
        return [w_job(cp, q, kk, phases)
                for q in (qs or range(nq)) for kk in range(8)]

    def run_now(jobs):
        for j in jobs:
            for _ in j:
                pass

    def xj(b, gs, qs, phases=(0, 1, 2, 3), by_phase=False):
        if by_phase:
            return [j for ph in phases for j in xj(b, gs, qs, (ph,))]
        return [j for g in gs for j in xjobs(b, g, qs, phases)]

    def wj(cp, qs, phases=(0, 1, 2, 3), by_phase=False):
        if by_phase:
            return [j for ph in phases for j in wjobs(cp, qs, (ph,))]
        return wjobs(cp, qs, phases)

    def background(jobs, rate, span=0):
        bg['jobs'] += jobs
        every = span // max(len(bg['jobs']), 1)
        bg.update(every=every, rate=rate, since=every)

    def jit(jobs, n_eager, rate):
        run_now(jobs[:n_eager])
        background(jobs[n_eager:], rate)

    XR = 8 * _RG
    nxc = seq // XR
    qa, qb = tuple(range(nq // 2)), tuple(range(nq // 2, nq))
    kh = ch // 2
    cxa = [x_copies(0, i * XR, XR, range(nct // 2)) for i in range(nxc)]
    cxb = [x_copies(0, i * XR, XR, range(nct // 2, nct)) for i in range(nxc)]
    cwa = [w_copies(cp, k0=0, nk=kh) for cp in range(2)]
    cwb = [w_copies(cp, k0=kh, nk=kh) for cp in range(2)]
    cw = {cp: w_copies(cp) for cp in range(2, ncp)}
    cx1 = x_copies(1, 0, seq)
    psem = new_sem()
    cp_ = [pltpu.make_async_copy(src, pbuf[i], psem)
           for i, src in enumerate((mean_hbm, var_hbm, g_hbm, b_hbm))]
    zsem = new_sem()
    cz = [pltpu.make_async_copy(zsrc, d, zsem) for d in (
        zer, xs.at[5, 6, nb - 1, pl.ds(T // 4 - 8, 8), pl.ds(0, _L)],
        ws.at[ncp - 1, 4, 6, pl.ds(0, 8), :])]
    G = lambda i: (2 * i, 2 * i + 1)
    S = CFG

    start(cwa[0])
    zsrc[...] = jnp.zeros((8, _L), _U32)
    start(cz)
    for c in (cxa[0], cxa[1], cwa[1], cxa[2], cxa[3], cp_, cwb[0], cxb[0],
              cxb[1], cwb[1], cxb[2], cxb[3]):
        start(c)
    zero = jnp.zeros((_HALO, _L), _F32)
    for s in range(nslot):
        for c in range(2):
            acc[s, c, 0, _HALO + T:2 * _HALO + T, :] = zero
            acc[s, c, 5, 0:_HALO, :] = zero

    wait(cwa[0])
    wait(cz)
    run_now(wj(0, qa))
    for i in range(2):
        wait(cxa[i])
        jit(xj(0, G(i), qa, by_phase=True), S['n1'], S['r1'])
        tiles([(0, G(i), 0)], qa, last=False, two_phase=False)
    wait(cwa[1])
    start(cw[2])
    start(cw[3])
    start(cx1)
    jit(wj(1, qa, by_phase=True), S['n2'], S['r2'])
    tiles([(0, G(0), 1), (0, G(1), 1)], qa, last=False, two_phase=False)
    wait(cxa[2])
    wait(cxa[3])
    jit(xj(0, G(2) + G(3), qa, by_phase=True), S['n3'], S['r2'])
    tiles([(0, G(2), 0), (0, G(3), 0)], qa, last=False, two_phase=False)
    wait(cp_)
    wait(cwb[0])
    wait(cxb[0])
    mean, var, gam, bet = (pbuf[i][...].astype(_F32).reshape(1, ch) for i in range(4))
    s = gam * jax.lax.rsqrt(var + _EPS)
    col = jax.lax.broadcasted_iota(jnp.int32, (1, ch), 1)
    sm = jnp.where((col & _L) == 0, s * (1.0 / _GAM), s)
    for k, v in enumerate((0.5 * sm, (0.5 * _C) * sm, 0.5 * (bet - mean * s))):
        for j in range(nct):
            scsh[k, j] = jnp.broadcast_to(v[:, j * _L:(j + 1) * _L], (8, _L))
    background(wj(0, qb) + xj(0, G(0), qb), S['r3'])
    tiles([(0, G(2), 1), (0, G(3), 1)], qa, last=False, two_phase=False)
    wait(cxb[1])
    wait(cwb[1])
    background(xj(0, G(1), qb) + wj(1, qb), S['r3'])
    tiles([(0, G(0), 0)], qb, first=False, two_phase=False)
    tiles([(0, G(1), 0)], qb, first=False, two_phase=False)
    wait(cxb[2])
    wait(cxb[3])
    background(xj(0, G(2) + G(3), qb), S['r3'])
    tiles([(0, G(0), 1), (0, G(1), 1)], qb, first=False, two_phase=False)
    wait(cw[2])
    background(wj(2, None), S['r4'])
    for cp in range(2):
        for i in (2, 3):
            tiles([(0, G(i), cp)], qb, first=False, two_phase=False)
    if S['trunc'] == 1:
        tiles([(0, G(0), 2)])
        drain()
        wait(cw[3]); wait(cx1); wait(o_copies)
        return
    wait(cw[3])
    span = (nxc * 42 - 8) * 64
    background(wj(3, None), S['r5'], span)
    for i in range(nxc):
        tiles([(0, G(i), 2)])
    wait(cx1)
    background(xj(1, G(0), None), S['r5'], span)
    for i in range(nxc):
        tiles([(0, G(i), 3)])
    for i in range(nxc):
        if i + 1 < nxc:
            background(xj(1, G(i + 1), None), S['r5'], span)
        for cp in range(ncp):
            tiles([(1, G(i), cp)], out_rows=256)
    drain()
    wait(o_copies)


@jax.jit
def pallas_standalone__batchnorm__prompt_kernel(
    x: jax.Array,
    w: jax.Array,
    mean: jax.Array,
    var: jax.Array,
    g: jax.Array,
    b: jax.Array,
):
    nb, seq, ch = x.shape
    T = seq // 4
    nct = ch // _L

    def kernel(*refs):
        _kernel(*refs, nb=nb, seq=seq, ch=ch)

    any_spec = pl.BlockSpec(memory_space=pl.ANY)
    return pl.pallas_call(
        kernel,
        out_shape=jax.ShapeDtypeStruct(x.shape, x.dtype),
        in_specs=[any_spec] * 6,
        out_specs=any_spec,
        scratch_shapes=[
            pltpu.VMEM((nb, nct, seq, _L), _BF16),
            pltpu.VMEM((nct, 3, ch, _L), _BF16),
            pltpu.VMEM((ch,), _BF16),
            pltpu.VMEM((ch,), _BF16),
            pltpu.VMEM((ch,), _BF16),
            pltpu.VMEM((ch,), _BF16),
            pltpu.VMEM((6, 7, nb, T // 4, ch // 2), _U32),
            pltpu.VMEM((nct // 2, 6, 7, ch // 4, _L), _U32),
            pltpu.VMEM((nct // 2, 2, 6, T + 2 * _HALO, _L), _F32),
            pltpu.VMEM((nb * nct, seq // 2, _L), _U32),
            pltpu.VMEM((3, nct, 8, _L), _F32),
            pltpu.VMEM((8, _L), _U32),
            pltpu.VMEM((8, _L), _U32),
            pltpu.SemaphoreType.DMA((17,)),
            pltpu.SemaphoreType.DMA((1,)),
        ],
        compiler_params=pltpu.CompilerParams(vmem_limit_bytes=110 * 1024 * 1024),
    )(x, w, mean, var, g, b)
```

```python
import jax
import jax.numpy as jnp
import jax.experimental.pallas as pl
import jax.experimental.pallas.tpu as pltpu

_A = 1.5
_B = 1.0 / _A
_A2 = _A * _A
_B2 = _B * _B
_C = _A2 + _B2
_LA = 1.0 / (2.0 * _A2 * (_A2 - _B2))
_LB = 1.0 / (2.0 * _B2 * (_A2 - _B2))
_GAM = 1.35
_EPS = 1e-5
_L = 128
_HALO = 8
_RG = 64
_POINTS = (0, 5, 1, 2, 3, 4)

_F32 = jnp.float32
_BF16 = jnp.bfloat16
_U32 = jnp.uint32

CFG = dict(r1=3.2, r2=2.8,
           r3=2.8, r4=2.2,
           r5=1.8, n1=8, n2=8, n3=8,
           h1=4, h2=3, h3=1, h4=1,
           h5=3, lag=128, etail=0, ehead=350,
           trunc=0)


def _kernel(x_hbm, w_hbm, mean_hbm, var_hbm, g_hbm, b_hbm, o_hbm,
            xb, wr, pb0, pb1, pb2, pb3, xs, ws, acc, ob, scsh, zsrc, zer,
            sem_i, sem_o, *, nb, seq, ch):
    pbuf = (pb0, pb1, pb2, pb3)
    T = seq // 4
    nct = ch // _L
    ncp = nct // 2
    nq = nct // 2
    ng = T // _RG
    nblk = T // 8
    nslot = acc.shape[0]
    c1 = [2 * q for q in range(nq)]
    c2 = [2 * q + 1 for q in range(nq)]

    free_sems = list(range(sem_i.shape[0]))
    inflight = {}

    def copies(name, sem):
        kind = name[0]
        if kind == 'X':
            _, b, r0, nr, qs = name
            return [pltpu.make_async_copy(
                x_hbm.at[b, pl.ds(r0, nr), pl.ds(ct * _L, _L)],
                xb.at[b, ct, pl.ds(r0, nr), :], sem)
                for ct in range(2 * qs[0], 2 * qs[-1] + 2)]
        if kind == 'W':
            _, cp, qs = name
            k0, nk = 2 * _L * qs[0], 2 * _L * len(qs)
            return [pltpu.make_async_copy(
                w_hbm.at[k, pl.ds(k0, nk), pl.ds(j * _L, _L)],
                wr.at[j, k, pl.ds(k0, nk), :], sem)
                for k in (2, 0, 1) for j in (2 * cp, 2 * cp + 1)]
        if kind == 'P':
            return [pltpu.make_async_copy(src, pbuf[i], sem) for i, src in
                    enumerate((mean_hbm, var_hbm, g_hbm, b_hbm))]
        return [pltpu.make_async_copy(zsrc, d, sem) for d in (
            zer, xs.at[5, 6, nb - 1, pl.ds(T // 4 - 8, 8), pl.ds(0, _L)],
            ws.at[ncp - 1, 4, 6, pl.ds(0, 8), :])]

    def fetch_in(*groups):
        for names in groups:
            k = free_sems.pop(0)
            cs = [c for n in names for c in copies(n, sem_i.at[k])]
            inflight[names] = (k, cs)
            start(cs)

    def arrive(*groups):
        for names in groups:
            k, cs = inflight.pop(names)
            wait(cs)
            free_sems.append(k)

    o_copies = []

    def start_out(b, j, r0, nr):
        c = pltpu.make_async_copy(
            ob.at[b * nct + j].bitcast(_BF16).at[pl.ds(r0, nr), :],
            o_hbm.at[b, pl.ds(r0, nr), pl.ds(j * _L, _L)], sem_o.at[0])
        c.start()
        o_copies.append(c)

    def start(cs):
        for c in cs:
            c.start()

    def wait(cs):
        if hist:
            n, cyc = len(hist), 0
            while n > 1 and cyc < CFG['lag']:
                n -= 1
                cyc += hist[n][1]
            burst(CFG['etail'], hist[n][0])
            hist.clear()
        bg['tok'] = None
        for c in cs:
            c.wait()

    tok_cache = {}

    def tok0(tok, rows):
        if id(tok) not in tok_cache:
            tok_cache[id(tok)] = (tok, pltpu.bitcast(tok, _U32) & zer[...])
        z = tok_cache[id(tok)][1]
        return jnp.tile(z, (rows // 8, 1)) if rows > 8 else z

    def unpackers(tok, rows):
        if tok is None:
            sh = jnp.full((rows, _L), 16, _U32)
            mk = jnp.full((rows, _L), 0xFFFF0000, _U32)
        else:
            z = tok0(tok, 8)
            sh = jnp.tile(z | jnp.uint32(16), (rows // 8, 1))
            mk = jnp.tile(z | jnp.uint32(0xFFFF0000), (rows // 8, 1))
        return (lambda u: pltpu.bitcast(u << sh, _F32),
                lambda u: pltpu.bitcast(u & mk, _F32))

    def pack(lo, hi):
        return pltpu.pack_elementwise([lo, hi], packed_dtype=_BF16)

    def cat(vs, axis=0):
        return vs[0] if len(vs) == 1 else jnp.concatenate(vs, axis=axis)

    have = set()

    def x_job(b, g, q, h, phases):
        def words(half, ct, o):
            xu = xb.at[b, ct].bitcast(_U32)
            t = g * _RG + 32 * half + 16 * h
            return cat([xu[pl.ds(2 * (t + par) + o, 8, stride=4), :]
                        for par in range(2)])

        blocks = [(half, ct) for half in range(2) for ct in (c1[q], c2[q])]
        for phase in phases:
            if phase < 2:
                lo, hi = unpackers((yield 27), 16)
                if phase == 0:
                    outs = {0: [lo(words(*bl, 0)) for bl in blocks]}
                else:
                    outs = {5: [hi(words(*bl, 1)) for bl in blocks]}
            else:
                c = _A if phase == 2 else _B
                p = 2 * phase - 3
                outs = {p: [], p + 1: []}
                for bl in blocks:
                    lo, hi = unpackers((yield 42 if bl == blocks[-1] else 25), 16)
                    we, wo = words(*bl, 0), words(*bl, 1)
                    e = lo(we) + (c * c) * lo(wo)
                    o = c * hi(we) + (c * c * c) * hi(wo)
                    outs[p].append(e + o)
                    outs[p + 1].append(e - o)
            for p, (a11, a12, a21, a22) in outs.items():
                if phase >= 2 and p % 2 == 0:
                    tok = yield 22
                    a11, a22 = tie(a11, tok), tie(a22, tok)
                ss = (a11 + a22, a21 + a22, a11, a22, a11 + a12, a21 - a11,
                      a12 - a22)
                for i, s in enumerate(ss):
                    r = 16 * g + 8 * h
                    xs[p, i, b, r:r + 8, q * _L:(q + 1) * _L] = pack(
                        s[0:8], s[8:16])
                have.add(('x', p, b, g, q, h))

    def w_job(cp, q, kk, phases):
        def vals(tap, j, lo, hi):
            wu = wr.at[j, tap].bitcast(_U32)
            u = cat([wu[ct * 64 + 8 * kk:ct * 64 + 8 * kk + 8, :]
                     for ct in (c1[q], c2[q])])
            return cat([lo(u), hi(u)])

        j1, j2 = 2 * cp, 2 * cp + 1
        gh = 0.5 * _GAM
        for phase in phases:
            if phase < 2:
                lo, hi = unpackers((yield 34), 16)
                tap = 2 if phase == 0 else 0
                p = 0 if phase == 0 else 5
                outs = {p: (gh * vals(tap, j1, lo, hi), vals(tap, j2, lo, hi))}
            else:
                c, lam = (_A, _LA) if phase == 2 else (_B, _LB)
                p = 2 * phase - 3
                uv = []
                for j, s in ((j1, gh * lam), (j2, lam)):
                    lo, hi = unpackers((yield 39), 16)
                    e = s * vals(2, j, lo, hi) + (s * c * c) * vals(0, j, lo, hi)
                    o = (s * c) * vals(1, j, lo, hi)
                    uv.append((e + o, e - o))
                outs = {p: (uv[0][0], uv[1][0]), p + 1: (uv[0][1], uv[1][1])}
            for p, (u, v) in outs.items():
                half = jnp.full((16, _L), 0.5, _F32)
                if phase >= 2:
                    half = tie(half, (yield 23))
                sel = lambda a, n: cat(
                    [a[8 * n:8 * n + 8], a[16 + 8 * n:24 + 8 * n]])
                u1, u2, v1, v2 = sel(u, 0), sel(u, 1), sel(v, 0), sel(v, 1)
                t2 = half * v1 + u1
                t5 = half * v2 - u2
                t1 = t2 + t5
                ts = [t1, t2, v1 - t1, v2 - t1, t5]
                if phase >= 2:
                    ts += [v1, v2]
                for i, t in enumerate(ts):
                    r = 64 * q + 8 * kk
                    ws[cp, p, i, r:r + 8, :] = pack(t[0:8], t[8:16])
                have.add(('w', p, cp, q, kk))

    def lhs(p, i, b, gs, qs):
        return pltpu.bitcast(
            xs[p, i, b, 16 * gs[0]:16 * (gs[-1] + 1),
               qs[0] * _L:(qs[-1] + 1) * _L], _BF16)

    def rhs(p, i, cp, qs):
        if p in (0, 5) and i >= 5:
            wu = wr.at[2 * cp + 1, 2 if p == 0 else 0].bitcast(_U32)
            cts = [(c1 if i == 5 else c2)[q] for q in qs]
            r = cat([wu[64 * ct:64 * ct + 64, :] for ct in cts])
        else:
            r = ws[cp, p, i, 64 * qs[0]:64 * (qs[-1] + 1), :]
        return pltpu.bitcast(r, _BF16)

    def tie(v, tok):
        if tok is None:
            return v
        return pltpu.bitcast(pltpu.bitcast(v, _U32) | tok0(tok, v.shape[0]), _F32)

    def ep_job(b, cp, slot, r0, n, outs):
        q = _HALO + r0
        ys = []
        for c in range(2):
            def ld(p, o=0, c=c):
                return acc[slot, c, p, q + o:q + o + n, :]

            m, mb = tie(ld(4), (yield 24)), ld(3)
            db = mb - m
            sb = mb + m
            ma, mna, z0, z5 = ld(1), ld(2), ld(0), ld(5)
            y0 = (_B * (((_A / _B) * db - ma) + mna) + z5) + ld(5, -1)
            t2 = (_A / _C) * ((ma - (_B / _A) * db) - mna) - z5
            z4 = ((ma - sb) + mna) + z0
            y3 = z4 + ld(0, 1)
            y1 = _A2 * (sb - z0) - _B2 * (z4 + sb)
            ys.append((y0, y1, t2, y3))
        for c in range(2):
            j = 2 * cp + c
            tok = yield 25
            sc, scc, sh = tie(scsh[0, j], tok), tie(scsh[1, j], tok), scsh[2, j]
            if n > 8:
                sc, scc, sh = (jnp.tile(v, (n // 8, 1)) for v in (sc, scc, sh))
            os_ = []
            for k in range(4):
                y = ys[0][k] - ys[1][k] if c == 0 else ys[0][k] + ys[1][k]
                h = y * (scc if k == 2 else sc) + sh
                os_.append(h * jnp.tanh(h) + h)
            o_ = ob.at[b * nct + j]
            o_[pl.ds(2 * r0, n, stride=2), :] = pack(os_[0], os_[1])
            o_[pl.ds(2 * r0 + 1, n, stride=2), :] = pack(os_[2], os_[3])
        st(b, cp)['emitted'].add(r0 // 8)
        for o in outs:
            start_out(*o)

    epq = []
    bg = dict(jobs=[], every=0, rate=2.0, budget=0.0, since=0, active=None,
              cost=0, tok=None)

    hist = []

    def burst(ops, tok):
        while ops > 0 and fetch():
            ops -= bg['cost']
            advance(tok)

    def fetch(force=False):
        if bg['active'] is None:
            if bg['jobs'] and (force or bg['since'] >= bg['every']):
                bg['since'] = min(bg['since'] - bg['every'], 4 * bg['every'])
                bg['active'] = bg['jobs'].pop(0)
            elif epq:
                bg['active'] = epq.pop(0)
            else:
                return False
            bg['cost'] = next(bg['active'])
        return True

    def advance(tok, force=False):
        if fetch(force):
            try:
                bg['cost'] = bg['active'].send(tok)
            except StopIteration:
                bg['active'] = None

    def clock(tok, cycles):
        bg['since'] += cycles
        bg['tok'] = tok
        hist.append((tok, cycles))
        bg['budget'] += bg['rate'] * cycles
        if not fetch():
            bg['budget'] = 0.0
        elif bg['budget'] >= bg['cost']:
            bg['budget'] = min(bg['budget'] - bg['cost'], 16.0)
            advance(tok)

    def require(keys):
        while not all(k in have for k in keys):
            assert bg['active'] is not None or bg['jobs'], keys
            bg['late'] = bg.get('late', 0) + 1
            advance(bg['tok'], force=True)

    def drain():
        bg['every'] = 0
        while bg['active'] is not None or epq or bg['jobs']:
            advance(None)

    state = {}
    owner = {}

    def st(b, cp):
        return state.setdefault((b, cp), dict(
            full={p: set() for p in range(6)}, done=set(), emitted=set(),
            sent=0))

    def flush(b, cp, slot, out_rows):
        s = st(b, cp)
        f = s['full']
        ready = [r for r in range(nblk) if r not in s['done']
                 and all(r in f[p] for p in range(6))
                 and (r + 1 == nblk or r + 1 in f[0])
                 and (r == 0 or r - 1 in f[5])]
        for r in ready:
            s['done'].add(r)
            e = s['sent']
            while e in s['done']:
                e += 1
            outs = []
            if r == ready[-1] and e > s['sent'] and (
                    32 * (e - s['sent']) >= out_rows or e == nblk):
                outs = [(b, j, 32 * s['sent'], 32 * (e - s['sent']))
                        for j in (2 * cp, 2 * cp + 1)]
                s['sent'] = e
            epq.append(ep_job(b, cp, slot, 8 * r, 8, outs))

    kdone = {}

    def tiles(subs, qs=None, out_rows=None, two_phase=True, hooks=None):
        qs = tuple(qs or range(nq))
        out_rows = out_rows or seq
        hooks = hooks or {}
        fl = {(not kdone.get(t), len(kdone.get(t, ())) + len(qs) == nq)
              for t in subs}
        assert len(fl) == 1
        first, last = fl.pop()
        for t in subs:
            kdone[t] = kdone.get(t, ()) + qs
        held = []

        def release():
            for k in range(0, held[0].shape[0], 8):
                for r in held:
                    clock(r[k:k + 8], 2 * len(qs))
            held.clear()

        def prod(t, p, i):
            b, gs, cp = t
            require([('x', p, b, g, q, h) for g in gs for q in qs for h in range(2)]
                    + [('w', p, cp, q, kk) for q in qs for kk in range(8)])
            r = jnp.dot(lhs(p, i, b, gs, qs), rhs(p, i, cp, qs),
                        preferred_element_type=_F32)
            held.append(r)
            if len(held) * len(qs) >= 4:
                release()
            return r

        def put(t, p, half, c, v, init, final):
            b, gs, cp = t
            slot = (b * ncp + cp) % nslot
            owner.setdefault(slot, (b, cp))
            if owner[slot] != (b, cp):
                assert len(st(*owner[slot])['emitted']) == nblk
                owner[slot] = (b, cp)
            for n, g in enumerate(gs):
                q = _HALO + g * _RG + 32 * half
                part = v[32 * n:32 * n + 32]
                if not init:
                    part = part + acc[slot, c, p, q:q + 32, :]
                acc[slot, c, p, q:q + 32, :] = part
                if final and last and c == 1:
                    st(b, cp)['full'][p].update(
                        range(8 * g + 4 * half, 8 * g + 4 * half + 4))

        def upper(t, p):
            p1 = prod(t, p, 0)
            c11 = p1 + prod(t, p, 6)
            p4 = prod(t, p, 3)
            c11 = c11 + p4
            p3 = prod(t, p, 2)
            c22 = p1 + p3
            p5 = prod(t, p, 4)
            put(t, p, 0, 0, c11 - p5, first, True)
            put(t, p, 0, 1, p3 + p5, first, True)
            if not two_phase:
                return p4, c22
            put(t, p, 1, 0, p4, first, False)
            put(t, p, 1, 1, c22, first, False)

        def lower(t, p, part=None):
            p6 = prod(t, p, 5)
            if part:
                p6 = p6 + part[1]
            p2 = prod(t, p, 1)
            put(t, p, 1, 0, p2 + part[0] if part else p2, first and part, True)
            put(t, p, 1, 1, p6 - p2, first and part, True)

        def flush_all():
            for b, _, cp in subs:
                flush(b, cp, (b * ncp + cp) % nslot, out_rows)

        if two_phase:
            for p in _POINTS:
                for t in subs:
                    upper(t, p)
            flush_all()
            for p in _POINTS:
                for t in subs:
                    lower(t, p)
        else:
            for n, p in enumerate(_POINTS):
                if n in hooks:
                    if held:
                        release()
                    hooks[n]()
                for t in subs:
                    lower(t, p, upper(t, p))
        if held:
            release()
        flush_all()

    def xjobs(b, g, qs=None, phases=(0, 1, 2, 3)):
        return [x_job(b, g, q, h, phases)
                for q in (qs or range(nq)) for h in range(2)]

    def wjobs(cp, qs=None, phases=(0, 1, 2, 3)):
        return [w_job(cp, q, kk, phases)
                for q in (qs or range(nq)) for kk in range(8)]

    def run_now(jobs):
        for j in jobs:
            for _ in j:
                pass

    def xj(b, gs, qs, phases=(0, 1, 2, 3), by_phase=False):
        if by_phase:
            return [j for ph in phases for j in xj(b, gs, qs, (ph,))]
        return [j for g in gs for j in xjobs(b, g, qs, phases)]

    def wj(cp, qs, phases=(0, 1, 2, 3), by_phase=False):
        if by_phase:
            return [j for ph in phases for j in wjobs(cp, qs, (ph,))]
        return wjobs(cp, qs, phases)

    def background(jobs, rate, span=0):
        bg['jobs'] += jobs
        every = span // max(len(bg['jobs']), 1)
        bg.update(every=every, rate=rate, since=every)

    def jit(jobs, n_eager, rate):
        run_now(jobs[:n_eager])
        background(jobs[n_eager:], rate)

    XR = 8 * _RG
    nxc = seq // XR
    allq = tuple(range(nq))
    G = lambda i: (2 * i, 2 * i + 1)
    X = lambda i, *qs: ('X', 0, i * XR, XR, qs)
    W = lambda cp, *qs: ('W', cp, qs)
    S = CFG

    def params():
        mean, var, gam, bet = (
            pbuf[i][...].astype(_F32).reshape(1, ch) for i in range(4))
        s = gam * jax.lax.rsqrt(var + _EPS)
        col = jax.lax.broadcasted_iota(jnp.int32, (1, ch), 1)
        sm = jnp.where((col & _L) == 0, s * (1.0 / _GAM), s)
        for k, v in enumerate((0.5 * sm, (0.5 * _C) * sm, 0.5 * (bet - mean * s))):
            for j in range(nct):
                scsh[k, j] = jnp.broadcast_to(v[:, j * _L:(j + 1) * _L], (8, _L))

    def ktiles(subs, qs, hooks=None):
        tiles([(0, G(i), cp) for i, cp in subs], qs, two_phase=False, hooks=hooks)

    qb = allq[2:]
    A1, B1 = (W(0, 1), X(0, 1), X(1, 1)), (X(2, 1), X(3, 1), W(1, 1))
    Ab, Bb = (W(0, *qb), X(0, *qb), ('P',)), (X(1, *qb), W(1, *qb))
    Cb = (X(2, *qb), X(3, *qb))
    w2, w3, x1 = (W(2, *allq),), (W(3, *allq),), (('X', 1, 0, seq, allq),)
    fetch_in((W(0, 0),))
    zsrc[...] = jnp.zeros((8, _L), _U32)
    fetch_in((('Z',),), (X(0, 0),), (X(1, 0),), (X(2, 0), X(3, 0)), (W(1, 0),),
             A1, B1, Ab)
    zero = jnp.zeros((_HALO, _L), _F32)
    for s in range(nslot):
        for c in range(2):
            acc[s, c, 0, _HALO + T:2 * _HALO + T, :] = zero
            acc[s, c, 5, 0:_HALO, :] = zero

    def get(group, jobs, rate):
        def f():
            arrive(group)
            background(jobs(), rate)
            burst(S['ehead'], None)
        return f

    arrive((W(0, 0),), (('Z',),))
    run_now(wj(0, (0,)))
    for i in range(2):
        arrive((X(i, 0),))
        jit(xj(0, G(i), (0,), by_phase=True), S['n1'], S['r1'])
        ktiles([(i, 0)], (0,))
    arrive((X(2, 0), X(3, 0)))
    fetch_in(Bb, Cb)
    jit(xj(0, G(2) + G(3), (0,), by_phase=True), S['n3'], S['r2'])
    ktiles([(2, 0), (3, 0)], (0,))
    arrive((W(1, 0),))
    jit(wj(1, (0,), by_phase=True), S['n2'], S['r2'])
    ktiles([(i, 1) for i in range(4)], (0,), hooks={S['h1']: get(
        A1, lambda: wj(0, (1,), by_phase=True)
        + xj(0, G(0) + G(1), (1,), by_phase=True), S['r3'])})
    ktiles([(0, 0), (1, 0)], (1,))
    arrive(B1)
    fetch_in(w2 + w3, x1)
    jit(xj(0, G(2) + G(3), (1,), by_phase=True), S['n3'], S['r2'])
    background(wj(1, (1,), by_phase=True), S['r2'])
    ktiles([(2, 0), (3, 0)], (1,))
    ktiles([(i, 1) for i in range(4)], (1,), hooks={S['h2']: get(
        Ab, lambda: [j for ph in range(4) for j in
                     wj(0, qb, (ph,)) + xj(0, G(0), qb, (ph,))], S['r3'])})
    params()
    ktiles([(0, 0)], qb)
    arrive(Bb)
    jit(xj(0, G(1), qb, by_phase=True), S['n3'], S['r2'])
    background(wj(1, qb, by_phase=True), S['r2'])
    ktiles([(1, 0)], qb)
    ktiles([(0, 1), (1, 1)], qb, hooks={S['h3']: get(
        Cb, lambda: xj(0, G(2), qb, by_phase=True) + xj(0, G(3), qb), S['r3'])})
    ktiles([(2, 0)], qb)
    ktiles([(3, 0)], qb)
    ktiles([(2, 1)], qb, hooks={S['h4']: get(
        w2 + w3, lambda: wj(2, None, by_phase=True), S['r4'])})
    ktiles([(3, 1)], qb)
    ktiles([(i, 2) for i in range(4)], allq, hooks={4: lambda: background(
        wj(3, None, by_phase=True), S['r4'])})
    if S['trunc']:
        drain()
        arrive(x1)
        wait(o_copies)
        for n in range(24 if S['trunc'] == 2 else 0):
            for u in range(32):
                acc[3, 0, 1, 8:72, :] = jnp.dot(
                    lhs(u % 6, u % 7, 0, (0, 1), allq), rhs(1, u % 7, 0, allq),
                    preferred_element_type=_F32) + acc[3, 0, 1, 8:72, :]
            fetch_in((('Z',),))
            arrive((('Z',),))
        return
    span = (nxc * 42 - 8) * 64
    ktiles([(i, 3) for i in range(4)], allq, hooks={S['h5']: get(
        x1, lambda: xj(1, G(0), None), S['r4'])})
    for i in range(nxc):
        if i + 1 < nxc:
            background(xj(1, G(i + 1), None), S['r5'], span)
        for cp in range(ncp):
            tiles([(1, G(i), cp)], out_rows=256)
    drain()
    wait(o_copies)


@jax.jit
def pallas_standalone__batchnorm__prompt_kernel(
    x: jax.Array,
    w: jax.Array,
    mean: jax.Array,
    var: jax.Array,
    g: jax.Array,
    b: jax.Array,
):
    nb, seq, ch = x.shape
    T = seq // 4
    nct = ch // _L

    def kernel(*refs):
        _kernel(*refs, nb=nb, seq=seq, ch=ch)

    any_spec = pl.BlockSpec(memory_space=pl.ANY)
    return pl.pallas_call(
        kernel,
        out_shape=jax.ShapeDtypeStruct(x.shape, x.dtype),
        in_specs=[any_spec] * 6,
        out_specs=any_spec,
        scratch_shapes=[
            pltpu.VMEM((nb, nct, seq, _L), _BF16),
            pltpu.VMEM((nct, 3, ch, _L), _BF16),
            pltpu.VMEM((ch,), _BF16),
            pltpu.VMEM((ch,), _BF16),
            pltpu.VMEM((ch,), _BF16),
            pltpu.VMEM((ch,), _BF16),
            pltpu.VMEM((6, 7, nb, T // 4, ch // 2), _U32),
            pltpu.VMEM((nct // 2, 6, 7, ch // 4, _L), _U32),
            pltpu.VMEM((nct // 2, 2, 6, T + 2 * _HALO, _L), _F32),
            pltpu.VMEM((nb * nct, seq // 2, _L), _U32),
            pltpu.VMEM((3, nct, 8, _L), _F32),
            pltpu.VMEM((8, _L), _U32),
            pltpu.VMEM((8, _L), _U32),
            pltpu.SemaphoreType.DMA((10,)),
            pltpu.SemaphoreType.DMA((1,)),
        ],
        compiler_params=pltpu.CompilerParams(vmem_limit_bytes=110 * 1024 * 1024),
    )(x, w, mean, var, g, b)
```

```python
import jax
import jax.numpy as jnp
import jax.experimental.pallas as pl
import jax.experimental.pallas.tpu as pltpu

_A = 1.5
_B = 1.0 / _A
_A2 = _A * _A
_B2 = _B * _B
_C = _A2 + _B2
_LA = 1.0 / (2.0 * _A2 * (_A2 - _B2))
_LB = 1.0 / (2.0 * _B2 * (_A2 - _B2))
_GAM = 1.35
_EPS = 1e-5
_L = 128
_HALO = 8
_RG = 64
_POINTS = (0, 5, 1, 2, 3, 4)

_F32 = jnp.float32
_BF16 = jnp.bfloat16
_U32 = jnp.uint32

CFG = dict(r1=3.2, r2=3.1,
           r3=2.8, r4=2.2,
           r5=1.8, r6=2.8,
           n1=8, n2=8,
           n3=8, h1=4,
           h2=2, h3=0,
           h4=1, h5=3,
           rep=2.0, r7=3.2, n4=16,
           ehead=350, ramp=1,
           sel=1, trunc=0)


def _kernel(x_hbm, w_hbm, mean_hbm, var_hbm, g_hbm, b_hbm, o_hbm,
            xb, wr, pb0, pb1, pb2, pb3, xs, ws, acc, ob, scsh, zsrc, zer,
            sem_i, sem_o, *, nb, seq, ch):
    assert nb == 2 and seq == 32 * _RG and ch == 8 * _L
    pbuf = (pb0, pb1, pb2, pb3)
    T = seq // 4
    nct = ch // _L
    ncp = nct // 2
    nq = nct // 2
    nblk = T // 8
    S = CFG

    free_sems = list(range(sem_i.shape[0]))
    inflight = {}

    def copies(name, sem):
        kind = name[0]
        if kind == 'X':
            _, b, r0, nr, qs = name
            return [pltpu.make_async_copy(
                x_hbm.at[b, pl.ds(r0, nr), pl.ds(ct * _L, _L)],
                xb.at[b, ct, pl.ds(r0, nr), :], sem)
                for ct in range(2 * qs[0], 2 * qs[-1] + 2)]
        if kind == 'W':
            _, cp, qs = name
            k0, nk = 2 * _L * qs[0], 2 * _L * len(qs)
            return [pltpu.make_async_copy(
                w_hbm.at[k, pl.ds(k0, nk), pl.ds(j * _L, _L)],
                wr.at[j, k, pl.ds(k0, nk), :], sem)
                for k in (2, 0, 1) for j in (2 * cp, 2 * cp + 1)]
        if kind == 'P':
            return [pltpu.make_async_copy(src, pbuf[i], sem) for i, src in
                    enumerate((mean_hbm, var_hbm, g_hbm, b_hbm))]
        return [pltpu.make_async_copy(zsrc, d, sem) for d in (
            zer, xs.at[5, 6, nb - 1, pl.ds(T // 4 - 8, 8), pl.ds(0, _L)],
            ws.at[ncp - 1, 4, 6, pl.ds(0, 8), :])]

    def fetch_in(*groups):
        for names in groups:
            k = free_sems.pop(0)
            cs = [c for n in names for c in copies(n, sem_i.at[k])]
            inflight[names] = (k, cs)
            for c in cs:
                c.start()

    def arrive(*groups):
        for names in groups:
            k, cs = inflight.pop(names)
            wait(cs)
            free_sems.append(k)

    def wait(cs):
        bg['tok'] = None
        for c in cs:
            c.wait()

    o_copies = []

    def out_copy(b, j, r0, nr):
        return pltpu.make_async_copy(
            ob.at[b * nct + j, pl.ds(r0 // 2, nr // 2), :].bitcast(_BF16),
            o_hbm.at[b, pl.ds(r0, nr), pl.ds(j * _L, _L)], sem_o.at[0])

    def start_out(b, cp, r0, nr):
        for c in range(2):
            o_copies.append(out_copy(b, 2 * cp + c, r0, nr))
            o_copies[-1].start()

    tok_cache = {}

    def tie_u(u, tok):
        if tok is None:
            return u
        t = pltpu.bitcast(tok, _U32)
        reps = (u.shape[0] // 8, 1)
        if S['sel']:
            return jnp.where(jnp.tile(zer[...] == 0, reps), u, jnp.tile(t, reps))
        if id(tok) not in tok_cache:
            tok_cache[id(tok)] = (tok, t & zer[...])
        return u | jnp.tile(tok_cache[id(tok)][1], reps)

    def tie(v, tok):
        if tok is None:
            return v
        return pltpu.bitcast(tie_u(pltpu.bitcast(v, _U32), tok), _F32)

    def unpackers(tok):
        sh = jnp.tile(tie_u(jnp.full((8, _L), 16, _U32), tok), (2, 1))
        mk = jnp.tile(tie_u(jnp.full((8, _L), 0xFFFF0000, _U32), tok), (2, 1))
        return (lambda u: pltpu.bitcast(u << sh, _F32),
                lambda u: pltpu.bitcast(u & mk, _F32))

    def pack(lo, hi):
        return pltpu.pack_elementwise([lo, hi], packed_dtype=_BF16)

    def cat(vs, axis=0):
        return vs[0] if len(vs) == 1 else jnp.concatenate(vs, axis=axis)

    have = set()

    def x_job(b, g, q, h, phases):
        def words(half, ct, o):
            t = g * _RG + 32 * half + 16 * h
            xu = xb.at[b, ct, pl.ds(4 * t, 64), :].bitcast(_U32)
            return cat([xu[pl.ds(2 * par + o, 8, stride=4), :] for par in range(2)])

        blocks = [(half, ct) for half in range(2) for ct in (2 * q, 2 * q + 1)]
        for phase in phases:
            if phase < 2:
                lo, hi = unpackers((yield 27))
                if phase == 0:
                    outs = {0: [lo(words(*bl, 0)) for bl in blocks]}
                else:
                    outs = {5: [hi(words(*bl, 1)) for bl in blocks]}
            else:
                c = _A if phase == 2 else _B
                p = 2 * phase - 3
                outs = {p: [], p + 1: []}
                for bl in blocks:
                    lo, hi = unpackers((yield 42 if bl == blocks[-1] else 25))
                    we, wo = words(*bl, 0), words(*bl, 1)
                    e = lo(we) + (c * c) * lo(wo)
                    o = c * hi(we) + (c * c * c) * hi(wo)
                    outs[p].append(e + o)
                    outs[p + 1].append(e - o)
            for p, (a11, a12, a21, a22) in outs.items():
                if phase >= 2 and p % 2 == 0:
                    tok = yield 22
                    a11, a22 = tie(a11, tok), tie(a22, tok)
                ss = (a11 - a22, a21 - a22, a11, a22, a11 - a12, a21 - a11,
                      a12 - a22)
                for i, s in enumerate(ss):
                    r = 16 * g + 8 * h
                    xs[p, i, b, r:r + 8, q * _L:(q + 1) * _L] = pack(
                        s[0:8], s[8:16])
                have.add(('x', p, b, g, q, h))

    def w_job(cp, q, kk, phases):
        def vals(tap, j, lo, hi):
            u = cat([wr.at[j, tap, pl.ds(ct * _L + 16 * kk, 16), :].bitcast(_U32)[...]
                     for ct in (2 * q, 2 * q + 1)])
            return cat([lo(u), hi(u)])

        j1, j2 = 2 * cp, 2 * cp + 1
        gh = 0.5 * _GAM
        for phase in phases:
            if phase < 2:
                lo, hi = unpackers((yield 34))
                tap = 2 if phase == 0 else 0
                p = 0 if phase == 0 else 5
                outs = {p: (gh * vals(tap, j1, lo, hi), vals(tap, j2, lo, hi))}
            else:
                c, lam = (_A, _LA) if phase == 2 else (_B, _LB)
                p = 2 * phase - 3
                uv = []
                for j, s in ((j1, gh * lam), (j2, lam)):
                    lo, hi = unpackers((yield 39))
                    e = s * vals(2, j, lo, hi) + (s * c * c) * vals(0, j, lo, hi)
                    o = (s * c) * vals(1, j, lo, hi)
                    uv.append((e + o, e - o))
                outs = {p: (uv[0][0], uv[1][0]), p + 1: (uv[0][1], uv[1][1])}
            for p, (u, v) in outs.items():
                half = jnp.full((8, _L), 0.5, _F32)
                if phase >= 2:
                    half = tie(half, (yield 23))
                half = jnp.tile(half, (2, 1))
                sel = lambda a, n: cat(
                    [a[8 * n:8 * n + 8], a[16 + 8 * n:24 + 8 * n]])
                u1, u2, v1, v2 = sel(u, 0), sel(u, 1), sel(v, 0), sel(v, 1)
                t2 = half * v1 + u1
                t5 = half * v2 - u2
                t1 = t2 - t5
                ts = [t1, t2, v1 - t1, v2 + t1, t5]
                if phase >= 2:
                    ts += [v1, v2]
                for i, t in enumerate(ts):
                    r = 64 * q + 8 * kk
                    ws[cp, p, i, r:r + 8, :] = pack(t[0:8], t[8:16])
                have.add(('w', p, cp, q, kk))

    def lhs(p, i, b, gs, qs):
        return pltpu.bitcast(
            xs[p, i, b, 16 * gs[0]:16 * (gs[-1] + 1),
               qs[0] * _L:(qs[-1] + 1) * _L], _BF16)

    def rhs(p, i, cp, qs):
        if p in (0, 5) and i >= 5:
            r = cat([wr.at[2 * cp + 1, 2 if p == 0 else 0,
                           pl.ds((2 * q + i - 5) * _L, _L), :].bitcast(_U32)[...]
                     for q in qs])
        else:
            r = ws[cp, p, i, 64 * qs[0]:64 * (qs[-1] + 1), :]
        return pltpu.bitcast(r, _BF16)

    def ep_job(acc, b, cp, blk, out=None):
        q = _HALO + 8 * blk
        ys = []
        for c in range(2):
            def ld(p, o=0, c=c):
                return acc[c, p, q + o:q + o + 8, :]

            m, mb = tie(ld(4), (yield 24)), ld(3)
            db = mb - m
            sb = mb + m
            ma, mna, z0, z5 = ld(1), ld(2), ld(0), ld(5)
            y0 = (_B * (((_A / _B) * db - ma) + mna) + z5) + ld(5, -1)
            t2 = (_A / _C) * ((ma - (_B / _A) * db) - mna) - z5
            z4 = ((ma - sb) + mna) + z0
            y3 = z4 + ld(0, 1)
            y1 = _A2 * (sb - z0) - _B2 * (z4 + sb)
            ys.append((y0, y1, t2, y3))
        for c in range(2):
            j = 2 * cp + c
            tok = yield 25
            sc, scc, sh = tie(scsh[0, j], tok), tie(scsh[1, j], tok), scsh[2, j]
            os_ = []
            for k in range(4):
                y = ys[0][k] - ys[1][k] if c == 0 else ys[0][k] + ys[1][k]
                h = y * (scc if k == 2 else sc) + sh
                os_.append(h * jnp.tanh(h) + h)
            o_ = ob.at[b * nct + j]
            o_[pl.ds(16 * blk, 8, stride=2), :] = pack(os_[0], os_[1])
            o_[pl.ds(16 * blk + 1, 8, stride=2), :] = pack(os_[2], os_[3])
        if out:
            start_out(b, cp, *out)

    epq = []
    bg = dict(jobs=[], every=0, rate=2.0, budget=0.0, since=0, active=None,
              cost=0, tok=None, late=0)

    def fetch(force=False):
        if bg['active'] is None:
            if bg['jobs'] and (force or bg['since'] >= bg['every']):
                bg['since'] = min(bg['since'] - bg['every'], 4 * bg['every'])
                bg['active'] = bg['jobs'].pop(0)
                bg['cap'] = 4.0
            elif epq:
                bg['active'] = epq.pop(0)
                bg['cap'] = S['rep']
            else:
                return False
            bg['cost'] = next(bg['active'])
        return True

    def advance(tok, force=False):
        if fetch(force):
            try:
                bg['cost'] = bg['active'].send(tok)
            except StopIteration:
                bg['active'] = None

    def clock(tok, cycles):
        bg['since'] += cycles
        bg['tok'] = tok
        if not fetch():
            bg['budget'] = 0.0
            return
        bg['budget'] += min(bg['rate'], bg['cap']) * cycles
        if bg['budget'] >= bg['cost']:
            bg['budget'] = min(bg['budget'] - bg['cost'], 16.0)
            advance(tok)

    def burst(ops):
        while ops > 0 and fetch():
            ops -= bg['cost']
            advance(None)

    def require(keys):
        while not all(k in have for k in keys):
            assert bg['active'] is not None or bg['jobs'], keys
            bg['late'] += 1
            advance(bg['tok'], force=True)

    def drain():
        bg['every'] = 0
        while bg['active'] is not None or epq or bg['jobs']:
            bg['late'] += 1
            advance(bg['tok'])

    def background(jobs, rate, span=0):
        bg['jobs'] += jobs
        every = span // max(len(bg['jobs']), 1)
        bg.update(every=every, rate=rate, since=every)

    def run_now(jobs):
        for j in jobs:
            for _ in j:
                pass

    def jit(jobs, n_eager, rate):
        run_now(jobs[:n_eager])
        background(jobs[n_eager:], rate)

    def xj(b, gs, qs, phases=(0, 1, 2, 3), by_phase=False):
        if by_phase:
            return [j for ph in phases for j in xj(b, gs, qs, (ph,))]
        return [x_job(b, g, q, h, phases) for g in gs for q in qs for h in range(2)]

    def wj(cp, qs, phases=(0, 1, 2, 3), by_phase=False):
        if by_phase:
            return [j for ph in phases for j in wj(cp, qs, (ph,))]
        return [w_job(cp, q, kk, phases) for q in qs for kk in range(8)]

    class Col:
        def __init__(self, b, cp, out_rows):
            self.b, self.cp, self.out_rows = b, cp, out_rows
            self.acc = acc.at[cp]
            self.todo = list(range(nblk))
            self.sent = 0
            self.jobs = []
            self.full = {p: set() for p in range(6)}
            self.kdone = {}

        def flush(self):
            f = self.full
            ready = [r for r in self.todo
                     if all(r in f[p] for p in range(6))
                     and (r + 1 == nblk or r + 1 in f[0])
                     and (r == 0 or r - 1 in f[5])]
            for r in ready:
                self.todo.remove(r)
                e = min(self.todo, default=nblk)
                out = None
                if r == ready[-1] and (e == nblk or
                                       32 * (e - self.sent) >= self.out_rows):
                    out = (32 * self.sent, 32 * (e - self.sent))
                    self.sent = e
                self.jobs.append(ep_job(self.acc, self.b, self.cp, r, out))
                epq.append(self.jobs[-1])

        def finished(self):
            return not self.todo and not any(
                j in epq or j is bg['active'] for j in self.jobs)

    def tiles(subs, qs, two_phase=False, hooks=None):
        hooks = hooks or {}
        subs = [(c, i if isinstance(i, tuple) else (i,)) for c, i in subs]
        fl = {(i not in c.kdone, c.kdone.get(i, 0) + len(qs) == nq) for c, i in subs}
        assert len(fl) == 1
        first, last = fl.pop()
        for c, i in subs:
            c.kdone[i] = c.kdone.get(i, 0) + len(qs)
        held = []

        def release():
            for k in range(0, held[0].shape[0], 8):
                for r in held:
                    clock(r[k:k + 8], 2 * len(qs))
            held.clear()

        def prod(t, p, i):
            col, gs = t[0], tuple(range(2 * t[1][0], 2 * t[1][-1] + 2))
            require([('x', p, col.b, g, q, h)
                     for g in gs for q in qs for h in range(2)]
                    + [('w', p, col.cp, q, kk) for q in qs for kk in range(8)])
            r = jnp.dot(lhs(p, i, col.b, gs, qs), rhs(p, i, col.cp, qs),
                        preferred_element_type=_F32)
            held.append(r)
            if len(held) * len(qs) >= 4:
                release()
            return r

        def put(t, p, half, c, v, init, final):
            col = t[0]
            for n, g in enumerate(range(2 * t[1][0], 2 * t[1][-1] + 2)):
                q = _HALO + g * _RG + 32 * half
                part = v[32 * n:32 * n + 32]
                if not init:
                    part = part + col.acc[c, p, q:q + 32, :]
                col.acc[c, p, q:q + 32, :] = part
                if final and last and c == 1:
                    col.full[p].update(range(8 * g + 4 * half, 8 * g + 4 * half + 4))

        def upper(t, p):
            p1 = prod(t, p, 0)
            c11 = p1 + prod(t, p, 6)
            p4 = prod(t, p, 3)
            c11 = c11 + p4
            p3 = prod(t, p, 2)
            c22 = p1 + p3
            p5 = prod(t, p, 4)
            put(t, p, 0, 0, c11 + p5, first, True)
            put(t, p, 0, 1, p3 - p5, first, True)
            if not two_phase:
                return p4, c22
            put(t, p, 1, 0, p4, first, False)
            put(t, p, 1, 1, c22, first, False)

        def lower(t, p, part=None):
            p6 = prod(t, p, 5)
            if part:
                p6 = p6 + part[1]
            p2 = prod(t, p, 1)
            put(t, p, 1, 0, p2 + part[0] if part else p2, first and part, True)
            put(t, p, 1, 1, p6 - p2, first and part, True)

        def flush():
            if held:
                release()
            for c, _ in subs:
                c.flush()

        if two_phase:
            for p in _POINTS:
                for t in subs:
                    upper(t, p)
            flush()
            for p in _POINTS:
                for t in subs:
                    lower(t, p)
        else:
            for n, p in enumerate(_POINTS):
                if n in hooks:
                    flush()
                    hooks[n]()
                for t in subs:
                    lower(t, p, upper(t, p))
        flush()

    XR = 8 * _RG
    allq = tuple(range(nq))
    G = lambda i: (2 * i, 2 * i + 1)
    X = lambda i, *qs: ('X', 0, i * XR, XR, qs)
    W = lambda cp, *qs: ('W', cp, qs)

    col0 = [Col(0, cp, seq) for cp in range(ncp)]

    def params():
        mean, var, gam, bet = (
            pbuf[i][...].astype(_F32).reshape(1, ch) for i in range(4))
        s = gam * jax.lax.rsqrt(var + _EPS)
        col = jax.lax.broadcasted_iota(jnp.int32, (1, ch), 1)
        sm = jnp.where((col & _L) == 0, s * (1.0 / _GAM), s)
        for k, v in enumerate((0.5 * sm, (0.5 * _C) * sm, 0.5 * (bet - mean * s))):
            for j in range(nct):
                scsh[k, j] = jnp.broadcast_to(v[:, j * _L:(j + 1) * _L], (8, _L))

    def kt(subs, qs, hooks=None):
        tiles([(col0[cp], i) for i, cp in subs], qs, hooks=hooks)

    def get(group, jobs, rate):
        def f():
            arrive(group)
            background(jobs(), rate)
            burst(S['ehead'])
        return f

    qb = allq[2:]
    q0 = {0: [(X(0, 0),), (X(1, 0),), (X(2, 0), X(3, 0)), (W(1, 0),)],
          1: [(X(0, 0),), (X(1, 0), X(2, 0)), (X(3, 0), W(1, 0))]}[S['ramp']]
    A1, B1 = (W(0, 1), X(0, 1), X(1, 1)), (X(2, 1), X(3, 1), W(1, 1))
    Ab, Bb = (W(0, *qb), X(0, *qb), ('P',)), (X(1, *qb), W(1, *qb))
    Cb = (X(2, *qb), X(3, *qb))
    w23, x1 = (W(2, *allq), W(3, *allq)), (('X', 1, 0, seq, allq),)
    fetch_in((W(0, 0),))
    zsrc[...] = jnp.zeros((8, _L), _U32)
    fetch_in((('Z',),), *q0, A1, B1, Ab)
    zero = jnp.zeros((_HALO, _L), _F32)
    for cp in range(ncp):
        for c in range(2):
            acc[cp, c, 0, _HALO + T:2 * _HALO + T, :] = zero
            acc[cp, c, 5, 0:_HALO, :] = zero

    hook_a1 = {S['h1']: get(
        A1, lambda: wj(0, (1,), by_phase=True)
        + xj(0, G(0) + G(1), (1,), by_phase=True), S['r3'])}
    arrive((W(0, 0),), (('Z',),))
    run_now(wj(0, (0,)))
    arrive(q0[0])
    jit(xj(0, G(0), (0,), by_phase=True), S['n1'], S['r1'])
    kt([(0, 0)], (0,))
    arrive(q0[1])
    if S['ramp'] == 0:
        jit(xj(0, G(1), (0,), by_phase=True), S['n1'], S['r1'])
        kt([(1, 0)], (0,))
        arrive(q0[2])
        fetch_in(Bb, Cb)
        jit(xj(0, G(2) + G(3), (0,), by_phase=True), S['n3'], S['r2'])
        kt([(2, 0), (3, 0)], (0,))
        arrive(q0[3])
        jit(wj(1, (0,), by_phase=True), S['n2'], S['r2'])
    else:
        jit(xj(0, G(1) + G(2), (0,), by_phase=True), S['n3'], S['r2'])
        kt([(1, 0), (2, 0)], (0,))
        arrive(q0[2])
        fetch_in(Bb, Cb)
        jit(xj(0, G(3), (0,), by_phase=True), S['n1'], S['r1'])
        background(wj(1, (0,), by_phase=True), S['r1'])
        kt([(3, 0)], (0,))
        background([], S['r2'])
    kt([(i, 1) for i in range(4)], (0,), hooks=hook_a1)
    kt([(0, 0), (1, 0)], (1,))
    arrive(B1)
    fetch_in(w23, x1)
    jit(xj(0, G(2) + G(3), (1,), by_phase=True), S['n3'], S['r2'])
    background(wj(1, (1,), by_phase=True), S['r2'])
    kt([(2, 0), (3, 0)], (1,))
    kt([(i, 1) for i in range(4)], (1,), hooks={S['h2']: get(
        Ab, lambda: [j for ph in range(4) for j in
                     wj(0, qb, (ph,)) + xj(0, G(0), qb, (ph,))], S['r3'])})
    params()
    kt([(0, 0)], qb)
    arrive(Bb)
    jit(xj(0, G(1), qb, by_phase=True), S['n4'], S['r7'])
    background(wj(1, qb, by_phase=True), S['r7'])
    kt([(1, 0)], qb)
    kt([(0, 1), (1, 1)], qb, hooks={S['h3']: get(
        Cb, lambda: xj(0, G(2), qb, by_phase=True) + xj(0, G(3), qb), S['r6'])})
    kt([(2, 0)], qb)
    kt([(3, 0)], qb)
    kt([(2, 1)], qb)
    kt([(3, 1)], qb, hooks={S['h4']: get(
        w23, lambda: wj(2, allq, by_phase=True), S['r4'])})
    if S['trunc']:
        kt([(0, 2), (1, 2)], allq)
        drain()
        arrive(x1)
        wait(o_copies)
        for n in range(24 if S['trunc'] == 2 else 0):
            for u in range(32):
                acc[3, 0, 1, 8:72, :] = jnp.dot(
                    lhs(u % 6, u % 7, 0, (0, 1), allq), rhs(1, u % 7, 0, allq),
                    preferred_element_type=_F32) + acc[3, 0, 1, 8:72, :]
            fetch_in((('Z',),))
            arrive((('Z',),))
        return
    kt([(i, 2) for i in range(4)], allq, hooks={4: lambda: background(
        wj(3, allq, by_phase=True), S['r4'])})
    kt([(i, 3) for i in range(4)], allq, hooks={S['h5']: get(
        x1, lambda: xj(1, G(0), allq), S['r4'])})

    col1 = [Col(1, cp, 256) for cp in range(ncp)]
    for i in range(4):
        if i < 3:
            background(xj(1, G(i + 1), allq), S['r5'], 4 * 2688 - 512)
        for cp in range(ncp):
            assert col0[cp].finished()
            tiles([(col1[cp], i)], allq, two_phase=True)
    bg['tok'] = None
    drain()
    wait(o_copies)


@jax.jit
def pallas_standalone__batchnorm__prompt_kernel(
    x: jax.Array,
    w: jax.Array,
    mean: jax.Array,
    var: jax.Array,
    g: jax.Array,
    b: jax.Array,
):
    nb, seq, ch = x.shape
    T = seq // 4
    nct = ch // _L

    def kernel(*refs):
        _kernel(*refs, nb=nb, seq=seq, ch=ch)

    any_spec = pl.BlockSpec(memory_space=pl.ANY)
    return pl.pallas_call(
        kernel,
        out_shape=jax.ShapeDtypeStruct(x.shape, x.dtype),
        in_specs=[any_spec] * 6,
        out_specs=any_spec,
        scratch_shapes=[
            pltpu.VMEM((nb, nct, seq, _L), _BF16),
            pltpu.VMEM((nct, 3, ch, _L), _BF16),
            pltpu.VMEM((ch,), _BF16),
            pltpu.VMEM((ch,), _BF16),
            pltpu.VMEM((ch,), _BF16),
            pltpu.VMEM((ch,), _BF16),
            pltpu.VMEM((6, 7, nb, T // 4, ch // 2), _U32),
            pltpu.VMEM((nct // 2, 6, 7, ch // 4, _L), _U32),
            pltpu.VMEM((nct // 2, 2, 6, T + 2 * _HALO, _L), _F32),
            pltpu.VMEM((nb * nct, seq // 2, _L), _U32),
            pltpu.VMEM((3, nct, 8, _L), _F32),
            pltpu.VMEM((8, _L), _U32),
            pltpu.VMEM((8, _L), _U32),
            pltpu.SemaphoreType.DMA((10,)),
            pltpu.SemaphoreType.DMA((1,)),
        ],
        compiler_params=pltpu.CompilerParams(vmem_limit_bytes=110 * 1024 * 1024),
    )(x, w, mean, var, g, b)
```

```python
import jax
import jax.numpy as jnp
import jax.experimental.pallas as pl
import jax.experimental.pallas.tpu as pltpu

_A = 1.5
_B = 1.0 / _A
_A2 = _A * _A
_B2 = _B * _B
_C = _A2 + _B2
_LA = 1.0 / (2.0 * _A2 * (_A2 - _B2))
_LB = 1.0 / (2.0 * _B2 * (_A2 - _B2))
_GAM = 1.35
_EPS = 1e-5
_L = 128
_HALO = 8
_RG = 64
_POINTS = (0, 5, 1, 2, 3, 4)

_F32 = jnp.float32
_BF16 = jnp.bfloat16
_U32 = jnp.uint32

CFG = dict(r1=3.5, r2=3.3,
           r3=2.8, r4=2.2,
           r5=1.8, r6=2.5,
           n1=8, n2=8,
           n3=8, h1=1,
           h2=0, h3=0,
           h4=1, h5=3,
           rep=2.0, r7=2.8, n4=16,
           ehead=350, ramp=2,
           h0=2, hb=0, hc=0, ra=2.3,
           fp=1, gmask=1, trunc=0)


def _kernel(x_hbm, w_hbm, mean_hbm, var_hbm, g_hbm, b_hbm, o_hbm,
            xb, wr, pb0, pb1, pb2, pb3, xs, ws, acc, ob, scsh, zsrc, zer,
            sem_i, sem_o, *, nb, seq, ch):
    assert nb == 2 and seq == 32 * _RG and ch == 8 * _L
    pbuf = (pb0, pb1, pb2, pb3)
    T = seq // 4
    nct = ch // _L
    ncp = nct // 2
    nq = nct // 2
    nblk = T // 8
    S = CFG

    free_sems = list(range(sem_i.shape[0]))
    inflight = {}

    def copies(name, sem):
        kind = name[0]
        if kind == 'X':
            _, b, r0, nr, qs = name
            return [pltpu.make_async_copy(
                x_hbm.at[b, pl.ds(r0, nr), pl.ds(ct * _L, _L)],
                xb.at[b, ct, pl.ds(r0, nr), :], sem)
                for ct in range(2 * qs[0], 2 * qs[-1] + 2)]
        if kind == 'W':
            _, cp, qs = name
            k0, nk = 2 * _L * qs[0], 2 * _L * len(qs)
            return [pltpu.make_async_copy(
                w_hbm.at[k, pl.ds(k0, nk), pl.ds(j * _L, _L)],
                wr.at[j, k, pl.ds(k0, nk), :], sem)
                for k in (2, 0, 1) for j in (2 * cp, 2 * cp + 1)]
        if kind == 'P':
            return [pltpu.make_async_copy(src, pbuf[i], sem) for i, src in
                    enumerate((mean_hbm, var_hbm, g_hbm, b_hbm))]
        return [pltpu.make_async_copy(zsrc, d, sem) for d in (
            zer, xs.at[5, 6, nb - 1, pl.ds(T // 4 - 8, 8), pl.ds(0, _L)],
            ws.at[ncp - 1, 4, 6, pl.ds(0, 8), :])]

    def fetch_in(*groups):
        for names in groups:
            k = free_sems.pop(0)
            cs = [c for n in names for c in copies(n, sem_i.at[k])]
            inflight[names] = (k, cs)
            for c in cs:
                c.start()

    def arrive(*groups):
        for names in groups:
            k, cs = inflight.pop(names)
            wait(cs)
            free_sems.append(k)

    def wait(cs):
        bg['tok'] = None
        for c in cs:
            c.wait()

    o_copies = []

    def out_copy(b, j, r0, nr):
        return pltpu.make_async_copy(
            ob.at[b * nct + j, pl.ds(r0 // 2, nr // 2), :].bitcast(_BF16),
            o_hbm.at[b, pl.ds(r0, nr), pl.ds(j * _L, _L)], sem_o.at[0])

    def start_out(b, cp, r0, nr):
        for c in range(2):
            o_copies.append(out_copy(b, 2 * cp + c, r0, nr))
            o_copies[-1].start()

    keep = {}

    def tie(v, tok):
        if tok is None:
            return v
        if len(tok) == 2:
            tok.append({jnp.dtype(_F32): tok[0][tok[1]:tok[1] + 8]})
        if v.dtype not in tok[2]:
            tok[2][v.dtype] = pltpu.bitcast(tok[2][jnp.dtype(_F32)], v.dtype)
        t = tok[2][v.dtype]
        n = v.shape[0]
        if S['gmask'] == 0 or n not in keep:
            keep[n] = cat([zer[...]] * (n // 8)) == 0
        return jax.lax.select(keep[n], v, cat([t] * (n // 8)))

    sh16 = jnp.full((8, _L), 16, _U32)
    mk16 = jnp.full((8, _L), 0xFFFF0000, _U32)

    def unpackers(tok):
        sh, mk = cat([tie(sh16, tok)] * 2), cat([tie(mk16, tok)] * 2)
        return (lambda u: pltpu.bitcast(u << sh, _F32),
                lambda u: pltpu.bitcast(u & mk, _F32))

    def pack(lo, hi):
        return pltpu.pack_elementwise([lo, hi], packed_dtype=_BF16)

    def cat(vs, axis=0):
        return vs[0] if len(vs) == 1 else jnp.concatenate(vs, axis=axis)

    have = set()

    def x_job(b, g, q, h, phases):
        def words(half, ct, o):
            t = g * _RG + 32 * half + 16 * h
            xu = xb.at[b, ct, pl.ds(4 * t, 64), :].bitcast(_U32)
            return cat([xu[pl.ds(2 * par + o, 8, stride=4), :] for par in range(2)])

        blocks = [(half, ct) for half in range(2) for ct in (2 * q, 2 * q + 1)]
        for phase in phases:
            if phase < 2:
                lo, hi = unpackers((yield 27))
                if phase == 0:
                    outs = {0: [lo(words(*bl, 0)) for bl in blocks]}
                else:
                    outs = {5: [hi(words(*bl, 1)) for bl in blocks]}
            else:
                c = _A if phase == 2 else _B
                p = 2 * phase - 3
                outs = {p: [], p + 1: []}
                for bl in blocks:
                    lo, hi = unpackers((yield 42 if bl == blocks[-1] else 25))
                    we, wo = words(*bl, 0), words(*bl, 1)
                    e = lo(we) + (c * c) * lo(wo)
                    o = c * hi(we) + (c * c * c) * hi(wo)
                    outs[p].append(e + o)
                    outs[p + 1].append(e - o)
            for p, (a11, a12, a21, a22) in outs.items():
                if phase >= 2 and p % 2 == 0:
                    tok = yield 22
                    a11, a22 = tie(a11, tok), tie(a22, tok)
                ss = (a11 - a22, a21 - a22, a11, a22, a11 - a12, a21 - a11,
                      a12 - a22)
                for i, s in enumerate(ss):
                    r = 16 * g + 8 * h
                    xs[p, i, b, r:r + 8, q * _L:(q + 1) * _L] = pack(
                        s[0:8], s[8:16])
                have.add(('x', p, b, g, q, h))

    def w_job(cp, q, kk, phases):
        def vals(tap, j, lo, hi):
            u = cat([wr.at[j, tap, pl.ds(ct * _L + 16 * kk, 16), :].bitcast(_U32)[...]
                     for ct in (2 * q, 2 * q + 1)])
            return cat([lo(u), hi(u)])

        j1, j2 = 2 * cp, 2 * cp + 1
        gh = 0.5 * _GAM
        for phase in phases:
            if phase < 2:
                lo, hi = unpackers((yield 34))
                tap = 2 if phase == 0 else 0
                p = 0 if phase == 0 else 5
                outs = {p: (gh * vals(tap, j1, lo, hi), vals(tap, j2, lo, hi))}
            else:
                c, lam = (_A, _LA) if phase == 2 else (_B, _LB)
                p = 2 * phase - 3
                uv = []
                for j, s in ((j1, gh * lam), (j2, lam)):
                    lo, hi = unpackers((yield 39))
                    e = s * vals(2, j, lo, hi) + (s * c * c) * vals(0, j, lo, hi)
                    o = (s * c) * vals(1, j, lo, hi)
                    uv.append((e + o, e - o))
                outs = {p: (uv[0][0], uv[1][0]), p + 1: (uv[0][1], uv[1][1])}
            for p, (u, v) in outs.items():
                half = jnp.full((8, _L), 0.5, _F32)
                if phase >= 2:
                    half = tie(half, (yield 23))
                half = cat([half] * 2)
                sel = lambda a, n: cat(
                    [a[8 * n:8 * n + 8], a[16 + 8 * n:24 + 8 * n]])
                u1, u2, v1, v2 = sel(u, 0), sel(u, 1), sel(v, 0), sel(v, 1)
                t2 = half * v1 + u1
                t5 = half * v2 - u2
                t1 = t2 - t5
                ts = [t1, t2, v1 - t1, v2 + t1, t5]
                if phase >= 2:
                    ts += [v1, v2]
                for i, t in enumerate(ts):
                    r = 64 * q + 8 * kk
                    ws[cp, p, i, r:r + 8, :] = pack(t[0:8], t[8:16])
                have.add(('w', p, cp, q, kk))

    def lhs(p, i, b, gs, qs):
        return pltpu.bitcast(
            xs[p, i, b, 16 * gs[0]:16 * (gs[-1] + 1),
               qs[0] * _L:(qs[-1] + 1) * _L], _BF16)

    def rhs(p, i, cp, qs):
        if p in (0, 5) and i >= 5:
            r = cat([wr.at[2 * cp + 1, 2 if p == 0 else 0,
                           pl.ds((2 * q + i - 5) * _L, _L), :].bitcast(_U32)[...]
                     for q in qs])
        else:
            r = ws[cp, p, i, 64 * qs[0]:64 * (qs[-1] + 1), :]
        return pltpu.bitcast(r, _BF16)

    def ep_job(acc, b, cp, blk, out=None):
        q = _HALO + 8 * blk
        ys = []
        for c in range(2):
            def ld(p, o=0, c=c):
                return acc[c, p, q + o:q + o + 8, :]

            m, mb = tie(ld(4), (yield 24)), ld(3)
            db = mb - m
            sb = mb + m
            ma, mna, z0, z5 = ld(1), ld(2), ld(0), ld(5)
            y0 = (_B * (((_A / _B) * db - ma) + mna) + z5) + ld(5, -1)
            t2 = (_A / _C) * ((ma - (_B / _A) * db) - mna) - z5
            z4 = ((ma - sb) + mna) + z0
            y3 = z4 + ld(0, 1)
            y1 = _A2 * (sb - z0) - _B2 * (z4 + sb)
            ys.append((y0, y1, t2, y3))
        for c in range(2):
            j = 2 * cp + c
            tok = yield 25
            sc, scc, sh = tie(scsh[0, j], tok), tie(scsh[1, j], tok), scsh[2, j]
            os_ = []
            for k in range(4):
                y = ys[0][k] - ys[1][k] if c == 0 else ys[0][k] + ys[1][k]
                h = y * (scc if k == 2 else sc) + sh
                os_.append(h * jnp.tanh(h) + h)
            o_ = ob.at[b * nct + j]
            o_[pl.ds(16 * blk, 8, stride=2), :] = pack(os_[0], os_[1])
            o_[pl.ds(16 * blk + 1, 8, stride=2), :] = pack(os_[2], os_[3])
        if out:
            start_out(b, cp, *out)

    epq = []
    bg = dict(jobs=[], every=0, rate=2.0, budget=0.0, since=0, active=None,
              cost=0, tok=None, late=0)

    def fetch(force=False):
        if bg['active'] is None:
            if bg['jobs'] and (force or bg['since'] >= bg['every']):
                bg['since'] = min(bg['since'] - bg['every'], 4 * bg['every'])
                bg['active'] = bg['jobs'].pop(0)
                bg['cap'] = 4.0
            elif epq:
                bg['active'] = epq.pop(0)
                bg['cap'] = S['rep']
            else:
                return False
            bg['cost'] = next(bg['active'])
        return True

    def advance(tok, force=False):
        if fetch(force):
            try:
                bg['cost'] = bg['active'].send(tok)
            except StopIteration:
                bg['active'] = None

    def clock(tok, cycles):
        bg['since'] += cycles
        bg['tok'] = tok
        if not fetch():
            bg['budget'] = 0.0
            return
        bg['budget'] += min(bg['rate'], bg['cap']) * cycles
        if bg['budget'] >= bg['cost']:
            bg['budget'] = min(bg['budget'] - bg['cost'], 16.0)
            advance(tok)

    def burst(ops):
        while ops > 0 and fetch():
            ops -= bg['cost']
            advance(None)

    def require(keys):
        while not all(k in have for k in keys):
            assert bg['active'] is not None or bg['jobs'], keys
            bg['late'] += 1
            advance(bg['tok'], force=True)

    def drain():
        bg['every'] = 0
        while bg['active'] is not None or epq or bg['jobs']:
            bg['late'] += 1
            advance(bg['tok'])

    def background(jobs, rate, span=0):
        bg['jobs'] += jobs
        every = span // max(len(bg['jobs']), 1)
        bg.update(every=every, rate=rate, since=every)

    def run_now(jobs):
        for j in jobs:
            for _ in j:
                pass

    def jit(jobs, n_eager, rate):
        run_now(jobs[:n_eager])
        background(jobs[n_eager:], rate)

    def xj(b, gs, qs, phases=(0, 1, 2, 3), by_phase=False):
        if by_phase:
            return [j for ph in phases for j in xj(b, gs, qs, (ph,))]
        return [x_job(b, g, q, h, phases) for g in gs for q in qs for h in range(2)]

    def wj(cp, qs, phases=(0, 1, 2, 3), by_phase=False):
        if by_phase:
            return [j for ph in phases for j in wj(cp, qs, (ph,))]
        return [w_job(cp, q, kk, phases) for q in qs for kk in range(8)]

    class Col:
        def __init__(self, b, cp, out_rows):
            self.b, self.cp, self.out_rows = b, cp, out_rows
            self.acc = acc.at[cp]
            self.todo = list(range(nblk))
            self.sent = 0
            self.jobs = []
            self.full = {p: set() for p in range(6)}
            self.kdone = {}

        def flush(self):
            f = self.full
            ready = [r for r in self.todo
                     if all(r in f[p] for p in range(6))
                     and (r + 1 == nblk or r + 1 in f[0])
                     and (r == 0 or r - 1 in f[5])]
            for r in ready:
                self.todo.remove(r)
                e = min(self.todo, default=nblk)
                out = None
                if r == ready[-1] and (e == nblk or
                                       32 * (e - self.sent) >= self.out_rows):
                    out = (32 * self.sent, 32 * (e - self.sent))
                    self.sent = e
                self.jobs.append(ep_job(self.acc, self.b, self.cp, r, out))
                epq.append(self.jobs[-1])

        def finished(self):
            return not self.todo and not any(
                j in epq or j is bg['active'] for j in self.jobs)

    def tiles(subs, qs, two_phase=False, hooks=None):
        hooks = hooks or {}
        subs = [(c, i if isinstance(i, tuple) else (i,)) for c, i in subs]
        fl = {(i not in c.kdone, c.kdone.get(i, 0) + len(qs) == nq) for c, i in subs}
        assert len(fl) == 1
        first, last = fl.pop()
        for c, i in subs:
            c.kdone[i] = c.kdone.get(i, 0) + len(qs)
        held = []

        def release():
            for k in range(0, held[0].shape[0], 8):
                for r in held:
                    clock([r, k], 2 * len(qs))
            held.clear()

        def prod(t, p, i):
            col, gs = t[0], tuple(range(2 * t[1][0], 2 * t[1][-1] + 2))
            require([('x', p, col.b, g, q, h)
                     for g in gs for q in qs for h in range(2)]
                    + [('w', p, col.cp, q, kk) for q in qs for kk in range(8)])
            r = jnp.dot(lhs(p, i, col.b, gs, qs), rhs(p, i, col.cp, qs),
                        preferred_element_type=_F32)
            held.append(r)
            if len(held) * len(qs) >= 4:
                release()
            return r

        def put(t, p, half, c, v, init, final):
            col = t[0]
            for n, g in enumerate(range(2 * t[1][0], 2 * t[1][-1] + 2)):
                q = _HALO + g * _RG + 32 * half
                part = v[32 * n:32 * n + 32]
                if not init:
                    part = part + col.acc[c, p, q:q + 32, :]
                col.acc[c, p, q:q + 32, :] = part
                if final and last and c == 1:
                    col.full[p].update(range(8 * g + 4 * half, 8 * g + 4 * half + 4))

        def upper(t, p):
            p1 = prod(t, p, 0)
            c11 = p1 + prod(t, p, 6)
            p4 = prod(t, p, 3)
            c11 = c11 + p4
            p3 = prod(t, p, 2)
            c22 = p1 + p3
            p5 = prod(t, p, 4)
            put(t, p, 0, 0, c11 + p5, first, True)
            put(t, p, 0, 1, p3 - p5, first, True)
            if not two_phase:
                return p4, c22
            put(t, p, 1, 0, p4, first, False)
            put(t, p, 1, 1, c22, first, False)

        def lower(t, p, part=None):
            p6 = prod(t, p, 5)
            if part:
                p6 = p6 + part[1]
            p2 = prod(t, p, 1)
            put(t, p, 1, 0, p2 + part[0] if part else p2, first and part, True)
            put(t, p, 1, 1, p6 - p2, first and part, True)

        def flush():
            if held:
                release()
            for c, _ in subs:
                c.flush()

        if two_phase:
            for p in _POINTS:
                for t in subs:
                    upper(t, p)
            flush()
            for p in _POINTS:
                for t in subs:
                    lower(t, p)
        else:
            for n, p in enumerate(_POINTS):
                if n in hooks:
                    flush()
                    hooks[n]()
                for t in subs:
                    lower(t, p, upper(t, p))
        flush()

    XR = 8 * _RG
    allq = tuple(range(nq))
    G = lambda i: (2 * i, 2 * i + 1)
    X = lambda i, *qs: ('X', 0, i * XR, XR, qs)
    W = lambda cp, *qs: ('W', cp, qs)

    col0 = [Col(0, cp, seq) for cp in range(ncp)]

    def params():
        mean, var, gam, bet = (
            pbuf[i][...].astype(_F32).reshape(1, ch) for i in range(4))
        s = gam * jax.lax.rsqrt(var + _EPS)
        col = jax.lax.broadcasted_iota(jnp.int32, (1, ch), 1)
        sm = jnp.where((col & _L) == 0, s * (1.0 / _GAM), s)
        for k, v in enumerate((0.5 * sm, (0.5 * _C) * sm, 0.5 * (bet - mean * s))):
            for j in range(nct):
                scsh[k, j] = jnp.broadcast_to(v[:, j * _L:(j + 1) * _L], (8, _L))

    def kt(subs, qs, hooks=None):
        tiles([(col0[cp], i) for i, cp in subs], qs, hooks=hooks)

    def get(group, jobs, rate, fetch=()):
        def f():
            fetch_in(*fetch)
            arrive(group)
            background(jobs(), rate)
            burst(S['ehead'])
        return f

    qb = allq[2:]
    if S['ramp'] == 2:
        qr = allq[1:]
        q0 = [(X(0, 0),), (X(1, 0), X(2, 0)), (X(3, 0), W(1, 0)), (W(2, 0),)]
        A1, B1 = (W(0, 1), X(0, 1), X(1, 1)), (X(2, 1), X(3, 1), W(1, 1))
        Ab, Bb = (W(0, *qb), X(0, *qb), ('P',)), (X(1, *qb), W(1, *qb))
        Cb = (X(2, *qb), X(3, *qb))
        w23, x1 = (W(2, *qr), W(3, *allq)), (('X', 1, 0, seq, allq),)
        fetch_in((W(0, 0),))
        zsrc[...] = jnp.zeros((8, _L), _U32)
        fetch_in((('Z',),), *q0, A1, B1)
        zero = jnp.zeros((_HALO, _L), _F32)
        for cp in range(ncp):
            for c in range(2):
                acc[cp, c, 0, _HALO + T:2 * _HALO + T, :] = zero
                acc[cp, c, 5, 0:_HALO, :] = zero
        arrive((W(0, 0),), (('Z',),))
        run_now(wj(0, (0,)))
        arrive(q0[0])
        jit(xj(0, G(0), (0,), by_phase=True), S['n1'], S['r1'])
        kt([(0, 0)], (0,))
        fetch_in(Ab)
        arrive(q0[1])
        jit(xj(0, G(1) + G(2), (0,), by_phase=True), S['n3'], S['r2'])
        kt([(1, 0), (2, 0)], (0,))
        arrive(q0[2])
        jit(xj(0, G(3), (0,), by_phase=True), S['n1'], S['r1'])
        background(wj(1, (0,), by_phase=True), S['r1'])
        kt([(3, 0)], (0,))
        background([], S['r2'])
        kt([(i, 1) for i in range(4)], (0,), hooks={S['h0']: get(
            q0[3], lambda: wj(2, (0,), by_phase=True), S['ra'], (Bb, Cb))})
        kt([(i, 2) for i in range(4)], (0,), hooks={S['h1']: get(
            A1, lambda: wj(0, (1,), by_phase=True)
            + xj(0, G(0) + G(1), (1,), by_phase=True), S['ra'])})

        kt([(0, 0), (1, 0)], (1,), hooks={S['hb']: get(
            B1, lambda: xj(0, G(2) + G(3), (1,), by_phase=True)
            + wj(1, (1,), by_phase=True), S['ra'], (w23, x1))})
        kt([(2, 0), (3, 0)], (1,))
        kt([(i, 1) for i in range(4)], (1,), hooks={S['h2']: get(
            Ab, lambda: [j for ph in range(4) for j in
                         wj(0, qb, (ph,)) + xj(0, G(0), qb, (ph,))], S['r3'])})
        params()
        kt([(0, 0)], qb, hooks={S['hc']: get(
            Bb, lambda: xj(0, G(1), qb, by_phase=True)
            + wj(1, qb, by_phase=True), S['r7'])})
        kt([(1, 0)], qb)
        kt([(0, 1), (1, 1)], qb, hooks={S['h3']: get(
            Cb, lambda: xj(0, G(2), qb, by_phase=True) + xj(0, G(3), qb), S['r6'])})
        kt([(2, 0)], qb)
        kt([(3, 0)], qb)
        kt([(2, 1)], qb, hooks={S['h4']: get(
            w23, lambda: wj(2, qr, by_phase=True), S['r4'])})
        kt([(3, 1)], qb)
        q2 = qr
    else:
        q0 = {0: [(X(0, 0),), (X(1, 0),), (X(2, 0), X(3, 0)), (W(1, 0),)],
              1: [(X(0, 0),), (X(1, 0), X(2, 0)), (X(3, 0), W(1, 0))]}[S['ramp']]
        A1, B1 = (W(0, 1), X(0, 1), X(1, 1)), (X(2, 1), X(3, 1), W(1, 1))
        Ab, Bb = (W(0, *qb), X(0, *qb), ('P',)), (X(1, *qb), W(1, *qb))
        Cb = (X(2, *qb), X(3, *qb))
        w23, x1 = (W(2, *allq), W(3, *allq)), (('X', 1, 0, seq, allq),)
        fetch_in((W(0, 0),))
        zsrc[...] = jnp.zeros((8, _L), _U32)
        fetch_in((('Z',),), *q0, A1, B1, Ab)
        zero = jnp.zeros((_HALO, _L), _F32)
        for cp in range(ncp):
            for c in range(2):
                acc[cp, c, 0, _HALO + T:2 * _HALO + T, :] = zero
                acc[cp, c, 5, 0:_HALO, :] = zero

        hook_a1 = {S['h1']: get(
            A1, lambda: wj(0, (1,), by_phase=True)
            + xj(0, G(0) + G(1), (1,), by_phase=True), S['r3'])}
        arrive((W(0, 0),), (('Z',),))
        run_now(wj(0, (0,)))
        arrive(q0[0])
        jit(xj(0, G(0), (0,), by_phase=True), S['n1'], S['r1'])
        kt([(0, 0)], (0,))
        arrive(q0[1])
        if S['ramp'] == 0:
            jit(xj(0, G(1), (0,), by_phase=True), S['n1'], S['r1'])
            kt([(1, 0)], (0,))
            arrive(q0[2])
            fetch_in(Bb, Cb)
            jit(xj(0, G(2) + G(3), (0,), by_phase=True), S['n3'], S['r2'])
            kt([(2, 0), (3, 0)], (0,))
            arrive(q0[3])
            jit(wj(1, (0,), by_phase=True), S['n2'], S['r2'])
        else:
            jit(xj(0, G(1) + G(2), (0,), by_phase=True), S['n3'], S['r2'])
            kt([(1, 0), (2, 0)], (0,))
            arrive(q0[2])
            fetch_in(Bb, Cb)
            jit(xj(0, G(3), (0,), by_phase=True), S['n1'], S['r1'])
            background(wj(1, (0,), by_phase=True), S['r1'])
            kt([(3, 0)], (0,))
            background([], S['r2'])
        kt([(i, 1) for i in range(4)], (0,), hooks=hook_a1)
        kt([(0, 0), (1, 0)], (1,))
        arrive(B1)
        fetch_in(w23, x1)
        jit(xj(0, G(2) + G(3), (1,), by_phase=True), S['n3'], S['r2'])
        background(wj(1, (1,), by_phase=True), S['r2'])
        kt([(2, 0), (3, 0)], (1,))
        kt([(i, 1) for i in range(4)], (1,), hooks={S['h2']: get(
            Ab, lambda: [j for ph in range(4) for j in
                         wj(0, qb, (ph,)) + xj(0, G(0), qb, (ph,))], S['r3'])})
        params()
        kt([(0, 0)], qb)
        arrive(Bb)
        jit(xj(0, G(1), qb, by_phase=True), S['n4'], S['r7'])
        background(wj(1, qb, by_phase=True), S['r7'])
        kt([(1, 0)], qb)
        kt([(0, 1), (1, 1)], qb, hooks={S['h3']: get(
            Cb, lambda: xj(0, G(2), qb, by_phase=True) + xj(0, G(3), qb), S['r6'])})
        kt([(2, 0)], qb)
        kt([(3, 0)], qb)
        kt([(2, 1)], qb)
        kt([(3, 1)], qb, hooks={S['h4']: get(
            w23, lambda: wj(2, allq, by_phase=True), S['r4'])})
        q2 = allq
    if S['trunc']:
        kt([(0, 2), (1, 2)], q2)
        drain()
        arrive(x1)
        wait(o_copies)
        for n in range(24 if S['trunc'] == 2 else 0):
            for u in range(32):
                acc[3, 0, 1, 8:72, :] = jnp.dot(
                    lhs(u % 6, u % 7, 0, (0, 1), allq), rhs(1, u % 7, 0, allq),
                    preferred_element_type=_F32) + acc[3, 0, 1, 8:72, :]
            fetch_in((('Z',),))
            arrive((('Z',),))
        return
    kt([(i, 2) for i in range(4)], q2, hooks={4: lambda: background(
        wj(3, allq, by_phase=True), S['r4'])})
    kt([(i, 3) for i in range(4)], allq, hooks={S['h5']: get(
        x1, lambda: xj(1, G(0), allq), S['r4'])})

    col1 = [Col(1, cp, 256) for cp in range(ncp)]
    for i in range(4):
        if i < 3:
            background(xj(1, G(i + 1), allq), S['r5'], 4 * 2688 - 512)
        for cp in range(ncp):
            assert col0[cp].finished()
            tiles([(col1[cp], i)], allq, two_phase=True)
    bg['tok'] = None
    drain()
    wait(o_copies)


@jax.jit
def pallas_standalone__batchnorm__prompt_kernel(
    x: jax.Array,
    w: jax.Array,
    mean: jax.Array,
    var: jax.Array,
    g: jax.Array,
    b: jax.Array,
):
    nb, seq, ch = x.shape
    T = seq // 4
    nct = ch // _L

    def kernel(*refs):
        _kernel(*refs, nb=nb, seq=seq, ch=ch)

    any_spec = pl.BlockSpec(memory_space=pl.ANY)
    return pl.pallas_call(
        kernel,
        out_shape=jax.ShapeDtypeStruct(x.shape, x.dtype),
        in_specs=[any_spec] * 6,
        out_specs=any_spec,
        scratch_shapes=[
            pltpu.VMEM((nb, nct, seq, _L), _BF16),
            pltpu.VMEM((nct, 3, ch, _L), _BF16),
            pltpu.VMEM((ch,), _BF16),
            pltpu.VMEM((ch,), _BF16),
            pltpu.VMEM((ch,), _BF16),
            pltpu.VMEM((ch,), _BF16),
            pltpu.VMEM((6, 7, nb, T // 4, ch // 2), _U32),
            pltpu.VMEM((nct // 2, 6, 7, ch // 4, _L), _U32),
            pltpu.VMEM((nct // 2, 2, 6, T + 2 * _HALO, _L), _F32),
            pltpu.VMEM((nb * nct, seq // 2, _L), _U32),
            pltpu.VMEM((3, nct, 8, _L), _F32),
            pltpu.VMEM((8, _L), _U32),
            pltpu.VMEM((8, _L), _U32),
            pltpu.SemaphoreType.DMA((10,)),
            pltpu.SemaphoreType.DMA((1,)),
        ],
        compiler_params=pltpu.CompilerParams(vmem_limit_bytes=110 * 1024 * 1024),
    )(x, w, mean, var, g, b)
```

```python
import jax
import jax.numpy as jnp
import jax.experimental.pallas as pl
import jax.experimental.pallas.tpu as pltpu

_A = 1.5
_B = 1.0 / _A
_A2 = _A * _A
_B2 = _B * _B
_C = _A2 + _B2
_LA = 1.0 / (2.0 * _A2 * (_A2 - _B2))
_LB = 1.0 / (2.0 * _B2 * (_A2 - _B2))
_GAM = 1.35
_EPS = 1e-5
_L = 128
_HALO = 8
_RG = 64
_POINTS = (0, 5, 1, 2, 3, 4)

_F32 = jnp.float32
_BF16 = jnp.bfloat16
_U32 = jnp.uint32

CFG = dict(r1=3.5, r2=3.3,
           r3=2.8, r4=2.0,
           r5=1.8, r6=2.5,
           n1=8, n2=8,
           n3=8, h1=1,
           h2=0, h3=0,
           h4=1, h5=3,
           rep=1.8, r7=2.8, n4=16,
           ehead=350, ramp=2,
           h0=2, hb=0, hc=0, ra=2.3,
           fp=1, bp=2, gmask=1, trunc=0)


def _kernel(x_hbm, w_hbm, mean_hbm, var_hbm, g_hbm, b_hbm, o_hbm,
            xb, wr, pb0, pb1, pb2, pb3, xs, ws, acc, ob, scsh, zsrc, zer,
            sem_i, sem_o, *, nb, seq, ch):
    assert nb == 2 and seq == 32 * _RG and ch == 8 * _L
    pbuf = (pb0, pb1, pb2, pb3)
    T = seq // 4
    nct = ch // _L
    ncp = nct // 2
    nq = nct // 2
    nblk = T // 8
    S = CFG

    free_sems = list(range(sem_i.shape[0]))
    inflight = {}

    def copies(name, sem):
        kind = name[0]
        if kind == 'X':
            _, b, r0, nr, qs = name
            return [pltpu.make_async_copy(
                x_hbm.at[b, pl.ds(r0, nr), pl.ds(ct * _L, _L)],
                xb.at[b, ct, pl.ds(r0, nr), :], sem)
                for ct in range(2 * qs[0], 2 * qs[-1] + 2)]
        if kind == 'W':
            _, cp, qs = name
            k0, nk = 2 * _L * qs[0], 2 * _L * len(qs)
            return [pltpu.make_async_copy(
                w_hbm.at[k, pl.ds(k0, nk), pl.ds(j * _L, _L)],
                wr.at[j, k, pl.ds(k0, nk), :], sem)
                for k in (2, 0, 1) for j in (2 * cp, 2 * cp + 1)]
        if kind == 'P':
            return [pltpu.make_async_copy(src, pbuf[i], sem) for i, src in
                    enumerate((mean_hbm, var_hbm, g_hbm, b_hbm))]
        return [pltpu.make_async_copy(zsrc, d, sem) for d in (
            zer, xs.at[5, 6, nb - 1, pl.ds(T // 4 - 8, 8), pl.ds(0, _L)],
            ws.at[ncp - 1, 4, 6, pl.ds(0, 8), :])]

    def fetch_in(*groups):
        for names in groups:
            k = free_sems.pop(0)
            cs = [c for n in names for c in copies(n, sem_i.at[k])]
            inflight[names] = (k, cs)
            for c in cs:
                c.start()

    def arrive(*groups):
        for names in groups:
            k, cs = inflight.pop(names)
            wait(cs)
            free_sems.append(k)

    def wait(cs):
        bg['tok'] = None
        for c in cs:
            c.wait()

    o_copies = []

    def out_copy(b, j, r0, nr):
        return pltpu.make_async_copy(
            ob.at[b * nct + j, pl.ds(r0 // 2, nr // 2), :].bitcast(_BF16),
            o_hbm.at[b, pl.ds(r0, nr), pl.ds(j * _L, _L)], sem_o.at[0])

    def start_out(b, cp, r0, nr):
        for c in range(2):
            o_copies.append(out_copy(b, 2 * cp + c, r0, nr))
            o_copies[-1].start()

    keep = {}

    def tie(v, tok):
        if tok is None:
            return v
        if len(tok) == 2:
            tok.append({jnp.dtype(_F32): tok[0][tok[1]:tok[1] + 8]})
        if v.dtype not in tok[2]:
            tok[2][v.dtype] = pltpu.bitcast(tok[2][jnp.dtype(_F32)], v.dtype)
        t = tok[2][v.dtype]
        n = v.shape[0]
        if S['gmask'] == 0 or n not in keep:
            keep[n] = cat([zer[...]] * (n // 8)) == 0
        return jax.lax.select(keep[n], v, cat([t] * (n // 8)))

    sh16 = jnp.full((8, _L), 16, _U32)
    mk16 = jnp.full((8, _L), 0xFFFF0000, _U32)

    def unpackers(tok):
        sh, mk = cat([tie(sh16, tok)] * 2), cat([tie(mk16, tok)] * 2)
        return (lambda u: pltpu.bitcast(u << sh, _F32),
                lambda u: pltpu.bitcast(u & mk, _F32))

    def pack(lo, hi):
        return pltpu.pack_elementwise([lo, hi], packed_dtype=_BF16)

    def cat(vs, axis=0):
        return vs[0] if len(vs) == 1 else jnp.concatenate(vs, axis=axis)

    have = set()

    def x_job(b, g, q, h, phases):
        def words(half, ct, o):
            t = g * _RG + 32 * half + 16 * h
            xu = xb.at[b, ct, pl.ds(4 * t, 64), :].bitcast(_U32)
            return cat([xu[pl.ds(2 * par + o, 8, stride=4), :] for par in range(2)])

        blocks = [(half, ct) for half in range(2) for ct in (2 * q, 2 * q + 1)]
        for phase in phases:
            if phase < 2:
                lo, hi = unpackers((yield 27))
                if phase == 0:
                    outs = {0: [lo(words(*bl, 0)) for bl in blocks]}
                else:
                    outs = {5: [hi(words(*bl, 1)) for bl in blocks]}
            else:
                c = _A if phase == 2 else _B
                p = 2 * phase - 3
                outs = {p: [], p + 1: []}
                for bl in blocks:
                    lo, hi = unpackers((yield 42 if bl == blocks[-1] else 25))
                    we, wo = words(*bl, 0), words(*bl, 1)
                    e = lo(we) + (c * c) * lo(wo)
                    o = c * hi(we) + (c * c * c) * hi(wo)
                    outs[p].append(e + o)
                    outs[p + 1].append(e - o)
            for p, (a11, a12, a21, a22) in outs.items():
                if phase >= 2 and p % 2 == 0:
                    tok = yield 22
                    a11, a22 = tie(a11, tok), tie(a22, tok)
                ss = (a11 - a22, a21 - a22, a11, a22, a11 - a12, a21 - a11,
                      a12 - a22)
                for i, s in enumerate(ss):
                    r = 16 * g + 8 * h
                    xs[p, i, b, r:r + 8, q * _L:(q + 1) * _L] = pack(
                        s[0:8], s[8:16])
                have.add(('x', p, b, g, q, h))

    def w_job(cp, q, kk, phases):
        def vals(tap, j, lo, hi):
            u = cat([wr.at[j, tap, pl.ds(ct * _L + 16 * kk, 16), :].bitcast(_U32)[...]
                     for ct in (2 * q, 2 * q + 1)])
            return cat([lo(u), hi(u)])

        j1, j2 = 2 * cp, 2 * cp + 1
        gh = 0.5 * _GAM
        for phase in phases:
            if phase < 2:
                lo, hi = unpackers((yield 34))
                tap = 2 if phase == 0 else 0
                p = 0 if phase == 0 else 5
                outs = {p: (gh * vals(tap, j1, lo, hi), vals(tap, j2, lo, hi))}
            else:
                c, lam = (_A, _LA) if phase == 2 else (_B, _LB)
                p = 2 * phase - 3
                uv = []
                for j, s in ((j1, gh * lam), (j2, lam)):
                    lo, hi = unpackers((yield 39))
                    e = s * vals(2, j, lo, hi) + (s * c * c) * vals(0, j, lo, hi)
                    o = (s * c) * vals(1, j, lo, hi)
                    uv.append((e + o, e - o))
                outs = {p: (uv[0][0], uv[1][0]), p + 1: (uv[0][1], uv[1][1])}
            for p, (u, v) in outs.items():
                half = jnp.full((8, _L), 0.5, _F32)
                if phase >= 2:
                    half = tie(half, (yield 23))
                half = cat([half] * 2)
                sel = lambda a, n: cat(
                    [a[8 * n:8 * n + 8], a[16 + 8 * n:24 + 8 * n]])
                u1, u2, v1, v2 = sel(u, 0), sel(u, 1), sel(v, 0), sel(v, 1)
                t2 = half * v1 + u1
                t5 = half * v2 - u2
                t1 = t2 - t5
                ts = [t1, t2, v1 - t1, v2 + t1, t5]
                if phase >= 2:
                    ts += [v1, v2]
                for i, t in enumerate(ts):
                    r = 64 * q + 8 * kk
                    ws[cp, p, i, r:r + 8, :] = pack(t[0:8], t[8:16])
                have.add(('w', p, cp, q, kk))

    def lhs(p, i, b, gs, qs):
        return pltpu.bitcast(
            xs[p, i, b, 16 * gs[0]:16 * (gs[-1] + 1),
               qs[0] * _L:(qs[-1] + 1) * _L], _BF16)

    def rhs(p, i, cp, qs):
        if p in (0, 5) and i >= 5:
            r = cat([wr.at[2 * cp + 1, 2 if p == 0 else 0,
                           pl.ds((2 * q + i - 5) * _L, _L), :].bitcast(_U32)[...]
                     for q in qs])
        else:
            r = ws[cp, p, i, 64 * qs[0]:64 * (qs[-1] + 1), :]
        return pltpu.bitcast(r, _BF16)

    def ep_job(acc, b, cp, blk, out=None):
        q = _HALO + 8 * blk
        ys = []
        for c in range(2):
            def ld(p, o=0, c=c):
                return acc[c, p, q + o:q + o + 8, :]

            m, mb = tie(ld(4), (yield 24)), ld(3)
            db = mb - m
            sb = mb + m
            ma, mna, z0, z5 = ld(1), ld(2), ld(0), ld(5)
            y0 = (_B * (((_A / _B) * db - ma) + mna) + z5) + ld(5, -1)
            t2 = (_A / _C) * ((ma - (_B / _A) * db) - mna) - z5
            z4 = ((ma - sb) + mna) + z0
            y3 = z4 + ld(0, 1)
            y1 = _A2 * (sb - z0) - _B2 * (z4 + sb)
            ys.append((y0, y1, t2, y3))
        for c in range(2):
            j = 2 * cp + c
            tok = yield 25
            sc, scc, sh = tie(scsh[0, j], tok), tie(scsh[1, j], tok), scsh[2, j]
            os_ = []
            for k in range(4):
                y = ys[0][k] - ys[1][k] if c == 0 else ys[0][k] + ys[1][k]
                h = y * (scc if k == 2 else sc) + sh
                os_.append(h * jnp.tanh(h) + h)
            o_ = ob.at[b * nct + j]
            o_[pl.ds(16 * blk, 8, stride=2), :] = pack(os_[0], os_[1])
            o_[pl.ds(16 * blk + 1, 8, stride=2), :] = pack(os_[2], os_[3])
        if out:
            start_out(b, cp, *out)

    epq = []
    bg = dict(jobs=[], every=0, rate=2.0, budget=0.0, since=0, active=None,
              cost=0, tok=None, late=0)

    def fetch(force=False):
        if bg['active'] is None:
            if bg['jobs'] and (force or bg['since'] >= bg['every']):
                bg['since'] = min(bg['since'] - bg['every'], 4 * bg['every'])
                bg['active'] = bg['jobs'].pop(0)
                bg['cap'] = 4.0
            elif epq:
                bg['active'] = epq.pop(0)
                bg['cap'] = S['rep']
            else:
                return False
            bg['cost'] = next(bg['active'])
        return True

    def advance(tok, force=False):
        if fetch(force):
            try:
                bg['cost'] = bg['active'].send(tok)
            except StopIteration:
                bg['active'] = None

    def clock(tok, cycles):
        bg['since'] += cycles
        bg['tok'] = tok
        if not fetch():
            bg['budget'] = 0.0
            return
        bg['budget'] += min(bg['rate'], bg['cap']) * cycles
        if bg['budget'] >= bg['cost']:
            bg['budget'] = min(bg['budget'] - bg['cost'], 16.0)
            advance(tok)

    def burst(ops):
        while ops > 0 and fetch():
            ops -= bg['cost']
            advance(None)

    def require(keys):
        while not all(k in have for k in keys):
            assert bg['active'] is not None or bg['jobs'], keys
            bg['late'] += 1
            advance(bg['tok'], force=True)

    def drain():
        bg['every'] = 0
        while bg['active'] is not None or epq or bg['jobs']:
            bg['late'] += 1
            advance(bg['tok'])

    def background(jobs, rate, span=0):
        bg['jobs'] += jobs
        every = span // max(len(bg['jobs']), 1)
        bg.update(every=every, rate=rate, since=every)

    def run_now(jobs):
        for j in jobs:
            for _ in j:
                pass

    def jit(jobs, n_eager, rate):
        run_now(jobs[:n_eager])
        background(jobs[n_eager:], rate)

    def xj(b, gs, qs, phases=(0, 1, 2, 3), by_phase=False):
        if by_phase:
            return [j for ph in phases for j in xj(b, gs, qs, (ph,))]
        return [x_job(b, g, q, h, phases) for g in gs for q in qs for h in range(2)]

    def wj(cp, qs, phases=(0, 1, 2, 3), by_phase=False):
        if by_phase:
            return [j for ph in phases for j in wj(cp, qs, (ph,))]
        return [w_job(cp, q, kk, phases) for q in qs for kk in range(8)]

    class Col:
        def __init__(self, b, cp, out_rows):
            self.b, self.cp, self.out_rows = b, cp, out_rows
            self.acc = acc.at[cp]
            self.todo = list(range(nblk))
            self.sent = 0
            self.jobs = []
            self.full = {p: set() for p in range(6)}
            self.kdone = {}

        def flush(self):
            f = self.full
            ready = [r for r in self.todo
                     if all(r in f[p] for p in range(6))
                     and (r + 1 == nblk or r + 1 in f[0])
                     and (r == 0 or r - 1 in f[5])]
            for r in ready:
                self.todo.remove(r)
                e = min(self.todo, default=nblk)
                out = None
                if r == ready[-1] and (e == nblk or
                                       32 * (e - self.sent) >= self.out_rows):
                    out = (32 * self.sent, 32 * (e - self.sent))
                    self.sent = e
                self.jobs.append(ep_job(self.acc, self.b, self.cp, r, out))
                epq.append(self.jobs[-1])

        def finished(self):
            return not self.todo and not any(
                j in epq or j is bg['active'] for j in self.jobs)

    def tiles(subs, qs, two_phase=False, hooks=None):
        hooks = hooks or {}
        subs = [(c, i if isinstance(i, tuple) else (i,)) for c, i in subs]
        fl = {(i not in c.kdone, c.kdone.get(i, 0) + len(qs) == nq) for c, i in subs}
        assert len(fl) == 1
        first, last = fl.pop()
        for c, i in subs:
            c.kdone[i] = c.kdone.get(i, 0) + len(qs)
        held = []

        def release():
            for k in range(0, held[0].shape[0], 8):
                for r in held:
                    clock([r, k], 2 * len(qs))
            held.clear()

        def prod(t, p, i):
            col, gs = t[0], tuple(range(2 * t[1][0], 2 * t[1][-1] + 2))
            require([('x', p, col.b, g, q, h)
                     for g in gs for q in qs for h in range(2)]
                    + [('w', p, col.cp, q, kk) for q in qs for kk in range(8)])
            r = jnp.dot(lhs(p, i, col.b, gs, qs), rhs(p, i, col.cp, qs),
                        preferred_element_type=_F32)
            held.append(r)
            if len(held) * len(qs) >= 4:
                release()
            return r

        def put(t, p, half, c, v, init, final):
            col = t[0]
            for n, g in enumerate(range(2 * t[1][0], 2 * t[1][-1] + 2)):
                q = _HALO + g * _RG + 32 * half
                part = v[32 * n:32 * n + 32]
                if not init:
                    part = part + col.acc[c, p, q:q + 32, :]
                col.acc[c, p, q:q + 32, :] = part
                if final and last and c == 1:
                    col.full[p].update(range(8 * g + 4 * half, 8 * g + 4 * half + 4))

        def upper(t, p):
            p1 = prod(t, p, 0)
            c11 = p1 + prod(t, p, 6)
            p4 = prod(t, p, 3)
            c11 = c11 + p4
            p3 = prod(t, p, 2)
            c22 = p1 + p3
            p5 = prod(t, p, 4)
            put(t, p, 0, 0, c11 + p5, first, True)
            put(t, p, 0, 1, p3 - p5, first, True)
            if not two_phase:
                return p4, c22
            put(t, p, 1, 0, p4, first, False)
            put(t, p, 1, 1, c22, first, False)

        def lower(t, p, part=None):
            p6 = prod(t, p, 5)
            if part:
                p6 = p6 + part[1]
            p2 = prod(t, p, 1)
            put(t, p, 1, 0, p2 + part[0] if part else p2, first and part, True)
            put(t, p, 1, 1, p6 - p2, first and part, True)

        def flush():
            if held:
                release()
            for c, _ in subs:
                c.flush()

        if two_phase:
            for p in _POINTS:
                for t in subs:
                    upper(t, p)
            flush()
            for p in _POINTS:
                for t in subs:
                    lower(t, p)
        else:
            for n, p in enumerate(_POINTS):
                if n in hooks:
                    flush()
                    hooks[n]()
                for t in subs:
                    lower(t, p, upper(t, p))
        flush()

    XR = 8 * _RG
    allq = tuple(range(nq))
    G = lambda i: (2 * i, 2 * i + 1)
    X = lambda i, *qs: ('X', 0, i * XR, XR, qs)
    W = lambda cp, *qs: ('W', cp, qs)

    col0 = [Col(0, cp, seq) for cp in range(ncp)]

    def params():
        mean, var, gam, bet = (
            pbuf[i][...].astype(_F32).reshape(1, ch) for i in range(4))
        s = gam * jax.lax.rsqrt(var + _EPS)
        col = jax.lax.broadcasted_iota(jnp.int32, (1, ch), 1)
        sm = jnp.where((col & _L) == 0, s * (1.0 / _GAM), s)
        for k, v in enumerate((0.5 * sm, (0.5 * _C) * sm, 0.5 * (bet - mean * s))):
            for j in range(nct):
                scsh[k, j] = jnp.broadcast_to(v[:, j * _L:(j + 1) * _L], (8, _L))

    def kt(subs, qs, hooks=None):
        tiles([(col0[cp], i) for i, cp in subs], qs, hooks=hooks)

    def get(group, jobs, rate, fetch=()):
        def f():
            fetch_in(*fetch)
            arrive(group)
            background(jobs(), rate)
            burst(S['ehead'])
        return f

    qb = allq[2:]
    if S['ramp'] == 2:
        qr = allq[1:]
        q0 = [(X(0, 0),), (X(1, 0), X(2, 0)), (X(3, 0), W(1, 0)), (W(2, 0),)]
        A1, B1 = (W(0, 1), X(0, 1), X(1, 1)), (X(2, 1), X(3, 1), W(1, 1))
        Ab, Bb = (W(0, *qb), X(0, *qb), ('P',)), (X(1, *qb), W(1, *qb))
        Cb = (X(2, *qb), X(3, *qb))
        w23, x1 = (W(2, *qr), W(3, *allq)), (('X', 1, 0, seq, allq),)
        fetch_in((W(0, 0),))
        zsrc[...] = jnp.zeros((8, _L), _U32)
        fetch_in((('Z',),), *q0, A1, B1)
        zero = jnp.zeros((_HALO, _L), _F32)
        for cp in range(ncp):
            for c in range(2):
                acc[cp, c, 0, _HALO + T:2 * _HALO + T, :] = zero
                acc[cp, c, 5, 0:_HALO, :] = zero
        arrive((W(0, 0),), (('Z',),))
        run_now(wj(0, (0,)))
        arrive(q0[0])
        jit(xj(0, G(0), (0,), by_phase=True), S['n1'], S['r1'])
        kt([(0, 0)], (0,))
        fetch_in(Ab)
        arrive(q0[1])
        jit(xj(0, G(1) + G(2), (0,), by_phase=True), S['n3'], S['r2'])
        kt([(1, 0), (2, 0)], (0,))
        arrive(q0[2])
        jit(xj(0, G(3), (0,), by_phase=True), S['n1'], S['r1'])
        background(wj(1, (0,), by_phase=True), S['r1'])
        kt([(3, 0)], (0,))
        background([], S['r2'])
        kt([(i, 1) for i in range(4)], (0,), hooks={S['h0']: get(
            q0[3], lambda: wj(2, (0,), by_phase=True), S['ra'], (Bb, Cb))})
        kt([(i, 2) for i in range(4)], (0,), hooks={S['h1']: get(
            A1, lambda: wj(0, (1,), by_phase=True)
            + xj(0, G(0) + G(1), (1,), by_phase=S['bp'] & 1), S['ra'])})

        kt([(0, 0), (1, 0)], (1,), hooks={S['hb']: get(
            B1, lambda: xj(0, G(2) + G(3), (1,), by_phase=S['bp'] & 2)
            + wj(1, (1,), by_phase=True), S['ra'], (w23, x1))})
        kt([(2, 0), (3, 0)], (1,))
        kt([(i, 1) for i in range(4)], (1,), hooks={S['h2']: get(
            Ab, lambda: [j for ph in range(4) for j in
                         wj(0, qb, (ph,)) + xj(0, G(0), qb, (ph,))]
            if S['bp'] & 4 else xj(0, G(0), qb) + wj(0, qb, by_phase=True),
            S['r3'])})
        params()
        kt([(0, 0)], qb, hooks={S['hc']: get(
            Bb, lambda: xj(0, G(1), qb, by_phase=S['bp'] & 8)
            + wj(1, qb, by_phase=True), S['r7'])})
        kt([(1, 0)], qb)
        kt([(0, 1), (1, 1)], qb, hooks={S['h3']: get(
            Cb, lambda: xj(0, G(2), qb, by_phase=S['bp'] & 16) + xj(0, G(3), qb),
            S['r6'])})
        kt([(2, 0)], qb)
        kt([(3, 0)], qb)
        kt([(2, 1)], qb, hooks={S['h4']: get(
            w23, lambda: wj(2, qr, by_phase=True), S['r4'])})
        kt([(3, 1)], qb)
        q2 = qr
    else:
        q0 = {0: [(X(0, 0),), (X(1, 0),), (X(2, 0), X(3, 0)), (W(1, 0),)],
              1: [(X(0, 0),), (X(1, 0), X(2, 0)), (X(3, 0), W(1, 0))]}[S['ramp']]
        A1, B1 = (W(0, 1), X(0, 1), X(1, 1)), (X(2, 1), X(3, 1), W(1, 1))
        Ab, Bb = (W(0, *qb), X(0, *qb), ('P',)), (X(1, *qb), W(1, *qb))
        Cb = (X(2, *qb), X(3, *qb))
        w23, x1 = (W(2, *allq), W(3, *allq)), (('X', 1, 0, seq, allq),)
        fetch_in((W(0, 0),))
        zsrc[...] = jnp.zeros((8, _L), _U32)
        fetch_in((('Z',),), *q0, A1, B1, Ab)
        zero = jnp.zeros((_HALO, _L), _F32)
        for cp in range(ncp):
            for c in range(2):
                acc[cp, c, 0, _HALO + T:2 * _HALO + T, :] = zero
                acc[cp, c, 5, 0:_HALO, :] = zero

        hook_a1 = {S['h1']: get(
            A1, lambda: wj(0, (1,), by_phase=True)
            + xj(0, G(0) + G(1), (1,), by_phase=True), S['r3'])}
        arrive((W(0, 0),), (('Z',),))
        run_now(wj(0, (0,)))
        arrive(q0[0])
        jit(xj(0, G(0), (0,), by_phase=True), S['n1'], S['r1'])
        kt([(0, 0)], (0,))
        arrive(q0[1])
        if S['ramp'] == 0:
            jit(xj(0, G(1), (0,), by_phase=True), S['n1'], S['r1'])
            kt([(1, 0)], (0,))
            arrive(q0[2])
            fetch_in(Bb, Cb)
            jit(xj(0, G(2) + G(3), (0,), by_phase=True), S['n3'], S['r2'])
            kt([(2, 0), (3, 0)], (0,))
            arrive(q0[3])
            jit(wj(1, (0,), by_phase=True), S['n2'], S['r2'])
        else:
            jit(xj(0, G(1) + G(2), (0,), by_phase=True), S['n3'], S['r2'])
            kt([(1, 0), (2, 0)], (0,))
            arrive(q0[2])
            fetch_in(Bb, Cb)
            jit(xj(0, G(3), (0,), by_phase=True), S['n1'], S['r1'])
            background(wj(1, (0,), by_phase=True), S['r1'])
            kt([(3, 0)], (0,))
            background([], S['r2'])
        kt([(i, 1) for i in range(4)], (0,), hooks=hook_a1)
        kt([(0, 0), (1, 0)], (1,))
        arrive(B1)
        fetch_in(w23, x1)
        jit(xj(0, G(2) + G(3), (1,), by_phase=True), S['n3'], S['r2'])
        background(wj(1, (1,), by_phase=True), S['r2'])
        kt([(2, 0), (3, 0)], (1,))
        kt([(i, 1) for i in range(4)], (1,), hooks={S['h2']: get(
            Ab, lambda: [j for ph in range(4) for j in
                         wj(0, qb, (ph,)) + xj(0, G(0), qb, (ph,))], S['r3'])})
        params()
        kt([(0, 0)], qb)
        arrive(Bb)
        jit(xj(0, G(1), qb, by_phase=True), S['n4'], S['r7'])
        background(wj(1, qb, by_phase=True), S['r7'])
        kt([(1, 0)], qb)
        kt([(0, 1), (1, 1)], qb, hooks={S['h3']: get(
            Cb, lambda: xj(0, G(2), qb, by_phase=True) + xj(0, G(3), qb), S['r6'])})
        kt([(2, 0)], qb)
        kt([(3, 0)], qb)
        kt([(2, 1)], qb)
        kt([(3, 1)], qb, hooks={S['h4']: get(
            w23, lambda: wj(2, allq, by_phase=True), S['r4'])})
        q2 = allq
    if S['trunc']:
        kt([(0, 2), (1, 2)], q2)
        drain()
        arrive(x1)
        wait(o_copies)
        for n in range(24 if S['trunc'] == 2 else 0):
            for u in range(32):
                acc[3, 0, 1, 8:72, :] = jnp.dot(
                    lhs(u % 6, u % 7, 0, (0, 1), allq), rhs(1, u % 7, 0, allq),
                    preferred_element_type=_F32) + acc[3, 0, 1, 8:72, :]
            fetch_in((('Z',),))
            arrive((('Z',),))
        return
    kt([(i, 2) for i in range(4)], q2, hooks={4: lambda: background(
        wj(3, allq, by_phase=True), S['r4'])})
    kt([(i, 3) for i in range(4)], allq, hooks={S['h5']: get(
        x1, lambda: xj(1, G(0), allq), S['r4'])})

    col1 = [Col(1, cp, 256) for cp in range(ncp)]
    for i in range(4):
        if i < 3:
            background(xj(1, G(i + 1), allq), S['r5'], 4 * 2688 - 512)
        for cp in range(ncp):
            assert col0[cp].finished()
            tiles([(col1[cp], i)], allq, two_phase=True)
    bg['tok'] = None
    drain()
    wait(o_copies)


@jax.jit
def pallas_standalone__batchnorm__prompt_kernel(
    x: jax.Array,
    w: jax.Array,
    mean: jax.Array,
    var: jax.Array,
    g: jax.Array,
    b: jax.Array,
):
    nb, seq, ch = x.shape
    T = seq // 4
    nct = ch // _L

    def kernel(*refs):
        _kernel(*refs, nb=nb, seq=seq, ch=ch)

    any_spec = pl.BlockSpec(memory_space=pl.ANY)
    return pl.pallas_call(
        kernel,
        out_shape=jax.ShapeDtypeStruct(x.shape, x.dtype),
        in_specs=[any_spec] * 6,
        out_specs=any_spec,
        scratch_shapes=[
            pltpu.VMEM((nb, nct, seq, _L), _BF16),
            pltpu.VMEM((nct, 3, ch, _L), _BF16),
            pltpu.VMEM((ch,), _BF16),
            pltpu.VMEM((ch,), _BF16),
            pltpu.VMEM((ch,), _BF16),
            pltpu.VMEM((ch,), _BF16),
            pltpu.VMEM((6, 7, nb, T // 4, ch // 2), _U32),
            pltpu.VMEM((nct // 2, 6, 7, ch // 4, _L), _U32),
            pltpu.VMEM((nct // 2, 2, 6, T + 2 * _HALO, _L), _F32),
            pltpu.VMEM((nb * nct, seq // 2, _L), _U32),
            pltpu.VMEM((3, nct, 8, _L), _F32),
            pltpu.VMEM((8, _L), _U32),
            pltpu.VMEM((8, _L), _U32),
            pltpu.SemaphoreType.DMA((10,)),
            pltpu.SemaphoreType.DMA((1,)),
        ],
        compiler_params=pltpu.CompilerParams(vmem_limit_bytes=110 * 1024 * 1024),
    )(x, w, mean, var, g, b)
```

```python
import jax
import jax.numpy as jnp
import jax.experimental.pallas as pl
import jax.experimental.pallas.tpu as pltpu

_A = 1.5
_B = 1.0 / _A
_A2 = _A * _A
_B2 = _B * _B
_C = _A2 + _B2
_LA = 1.0 / (2.0 * _A2 * (_A2 - _B2))
_LB = 1.0 / (2.0 * _B2 * (_A2 - _B2))
_GAM = 1.35
_EPS = 1e-5
_L = 128
_HALO = 8
_RG = 64
_POINTS = (0, 5, 1, 2, 3, 4)

_F32 = jnp.float32
_BF16 = jnp.bfloat16
_U32 = jnp.uint32

CFG = dict(r1=3.5, r2=3.3,
           r3=2.8, r4=2.0,
           r5=1.8, r6=2.5,
           n1=8, n2=8,
           n3=8, h1=1,
           h2=0, h3=0,
           h4=1, h5=3,
           rep=1.8, r7=2.8, n4=16,
           ehead=350, ramp=2,
           h0=2, hb=0, hc=0, ra=2.3,
           fp=1, bp=2, lastrows=128, split=1, rlast=2.8, gmask=1, trunc=0)


def _kernel(x_hbm, w_hbm, mean_hbm, var_hbm, g_hbm, b_hbm, o_hbm,
            xb, wr, pb0, pb1, pb2, pb3, xs, ws, acc, ob, scsh, zsrc, zer,
            sem_i, sem_o, *, nb, seq, ch):
    assert nb == 2 and seq == 32 * _RG and ch == 8 * _L
    pbuf = (pb0, pb1, pb2, pb3)
    T = seq // 4
    nct = ch // _L
    ncp = nct // 2
    nq = nct // 2
    nblk = T // 8
    S = CFG

    free_sems = list(range(sem_i.shape[0]))
    inflight = {}

    def copies(name, sem):
        kind = name[0]
        if kind == 'X':
            _, b, r0, nr, qs = name
            return [pltpu.make_async_copy(
                x_hbm.at[b, pl.ds(r0, nr), pl.ds(ct * _L, _L)],
                xb.at[b, ct, pl.ds(r0, nr), :], sem)
                for ct in range(2 * qs[0], 2 * qs[-1] + 2)]
        if kind == 'W':
            _, cp, qs = name
            k0, nk = 2 * _L * qs[0], 2 * _L * len(qs)
            return [pltpu.make_async_copy(
                w_hbm.at[k, pl.ds(k0, nk), pl.ds(j * _L, _L)],
                wr.at[j, k, pl.ds(k0, nk), :], sem)
                for k in (2, 0, 1) for j in (2 * cp, 2 * cp + 1)]
        if kind == 'P':
            return [pltpu.make_async_copy(src, pbuf[i], sem) for i, src in
                    enumerate((mean_hbm, var_hbm, g_hbm, b_hbm))]
        return [pltpu.make_async_copy(zsrc, d, sem) for d in (
            zer, xs.at[4 * nb - 1, 5, 6, pl.ds(0, 8), pl.ds(0, _L)],
            ws.at[ncp - 1, 4, 6, pl.ds(0, 8), :])]

    def fetch_in(*groups):
        for names in groups:
            k = free_sems.pop(0)
            cs = [c for n in names for c in copies(n, sem_i.at[k])]
            inflight[names] = (k, cs)
            for c in cs:
                c.start()

    def arrive(*groups):
        for names in groups:
            k, cs = inflight.pop(names)
            wait(cs)
            free_sems.append(k)

    def wait(cs):
        bg['tok'] = None
        for c in cs:
            c.wait()

    o_copies = []

    def out_copy(b, j, r0, nr):
        return pltpu.make_async_copy(
            ob.at[b * nct + j, pl.ds(r0 // 2, nr // 2), :].bitcast(_BF16),
            o_hbm.at[b, pl.ds(r0, nr), pl.ds(j * _L, _L)], sem_o.at[0])

    def start_out(b, cp, r0, nr):
        for c in range(2):
            o_copies.append(out_copy(b, 2 * cp + c, r0, nr))
            o_copies[-1].start()

    keep = {}

    def tie(v, tok):
        if tok is None:
            return v
        if len(tok) == 2:
            tok.append({jnp.dtype(_F32): tok[0][tok[1]:tok[1] + 8]})
        if v.dtype not in tok[2]:
            tok[2][v.dtype] = pltpu.bitcast(tok[2][jnp.dtype(_F32)], v.dtype)
        t = tok[2][v.dtype]
        n = v.shape[0]
        if S['gmask'] == 0 or n not in keep:
            keep[n] = cat([zer[...]] * (n // 8)) == 0
        return jax.lax.select(keep[n], v, cat([t] * (n // 8)))

    sh16 = jnp.full((8, _L), 16, _U32)
    mk16 = jnp.full((8, _L), 0xFFFF0000, _U32)

    def unpackers(tok):
        sh, mk = cat([tie(sh16, tok)] * 2), cat([tie(mk16, tok)] * 2)
        return (lambda u: pltpu.bitcast(u << sh, _F32),
                lambda u: pltpu.bitcast(u & mk, _F32))

    def pack(lo, hi):
        return pltpu.pack_elementwise([lo, hi], packed_dtype=_BF16)

    def cat(vs, axis=0):
        return vs[0] if len(vs) == 1 else jnp.concatenate(vs, axis=axis)

    have = set()

    def x_job(b, g, q, h, phases):
        def words(half, ct, o):
            t = g * _RG + 32 * half + 16 * h
            xu = xb.at[b, ct, pl.ds(4 * t, 64), :].bitcast(_U32)
            return cat([xu[pl.ds(2 * par + o, 8, stride=4), :] for par in range(2)])

        blocks = [(half, ct) for half in range(2) for ct in (2 * q, 2 * q + 1)]
        for phase in phases:
            if phase < 2:
                lo, hi = unpackers((yield 27))
                if phase == 0:
                    outs = {0: [lo(words(*bl, 0)) for bl in blocks]}
                else:
                    outs = {5: [hi(words(*bl, 1)) for bl in blocks]}
            else:
                c = _A if phase == 2 else _B
                p = 2 * phase - 3
                outs = {p: [], p + 1: []}
                for bl in blocks:
                    lo, hi = unpackers((yield 42 if bl == blocks[-1] else 25))
                    we, wo = words(*bl, 0), words(*bl, 1)
                    e = lo(we) + (c * c) * lo(wo)
                    o = c * hi(we) + (c * c * c) * hi(wo)
                    outs[p].append(e + o)
                    outs[p + 1].append(e - o)
            for p, (a11, a12, a21, a22) in outs.items():
                if phase >= 2 and p % 2 == 0:
                    tok = yield 22
                    a11, a22 = tie(a11, tok), tie(a22, tok)
                ss = (a11 - a22, a21 - a22, a11, a22, a11 - a12, a21 - a11,
                      a12 - a22)
                for i, s in enumerate(ss):
                    r = 16 * (g % 2) + 8 * h
                    xs[4 * b + g // 2, p, i, r:r + 8, q * _L:(q + 1) * _L] = pack(
                        s[0:8], s[8:16])
                have.add(('x', p, b, g, q, h))

    def w_job(cp, q, kk, phases):
        def vals(tap, j, lo, hi):
            u = cat([wr.at[j, tap, pl.ds(ct * _L + 16 * kk, 16), :].bitcast(_U32)[...]
                     for ct in (2 * q, 2 * q + 1)])
            return cat([lo(u), hi(u)])

        j1, j2 = 2 * cp, 2 * cp + 1
        gh = 0.5 * _GAM
        for phase in phases:
            if phase < 2:
                lo, hi = unpackers((yield 34))
                tap = 2 if phase == 0 else 0
                p = 0 if phase == 0 else 5
                outs = {p: (gh * vals(tap, j1, lo, hi), vals(tap, j2, lo, hi))}
            else:
                c, lam = (_A, _LA) if phase == 2 else (_B, _LB)
                p = 2 * phase - 3
                uv = []
                for j, s in ((j1, gh * lam), (j2, lam)):
                    lo, hi = unpackers((yield 39))
                    e = s * vals(2, j, lo, hi) + (s * c * c) * vals(0, j, lo, hi)
                    o = (s * c) * vals(1, j, lo, hi)
                    uv.append((e + o, e - o))
                outs = {p: (uv[0][0], uv[1][0]), p + 1: (uv[0][1], uv[1][1])}
            for p, (u, v) in outs.items():
                half = jnp.full((8, _L), 0.5, _F32)
                if phase >= 2:
                    half = tie(half, (yield 23))
                half = cat([half] * 2)
                sel = lambda a, n: cat(
                    [a[8 * n:8 * n + 8], a[16 + 8 * n:24 + 8 * n]])
                u1, u2, v1, v2 = sel(u, 0), sel(u, 1), sel(v, 0), sel(v, 1)
                t2 = half * v1 + u1
                t5 = half * v2 - u2
                t1 = t2 - t5
                ts = [t1, t2, v1 - t1, v2 + t1, t5]
                if phase >= 2:
                    ts += [v1, v2]
                for i, t in enumerate(ts):
                    r = 64 * q + 8 * kk
                    ws[cp, p, i, r:r + 8, :] = pack(t[0:8], t[8:16])
                have.add(('w', p, cp, q, kk))

    def lhs(p, i, b, gs, qs):
        return pltpu.bitcast(
            xs[4 * b + gs[0] // 2, p, i, 16 * (gs[0] % 2):16 * (gs[-1] % 2 + 1),
               qs[0] * _L:(qs[-1] + 1) * _L], _BF16)

    def rhs(p, i, cp, qs):
        if p in (0, 5) and i >= 5:
            r = cat([wr.at[2 * cp + 1, 2 if p == 0 else 0,
                           pl.ds((2 * q + i - 5) * _L, _L), :].bitcast(_U32)[...]
                     for q in qs])
        else:
            r = ws[cp, p, i, 64 * qs[0]:64 * (qs[-1] + 1), :]
        return pltpu.bitcast(r, _BF16)

    def ep_job(acc, b, cp, blk, out=None):
        q = _HALO + 8 * blk
        ys = []
        for c in range(2):
            def ld(p, o=0, c=c):
                return acc[c, p, q + o:q + o + 8, :]

            m, mb = tie(ld(4), (yield 24)), ld(3)
            db = mb - m
            sb = mb + m
            ma, mna, z0, z5 = ld(1), ld(2), ld(0), ld(5)
            y0 = (_B * (((_A / _B) * db - ma) + mna) + z5) + ld(5, -1)
            t2 = (_A / _C) * ((ma - (_B / _A) * db) - mna) - z5
            z4 = ((ma - sb) + mna) + z0
            y3 = z4 + ld(0, 1)
            y1 = _A2 * (sb - z0) - _B2 * (z4 + sb)
            ys.append((y0, y1, t2, y3))
        for c in range(2):
            j = 2 * cp + c
            tok = yield 25
            sc, scc, sh = tie(scsh[0, j], tok), tie(scsh[1, j], tok), scsh[2, j]
            os_ = []
            for k in range(4):
                y = ys[0][k] - ys[1][k] if c == 0 else ys[0][k] + ys[1][k]
                h = y * (scc if k == 2 else sc) + sh
                os_.append(h * jnp.tanh(h) + h)
            o_ = ob.at[b * nct + j]
            o_[pl.ds(16 * blk, 8, stride=2), :] = pack(os_[0], os_[1])
            o_[pl.ds(16 * blk + 1, 8, stride=2), :] = pack(os_[2], os_[3])
        if out:
            start_out(b, cp, *out)

    epq = []
    bg = dict(jobs=[], every=0, rate=2.0, budget=0.0, since=0, active=None,
              cost=0, tok=None, late=0, rep=S['rep'])

    def fetch(force=False):
        if bg['active'] is None:
            if bg['jobs'] and (force or bg['since'] >= bg['every']):
                bg['since'] = min(bg['since'] - bg['every'], 4 * bg['every'])
                bg['active'] = bg['jobs'].pop(0)
                bg['cap'] = 4.0
            elif epq:
                bg['active'] = epq.pop(0)
                bg['cap'] = bg['rep']
            else:
                return False
            bg['cost'] = next(bg['active'])
        return True

    def advance(tok, force=False):
        if fetch(force):
            try:
                bg['cost'] = bg['active'].send(tok)
            except StopIteration:
                bg['active'] = None

    def clock(tok, cycles):
        bg['since'] += cycles
        bg['tok'] = tok
        if not fetch():
            bg['budget'] = 0.0
            return
        bg['budget'] += min(bg['rate'], bg['cap']) * cycles
        if bg['budget'] >= bg['cost']:
            bg['budget'] = min(bg['budget'] - bg['cost'], 16.0)
            advance(tok)

    def burst(ops):
        while ops > 0 and fetch():
            ops -= bg['cost']
            advance(None)

    def require(keys):
        while not all(k in have for k in keys):
            assert bg['active'] is not None or bg['jobs'], keys
            bg['late'] += 1
            advance(bg['tok'], force=True)

    def drain():
        bg['every'] = 0
        while bg['active'] is not None or epq or bg['jobs']:
            bg['late'] += 1
            advance(bg['tok'])

    def background(jobs, rate, span=0):
        bg['jobs'] += jobs
        every = span // max(len(bg['jobs']), 1)
        bg.update(every=every, rate=rate, since=every)

    def run_now(jobs):
        for j in jobs:
            for _ in j:
                pass

    def jit(jobs, n_eager, rate):
        run_now(jobs[:n_eager])
        background(jobs[n_eager:], rate)

    def xj(b, gs, qs, phases=(0, 1, 2, 3), by_phase=False):
        if by_phase:
            return [j for ph in phases for j in xj(b, gs, qs, (ph,))]
        return [x_job(b, g, q, h, phases) for g in gs for q in qs for h in range(2)]

    def wj(cp, qs, phases=(0, 1, 2, 3), by_phase=False):
        if by_phase:
            return [j for ph in phases for j in wj(cp, qs, (ph,))]
        return [w_job(cp, q, kk, phases) for q in qs for kk in range(8)]

    class Col:
        def __init__(self, b, cp, out_rows):
            self.b, self.cp, self.out_rows = b, cp, out_rows
            self.acc = acc.at[cp]
            self.todo = list(range(nblk))
            self.sent = 0
            self.jobs = []
            self.full = {p: set() for p in range(6)}
            self.kdone = {}

        def flush(self):
            f = self.full
            ready = [r for r in self.todo
                     if all(r in f[p] for p in range(6))
                     and (r + 1 == nblk or r + 1 in f[0])
                     and (r == 0 or r - 1 in f[5])]
            for r in ready:
                self.todo.remove(r)
                e = min(self.todo, default=nblk)
                out = None
                if e == nblk or 32 * (e - self.sent) >= self.out_rows:
                    out = (32 * self.sent, 32 * (e - self.sent))
                    self.sent = e
                self.jobs.append(ep_job(self.acc, self.b, self.cp, r, out))
                epq.append(self.jobs[-1])

        def finished(self):
            return not self.todo and not any(
                j in epq or j is bg['active'] for j in self.jobs)

    def tiles(subs, qs, two_phase=False, hooks=None, split=False):
        hooks = hooks or {}
        subs = [(c, (2 * i, 2 * i + 1)) for c, i in subs]
        fl = {(i not in c.kdone, c.kdone.get(i, 0) + len(qs) == nq) for c, i in subs}
        assert len(fl) == 1
        first, last = fl.pop()
        for c, i in subs:
            c.kdone[i] = c.kdone.get(i, 0) + len(qs)
        held = []

        def release():
            for k in range(0, held[0].shape[0], 8):
                for r in held:
                    clock([r, k], 2 * len(qs))
            held.clear()

        def prod(t, p, i):
            col, gs = t
            require([('x', p, col.b, g, q, h)
                     for g in gs for q in qs for h in range(2)]
                    + [('w', p, col.cp, q, kk) for q in qs for kk in range(8)])
            r = jnp.dot(lhs(p, i, col.b, gs, qs), rhs(p, i, col.cp, qs),
                        preferred_element_type=_F32)
            held.append(r)
            if len(held) * len(qs) >= 4:
                release()
            return r

        def put(t, p, half, c, v, init, final):
            col = t[0]
            for n, g in enumerate(t[1]):
                q = _HALO + g * _RG + 32 * half
                part = v[32 * n:32 * n + 32]
                if not init:
                    part = part + col.acc[c, p, q:q + 32, :]
                col.acc[c, p, q:q + 32, :] = part
                if final and last and c == 1:
                    col.full[p].update(range(8 * g + 4 * half, 8 * g + 4 * half + 4))

        def upper(t, p):
            p1 = prod(t, p, 0)
            c11 = p1 + prod(t, p, 6)
            p4 = prod(t, p, 3)
            c11 = c11 + p4
            p3 = prod(t, p, 2)
            c22 = p1 + p3
            p5 = prod(t, p, 4)
            put(t, p, 0, 0, c11 + p5, first, True)
            put(t, p, 0, 1, p3 - p5, first, True)
            if not two_phase:
                return p4, c22
            put(t, p, 1, 0, p4, first, False)
            put(t, p, 1, 1, c22, first, False)

        def lower(t, p, part=None):
            p6 = prod(t, p, 5)
            if part:
                p6 = p6 + part[1]
            p2 = prod(t, p, 1)
            put(t, p, 1, 0, p2 + part[0] if part else p2, first and part, True)
            put(t, p, 1, 1, p6 - p2, first and part, True)

        def flush():
            if held:
                release()
            for c, _ in subs:
                c.flush()

        if two_phase:
            for p in _POINTS:
                for t in subs:
                    upper(t, p)
            for part in ([[(c, (g,))] for c, gs in subs for g in gs]
                         if split else [subs]):
                flush()
                for p in _POINTS:
                    for t in part:
                        lower(t, p)
        else:
            for n, p in enumerate(_POINTS):
                if n in hooks:
                    flush()
                    hooks[n]()
                for t in subs:
                    lower(t, p, upper(t, p))
        flush()

    XR = 8 * _RG
    allq = tuple(range(nq))
    G = lambda i: (2 * i, 2 * i + 1)
    X = lambda i, *qs: ('X', 0, i * XR, XR, qs)
    W = lambda cp, *qs: ('W', cp, qs)

    col0 = [Col(0, cp, seq) for cp in range(ncp)]

    def params():
        mean, var, gam, bet = (
            pbuf[i][...].astype(_F32).reshape(1, ch) for i in range(4))
        s = gam * jax.lax.rsqrt(var + _EPS)
        col = jax.lax.broadcasted_iota(jnp.int32, (1, ch), 1)
        sm = jnp.where((col & _L) == 0, s * (1.0 / _GAM), s)
        for k, v in enumerate((0.5 * sm, (0.5 * _C) * sm, 0.5 * (bet - mean * s))):
            for j in range(nct):
                scsh[k, j] = jnp.broadcast_to(v[:, j * _L:(j + 1) * _L], (8, _L))

    def kt(subs, qs, hooks=None):
        tiles([(col0[cp], i) for i, cp in subs], qs, hooks=hooks)

    def get(group, jobs, rate, fetch=()):
        def f():
            fetch_in(*fetch)
            arrive(group)
            background(jobs(), rate)
            burst(S['ehead'])
        return f

    qb = allq[2:]
    if S['ramp'] == 2:
        qr = allq[1:]
        q0 = [(X(0, 0),), (X(1, 0), X(2, 0)), (X(3, 0), W(1, 0)), (W(2, 0),)]
        A1, B1 = (W(0, 1), X(0, 1), X(1, 1)), (X(2, 1), X(3, 1), W(1, 1))
        Ab, Bb = (W(0, *qb), X(0, *qb), ('P',)), (X(1, *qb), W(1, *qb))
        Cb = (X(2, *qb), X(3, *qb))
        w23, x1 = (W(2, *qr), W(3, *allq)), (('X', 1, 0, seq, allq),)
        fetch_in((W(0, 0),))
        zsrc[...] = jnp.zeros((8, _L), _U32)
        fetch_in((('Z',),), *q0, A1, B1)
        zero = jnp.zeros((_HALO, _L), _F32)
        for cp in range(ncp):
            for c in range(2):
                acc[cp, c, 0, _HALO + T:2 * _HALO + T, :] = zero
                acc[cp, c, 5, 0:_HALO, :] = zero
        arrive((W(0, 0),), (('Z',),))
        run_now(wj(0, (0,)))
        arrive(q0[0])
        jit(xj(0, G(0), (0,), by_phase=True), S['n1'], S['r1'])
        kt([(0, 0)], (0,))
        fetch_in(Ab)
        arrive(q0[1])
        jit(xj(0, G(1) + G(2), (0,), by_phase=True), S['n3'], S['r2'])
        kt([(1, 0), (2, 0)], (0,))
        arrive(q0[2])
        jit(xj(0, G(3), (0,), by_phase=True), S['n1'], S['r1'])
        background(wj(1, (0,), by_phase=True), S['r1'])
        kt([(3, 0)], (0,))
        background([], S['r2'])
        kt([(i, 1) for i in range(4)], (0,), hooks={S['h0']: get(
            q0[3], lambda: wj(2, (0,), by_phase=True), S['ra'], (Bb, Cb))})
        kt([(i, 2) for i in range(4)], (0,), hooks={S['h1']: get(
            A1, lambda: wj(0, (1,), by_phase=True)
            + xj(0, G(0) + G(1), (1,), by_phase=S['bp'] & 1), S['ra'])})

        kt([(0, 0), (1, 0)], (1,), hooks={S['hb']: get(
            B1, lambda: xj(0, G(2) + G(3), (1,), by_phase=S['bp'] & 2)
            + wj(1, (1,), by_phase=True), S['ra'], (w23, x1))})
        kt([(2, 0), (3, 0)], (1,))
        kt([(i, 1) for i in range(4)], (1,), hooks={S['h2']: get(
            Ab, lambda: [j for ph in range(4) for j in
                         wj(0, qb, (ph,)) + xj(0, G(0), qb, (ph,))]
            if S['bp'] & 4 else xj(0, G(0), qb) + wj(0, qb, by_phase=True),
            S['r3'])})
        params()
        kt([(0, 0)], qb, hooks={S['hc']: get(
            Bb, lambda: xj(0, G(1), qb, by_phase=S['bp'] & 8)
            + wj(1, qb, by_phase=True), S['r7'])})
        kt([(1, 0)], qb)
        kt([(0, 1), (1, 1)], qb, hooks={S['h3']: get(
            Cb, lambda: xj(0, G(2), qb, by_phase=S['bp'] & 16) + xj(0, G(3), qb),
            S['r6'])})
        kt([(2, 0)], qb)
        kt([(3, 0)], qb)
        kt([(2, 1)], qb, hooks={S['h4']: get(
            w23, lambda: wj(2, qr, by_phase=True), S['r4'])})
        kt([(3, 1)], qb)
        q2 = qr
    else:
        q0 = {0: [(X(0, 0),), (X(1, 0),), (X(2, 0), X(3, 0)), (W(1, 0),)],
              1: [(X(0, 0),), (X(1, 0), X(2, 0)), (X(3, 0), W(1, 0))]}[S['ramp']]
        A1, B1 = (W(0, 1), X(0, 1), X(1, 1)), (X(2, 1), X(3, 1), W(1, 1))
        Ab, Bb = (W(0, *qb), X(0, *qb), ('P',)), (X(1, *qb), W(1, *qb))
        Cb = (X(2, *qb), X(3, *qb))
        w23, x1 = (W(2, *allq), W(3, *allq)), (('X', 1, 0, seq, allq),)
        fetch_in((W(0, 0),))
        zsrc[...] = jnp.zeros((8, _L), _U32)
        fetch_in((('Z',),), *q0, A1, B1, Ab)
        zero = jnp.zeros((_HALO, _L), _F32)
        for cp in range(ncp):
            for c in range(2):
                acc[cp, c, 0, _HALO + T:2 * _HALO + T, :] = zero
                acc[cp, c, 5, 0:_HALO, :] = zero

        hook_a1 = {S['h1']: get(
            A1, lambda: wj(0, (1,), by_phase=True)
            + xj(0, G(0) + G(1), (1,), by_phase=True), S['r3'])}
        arrive((W(0, 0),), (('Z',),))
        run_now(wj(0, (0,)))
        arrive(q0[0])
        jit(xj(0, G(0), (0,), by_phase=True), S['n1'], S['r1'])
        kt([(0, 0)], (0,))
        arrive(q0[1])
        if S['ramp'] == 0:
            jit(xj(0, G(1), (0,), by_phase=True), S['n1'], S['r1'])
            kt([(1, 0)], (0,))
            arrive(q0[2])
            fetch_in(Bb, Cb)
            jit(xj(0, G(2) + G(3), (0,), by_phase=True), S['n3'], S['r2'])
            kt([(2, 0), (3, 0)], (0,))
            arrive(q0[3])
            jit(wj(1, (0,), by_phase=True), S['n2'], S['r2'])
        else:
            jit(xj(0, G(1) + G(2), (0,), by_phase=True), S['n3'], S['r2'])
            kt([(1, 0), (2, 0)], (0,))
            arrive(q0[2])
            fetch_in(Bb, Cb)
            jit(xj(0, G(3), (0,), by_phase=True), S['n1'], S['r1'])
            background(wj(1, (0,), by_phase=True), S['r1'])
            kt([(3, 0)], (0,))
            background([], S['r2'])
        kt([(i, 1) for i in range(4)], (0,), hooks=hook_a1)
        kt([(0, 0), (1, 0)], (1,))
        arrive(B1)
        fetch_in(w23, x1)
        jit(xj(0, G(2) + G(3), (1,), by_phase=True), S['n3'], S['r2'])
        background(wj(1, (1,), by_phase=True), S['r2'])
        kt([(2, 0), (3, 0)], (1,))
        kt([(i, 1) for i in range(4)], (1,), hooks={S['h2']: get(
            Ab, lambda: [j for ph in range(4) for j in
                         wj(0, qb, (ph,)) + xj(0, G(0), qb, (ph,))], S['r3'])})
        params()
        kt([(0, 0)], qb)
        arrive(Bb)
        jit(xj(0, G(1), qb, by_phase=True), S['n4'], S['r7'])
        background(wj(1, qb, by_phase=True), S['r7'])
        kt([(1, 0)], qb)
        kt([(0, 1), (1, 1)], qb, hooks={S['h3']: get(
            Cb, lambda: xj(0, G(2), qb, by_phase=True) + xj(0, G(3), qb), S['r6'])})
        kt([(2, 0)], qb)
        kt([(3, 0)], qb)
        kt([(2, 1)], qb)
        kt([(3, 1)], qb, hooks={S['h4']: get(
            w23, lambda: wj(2, allq, by_phase=True), S['r4'])})
        q2 = allq
    if S['trunc']:
        kt([(0, 2), (1, 2)], q2)
        drain()
        arrive(x1)
        wait(o_copies)
        for n in range(24 if S['trunc'] == 2 else 0):
            for u in range(32):
                acc[3, 0, 1, 8:72, :] = jnp.dot(
                    lhs(u % 6, u % 7, 0, (0, 1), allq), rhs(1, u % 7, 0, allq),
                    preferred_element_type=_F32) + acc[3, 0, 1, 8:72, :]
            fetch_in((('Z',),))
            arrive((('Z',),))
        return
    kt([(i, 2) for i in range(4)], q2, hooks={4: lambda: background(
        wj(3, allq, by_phase=True), S['r4'])})
    kt([(i, 3) for i in range(4)], allq, hooks={S['h5']: get(
        x1, lambda: xj(1, G(0), allq), S['r4'])})

    col1 = [Col(1, cp, 480) for cp in range(ncp)]
    for i in range(4):
        if i < 3:
            background(xj(1, G(i + 1), allq), S['r5'], 4 * 2688 - 512)
        for cp in range(ncp):
            assert col0[cp].finished()
            if (i, cp) == (3, ncp - 1):
                col1[cp].out_rows = S['lastrows']
                bg.update(rate=S['rlast'], rep=S['rlast'])
            tiles([(col1[cp], i)], allq, two_phase=True,
                  split=S['split'] and (i, cp) == (3, ncp - 1))
    bg['tok'] = None
    drain()
    wait(o_copies)


@jax.jit
def pallas_standalone__batchnorm__prompt_kernel(
    x: jax.Array,
    w: jax.Array,
    mean: jax.Array,
    var: jax.Array,
    g: jax.Array,
    b: jax.Array,
):
    nb, seq, ch = x.shape
    T = seq // 4
    nct = ch // _L

    def kernel(*refs):
        _kernel(*refs, nb=nb, seq=seq, ch=ch)

    any_spec = pl.BlockSpec(memory_space=pl.ANY)
    return pl.pallas_call(
        kernel,
        out_shape=jax.ShapeDtypeStruct(x.shape, x.dtype),
        in_specs=[any_spec] * 6,
        out_specs=any_spec,
        scratch_shapes=[
            pltpu.VMEM((nb, nct, seq, _L), _BF16),
            pltpu.VMEM((nct, 3, ch, _L), _BF16),
            pltpu.VMEM((ch,), _BF16),
            pltpu.VMEM((ch,), _BF16),
            pltpu.VMEM((ch,), _BF16),
            pltpu.VMEM((ch,), _BF16),
            pltpu.VMEM((4 * nb, 6, 7, 32, ch // 2), _U32),
            pltpu.VMEM((nct // 2, 6, 7, ch // 4, _L), _U32),
            pltpu.VMEM((nct // 2, 2, 6, T + 2 * _HALO, _L), _F32),
            pltpu.VMEM((nb * nct, seq // 2, _L), _U32),
            pltpu.VMEM((3, nct, 8, _L), _F32),
            pltpu.VMEM((8, _L), _U32),
            pltpu.VMEM((8, _L), _U32),
            pltpu.SemaphoreType.DMA((10,)),
            pltpu.SemaphoreType.DMA((1,)),
        ],
        compiler_params=pltpu.CompilerParams(vmem_limit_bytes=110 * 1024 * 1024),
    )(x, w, mean, var, g, b)
```

```python
import jax
import jax.numpy as jnp
import jax.experimental.pallas as pl
import jax.experimental.pallas.tpu as pltpu

_A = 1.5
_B = 1.0 / _A
_A2 = _A * _A
_B2 = _B * _B
_C = _A2 + _B2
_LA = 1.0 / (2.0 * _A2 * (_A2 - _B2))
_LB = 1.0 / (2.0 * _B2 * (_A2 - _B2))
_GAM = 1.35
_EPS = 1e-5
_L = 128
_HALO = 8
_RG = 64
_POINTS = (0, 5, 1, 2, 3, 4)

_F32 = jnp.float32
_BF16 = jnp.bfloat16
_U32 = jnp.uint32

CFG = dict(r1=3.5, r2=3.3,
           r3=2.8, r4=2.0,
           r5=1.8, r6=2.5,
           n1=8, n2=8,
           n3=8, h1=1,
           h2=0, h3=0,
           h4=1, h5=3,
           rep=1.8, r7=2.8, n4=16,
           ehead=350, ramp=5,
           h0=3, hb=0, hc=0, ra=2.3,
           fp=1, bp=2, lastrows=128, split=1, rlast=2.8, gmask=1, trunc=0)


def _kernel(x_hbm, w_hbm, mean_hbm, var_hbm, g_hbm, b_hbm, o_hbm,
            xb, wr, pb0, pb1, pb2, pb3, xs, ws, acc, ob, scsh, zsrc, zer,
            sem_i, sem_o, *, nb, seq, ch):
    assert nb == 2 and seq == 32 * _RG and ch == 8 * _L
    pbuf = (pb0, pb1, pb2, pb3)
    T = seq // 4
    nct = ch // _L
    ncp = nct // 2
    nq = nct // 2
    nblk = T // 8
    S = CFG

    free_sems = list(range(sem_i.shape[0]))
    inflight = {}

    def copies(name, sem):
        kind = name[0]
        if kind == 'X':
            _, b, r0, nr, qs = name
            return [pltpu.make_async_copy(
                x_hbm.at[b, pl.ds(r0, nr), pl.ds(ct * _L, _L)],
                xb.at[b, ct, pl.ds(r0, nr), :], sem)
                for ct in range(2 * qs[0], 2 * qs[-1] + 2)]
        if kind == 'W':
            _, cp, qs = name
            k0, nk = 2 * _L * qs[0], 2 * _L * len(qs)
            return [pltpu.make_async_copy(
                w_hbm.at[k, pl.ds(k0, nk), pl.ds(j * _L, _L)],
                wr.at[j, k, pl.ds(k0, nk), :], sem)
                for k in (2, 0, 1) for j in (2 * cp, 2 * cp + 1)]
        if kind == 'P':
            return [pltpu.make_async_copy(src, pbuf[i], sem) for i, src in
                    enumerate((mean_hbm, var_hbm, g_hbm, b_hbm))]
        return [pltpu.make_async_copy(zsrc, d, sem) for d in (
            zer, xs.at[4 * nb - 1, 5, 6, pl.ds(0, 8), pl.ds(0, _L)],
            ws.at[ncp - 1, 4, 6, pl.ds(0, 8), :])]

    def fetch_in(*groups):
        for names in groups:
            k = free_sems.pop(0)
            cs = [c for n in names for c in copies(n, sem_i.at[k])]
            inflight[names] = (k, cs)
            for c in cs:
                c.start()

    def arrive(*groups):
        for names in groups:
            k, cs = inflight.pop(names)
            wait(cs)
            free_sems.append(k)

    def wait(cs):
        bg['tok'] = None
        for c in cs:
            c.wait()

    o_copies = []

    def out_copy(b, j, r0, nr):
        return pltpu.make_async_copy(
            ob.at[b * nct + j, pl.ds(r0 // 2, nr // 2), :].bitcast(_BF16),
            o_hbm.at[b, pl.ds(r0, nr), pl.ds(j * _L, _L)], sem_o.at[0])

    def start_out(b, cp, r0, nr):
        for c in range(2):
            o_copies.append(out_copy(b, 2 * cp + c, r0, nr))
            o_copies[-1].start()

    keep = {}

    def tie(v, tok):
        if tok is None:
            return v
        if len(tok) == 2:
            tok.append({jnp.dtype(_F32): tok[0][tok[1]:tok[1] + 8]})
        if v.dtype not in tok[2]:
            tok[2][v.dtype] = pltpu.bitcast(tok[2][jnp.dtype(_F32)], v.dtype)
        t = tok[2][v.dtype]
        n = v.shape[0]
        if S['gmask'] == 0 or n not in keep:
            keep[n] = cat([zer[...]] * (n // 8)) == 0
        return jax.lax.select(keep[n], v, cat([t] * (n // 8)))

    sh16 = jnp.full((8, _L), 16, _U32)
    mk16 = jnp.full((8, _L), 0xFFFF0000, _U32)

    def unpackers(tok):
        sh, mk = cat([tie(sh16, tok)] * 2), cat([tie(mk16, tok)] * 2)
        return (lambda u: pltpu.bitcast(u << sh, _F32),
                lambda u: pltpu.bitcast(u & mk, _F32))

    def pack(lo, hi):
        return pltpu.pack_elementwise([lo, hi], packed_dtype=_BF16)

    def cat(vs, axis=0):
        return vs[0] if len(vs) == 1 else jnp.concatenate(vs, axis=axis)

    have = set()

    def x_job(b, g, q, h, phases):
        def words(half, ct, o):
            t = g * _RG + 32 * half + 16 * h
            xu = xb.at[b, ct, pl.ds(4 * t, 64), :].bitcast(_U32)
            return cat([xu[pl.ds(2 * par + o, 8, stride=4), :] for par in range(2)])

        blocks = [(half, ct) for half in range(2) for ct in (2 * q, 2 * q + 1)]
        for phase in phases:
            if phase < 2:
                lo, hi = unpackers((yield 27))
                if phase == 0:
                    outs = {0: [lo(words(*bl, 0)) for bl in blocks]}
                else:
                    outs = {5: [hi(words(*bl, 1)) for bl in blocks]}
            else:
                c = _A if phase == 2 else _B
                p = 2 * phase - 3
                outs = {p: [], p + 1: []}
                for bl in blocks:
                    lo, hi = unpackers((yield 42 if bl == blocks[-1] else 25))
                    we, wo = words(*bl, 0), words(*bl, 1)
                    e = lo(we) + (c * c) * lo(wo)
                    o = c * hi(we) + (c * c * c) * hi(wo)
                    outs[p].append(e + o)
                    outs[p + 1].append(e - o)
            for p, (a11, a12, a21, a22) in outs.items():
                if phase >= 2 and p % 2 == 0:
                    tok = yield 22
                    a11, a22 = tie(a11, tok), tie(a22, tok)
                ss = (a11 - a22, a21 - a22, a11, a22, a11 - a12, a21 - a11,
                      a12 - a22)
                for i, s in enumerate(ss):
                    r = 16 * (g % 2) + 8 * h
                    xs[4 * b + g // 2, p, i, r:r + 8, q * _L:(q + 1) * _L] = pack(
                        s[0:8], s[8:16])
                have.add(('x', p, b, g, q, h))

    def w_job(cp, q, kk, phases):
        def vals(tap, j, lo, hi):
            u = cat([wr.at[j, tap, pl.ds(ct * _L + 16 * kk, 16), :].bitcast(_U32)[...]
                     for ct in (2 * q, 2 * q + 1)])
            return cat([lo(u), hi(u)])

        j1, j2 = 2 * cp, 2 * cp + 1
        gh = 0.5 * _GAM
        for phase in phases:
            if phase < 2:
                lo, hi = unpackers((yield 34))
                tap = 2 if phase == 0 else 0
                p = 0 if phase == 0 else 5
                outs = {p: (gh * vals(tap, j1, lo, hi), vals(tap, j2, lo, hi))}
            else:
                c, lam = (_A, _LA) if phase == 2 else (_B, _LB)
                p = 2 * phase - 3
                uv = []
                for j, s in ((j1, gh * lam), (j2, lam)):
                    lo, hi = unpackers((yield 39))
                    e = s * vals(2, j, lo, hi) + (s * c * c) * vals(0, j, lo, hi)
                    o = (s * c) * vals(1, j, lo, hi)
                    uv.append((e + o, e - o))
                outs = {p: (uv[0][0], uv[1][0]), p + 1: (uv[0][1], uv[1][1])}
            for p, (u, v) in outs.items():
                half = jnp.full((8, _L), 0.5, _F32)
                if phase >= 2:
                    half = tie(half, (yield 23))
                half = cat([half] * 2)
                sel = lambda a, n: cat(
                    [a[8 * n:8 * n + 8], a[16 + 8 * n:24 + 8 * n]])
                u1, u2, v1, v2 = sel(u, 0), sel(u, 1), sel(v, 0), sel(v, 1)
                t2 = half * v1 + u1
                t5 = half * v2 - u2
                t1 = t2 - t5
                ts = [t1, t2, v1 - t1, v2 + t1, t5]
                if phase >= 2:
                    ts += [v1, v2]
                for i, t in enumerate(ts):
                    r = 64 * q + 8 * kk
                    ws[cp, p, i, r:r + 8, :] = pack(t[0:8], t[8:16])
                have.add(('w', p, cp, q, kk))

    def lhs(p, i, b, gs, qs):
        return pltpu.bitcast(
            xs[4 * b + gs[0] // 2, p, i, 16 * (gs[0] % 2):16 * (gs[-1] % 2 + 1),
               qs[0] * _L:(qs[-1] + 1) * _L], _BF16)

    def rhs(p, i, cp, qs):
        if p in (0, 5) and i >= 5:
            r = cat([wr.at[2 * cp + 1, 2 if p == 0 else 0,
                           pl.ds((2 * q + i - 5) * _L, _L), :].bitcast(_U32)[...]
                     for q in qs])
        else:
            r = ws[cp, p, i, 64 * qs[0]:64 * (qs[-1] + 1), :]
        return pltpu.bitcast(r, _BF16)

    def ep_job(acc, b, cp, blk, out=None):
        q = _HALO + 8 * blk
        ys = []
        for c in range(2):
            def ld(p, o=0, c=c):
                return acc[c, p, q + o:q + o + 8, :]

            m, mb = tie(ld(4), (yield 24)), ld(3)
            db = mb - m
            sb = mb + m
            ma, mna, z0, z5 = ld(1), ld(2), ld(0), ld(5)
            y0 = (_B * (((_A / _B) * db - ma) + mna) + z5) + ld(5, -1)
            t2 = (_A / _C) * ((ma - (_B / _A) * db) - mna) - z5
            z4 = ((ma - sb) + mna) + z0
            y3 = z4 + ld(0, 1)
            y1 = _A2 * (sb - z0) - _B2 * (z4 + sb)
            ys.append((y0, y1, t2, y3))
        for c in range(2):
            j = 2 * cp + c
            tok = yield 25
            sc, scc, sh = tie(scsh[0, j], tok), tie(scsh[1, j], tok), scsh[2, j]
            os_ = []
            for k in range(4):
                y = ys[0][k] - ys[1][k] if c == 0 else ys[0][k] + ys[1][k]
                h = y * (scc if k == 2 else sc) + sh
                os_.append(h * jnp.tanh(h) + h)
            o_ = ob.at[b * nct + j]
            o_[pl.ds(16 * blk, 8, stride=2), :] = pack(os_[0], os_[1])
            o_[pl.ds(16 * blk + 1, 8, stride=2), :] = pack(os_[2], os_[3])
        if out:
            start_out(b, cp, *out)

    epq = []
    bg = dict(jobs=[], every=0, rate=2.0, budget=0.0, since=0, active=None,
              cost=0, tok=None, late=0, rep=S['rep'])

    def fetch(force=False):
        if bg['active'] is None:
            if bg['jobs'] and (force or bg['since'] >= bg['every']):
                bg['since'] = min(bg['since'] - bg['every'], 4 * bg['every'])
                bg['active'] = bg['jobs'].pop(0)
                bg['cap'] = 4.0
            elif epq:
                bg['active'] = epq.pop(0)
                bg['cap'] = bg['rep']
            else:
                return False
            bg['cost'] = next(bg['active'])
        return True

    def advance(tok, force=False):
        if fetch(force):
            try:
                bg['cost'] = bg['active'].send(tok)
            except StopIteration:
                bg['active'] = None

    def clock(tok, cycles):
        bg['since'] += cycles
        bg['tok'] = tok
        if not fetch():
            bg['budget'] = 0.0
            return
        bg['budget'] += min(bg['rate'], bg['cap']) * cycles
        if bg['budget'] >= bg['cost']:
            bg['budget'] = min(bg['budget'] - bg['cost'], 16.0)
            advance(tok)

    def burst(ops):
        while ops > 0 and fetch():
            ops -= bg['cost']
            advance(None)

    def require(keys):
        while not all(k in have for k in keys):
            assert bg['active'] is not None or bg['jobs'], keys
            bg['late'] += 1
            advance(bg['tok'], force=True)

    def drain():
        bg['every'] = 0
        while bg['active'] is not None or epq or bg['jobs']:
            bg['late'] += 1
            advance(bg['tok'])

    def background(jobs, rate, span=0):
        bg['jobs'] += jobs
        every = span // max(len(bg['jobs']), 1)
        bg.update(every=every, rate=rate, since=every)

    def run_now(jobs):
        for j in jobs:
            for _ in j:
                pass

    def jit(jobs, n_eager, rate):
        run_now(jobs[:n_eager])
        background(jobs[n_eager:], rate)

    def xj(b, gs, qs, phases=(0, 1, 2, 3), by_phase=False):
        if by_phase:
            return [j for ph in phases for j in xj(b, gs, qs, (ph,))]
        return [x_job(b, g, q, h, phases) for g in gs for q in qs for h in range(2)]

    def wj(cp, qs, phases=(0, 1, 2, 3), by_phase=False):
        if by_phase:
            return [j for ph in phases for j in wj(cp, qs, (ph,))]
        return [w_job(cp, q, kk, phases) for q in qs for kk in range(8)]

    class Col:
        def __init__(self, b, cp, out_rows):
            self.b, self.cp, self.out_rows = b, cp, out_rows
            self.acc = acc.at[cp]
            self.todo = list(range(nblk))
            self.sent = 0
            self.jobs = []
            self.full = {p: set() for p in range(6)}
            self.kdone = {}

        def flush(self):
            f = self.full
            ready = [r for r in self.todo
                     if all(r in f[p] for p in range(6))
                     and (r + 1 == nblk or r + 1 in f[0])
                     and (r == 0 or r - 1 in f[5])]
            for r in ready:
                self.todo.remove(r)
                e = min(self.todo, default=nblk)
                out = None
                if e == nblk or 32 * (e - self.sent) >= self.out_rows:
                    out = (32 * self.sent, 32 * (e - self.sent))
                    self.sent = e
                self.jobs.append(ep_job(self.acc, self.b, self.cp, r, out))
                epq.append(self.jobs[-1])

        def finished(self):
            return not self.todo and not any(
                j in epq or j is bg['active'] for j in self.jobs)

    def tiles(subs, qs, two_phase=False, hooks=None, split=False):
        hooks = hooks or {}
        subs = [(c, (2 * i, 2 * i + 1)) for c, i in subs]
        fl = {(i not in c.kdone, c.kdone.get(i, 0) + len(qs) == nq) for c, i in subs}
        assert len(fl) == 1
        first, last = fl.pop()
        for c, i in subs:
            c.kdone[i] = c.kdone.get(i, 0) + len(qs)
        held = []

        def release():
            for k in range(0, held[0].shape[0], 8):
                for r in held:
                    clock([r, k], 2 * len(qs))
            held.clear()

        def prod(t, p, i):
            col, gs = t
            require([('x', p, col.b, g, q, h)
                     for g in gs for q in qs for h in range(2)]
                    + [('w', p, col.cp, q, kk) for q in qs for kk in range(8)])
            r = jnp.dot(lhs(p, i, col.b, gs, qs), rhs(p, i, col.cp, qs),
                        preferred_element_type=_F32)
            held.append(r)
            if len(held) * len(qs) >= 4:
                release()
            return r

        def put(t, p, half, c, v, init, final):
            col = t[0]
            for n, g in enumerate(t[1]):
                q = _HALO + g * _RG + 32 * half
                part = v[32 * n:32 * n + 32]
                if not init:
                    part = part + col.acc[c, p, q:q + 32, :]
                col.acc[c, p, q:q + 32, :] = part
                if final and last and c == 1:
                    col.full[p].update(range(8 * g + 4 * half, 8 * g + 4 * half + 4))

        def upper(t, p):
            p1 = prod(t, p, 0)
            c11 = p1 + prod(t, p, 6)
            p4 = prod(t, p, 3)
            c11 = c11 + p4
            p3 = prod(t, p, 2)
            c22 = p1 + p3
            p5 = prod(t, p, 4)
            put(t, p, 0, 0, c11 + p5, first, True)
            put(t, p, 0, 1, p3 - p5, first, True)
            if not two_phase:
                return p4, c22
            put(t, p, 1, 0, p4, first, False)
            put(t, p, 1, 1, c22, first, False)

        def lower(t, p, part=None):
            p6 = prod(t, p, 5)
            if part:
                p6 = p6 + part[1]
            p2 = prod(t, p, 1)
            put(t, p, 1, 0, p2 + part[0] if part else p2, first and part, True)
            put(t, p, 1, 1, p6 - p2, first and part, True)

        def flush():
            if held:
                release()
            for c, _ in subs:
                c.flush()

        if two_phase:
            for p in _POINTS:
                for t in subs:
                    upper(t, p)
            for part in ([[(c, (g,))] for c, gs in subs for g in gs]
                         if split else [subs]):
                flush()
                for p in _POINTS:
                    for t in part:
                        lower(t, p)
        else:
            for n, p in enumerate(_POINTS):
                if n in hooks:
                    flush()
                    hooks[n]()
                for t in subs:
                    lower(t, p, upper(t, p))
        flush()

    XR = 8 * _RG
    allq = tuple(range(nq))
    G = lambda i: (2 * i, 2 * i + 1)
    X = lambda i, *qs: ('X', 0, i * XR, XR, qs)
    W = lambda cp, *qs: ('W', cp, qs)

    col0 = [Col(0, cp, seq) for cp in range(ncp)]

    def params():
        mean, var, gam, bet = (
            pbuf[i][...].astype(_F32).reshape(1, ch) for i in range(4))
        s = gam * jax.lax.rsqrt(var + _EPS)
        col = jax.lax.broadcasted_iota(jnp.int32, (1, ch), 1)
        sm = jnp.where((col & _L) == 0, s * (1.0 / _GAM), s)
        for k, v in enumerate((0.5 * sm, (0.5 * _C) * sm, 0.5 * (bet - mean * s))):
            for j in range(nct):
                scsh[k, j] = jnp.broadcast_to(v[:, j * _L:(j + 1) * _L], (8, _L))

    def kt(subs, qs, hooks=None):
        tiles([(col0[cp], i) for i, cp in subs], qs, hooks=hooks)

    def get(group, jobs, rate, fetch=()):
        def f():
            fetch_in(*fetch)
            arrive(group)
            background(jobs(), rate)
            burst(S['ehead'])
        return f

    qb = allq[2:]
    if S['ramp'] >= 2:
        qr = allq[1:]
        q0 = [(X(0, 0),), (X(1, 0), X(2, 0)), (X(3, 0), W(1, 0)), (W(2, 0),)]
        if S['ramp'] == 3:
            q0 = [(X(0, 0),), (X(1, 0),), (X(2, 0), X(3, 0)), (W(1, 0), W(2, 0))]
        if S['ramp'] == 4:
            q0 = [(X(0, 0),), (X(1, 0),), (X(2, 0), X(3, 0)), (W(1, 0),), (W(2, 0),)]
        if S['ramp'] == 5:
            q0 = [(X(0, 0),), (X(1, 0),), (X(2, 0),), (X(3, 0),), (W(1, 0),), (W(2, 0),)]
        if S['ramp'] == 6:
            q0 = [(X(0, 0),), (X(1, 0),), (X(2, 0),), (X(3, 0), W(1, 0)), (W(2, 0),)]
        A1, B1 = (W(0, 1), X(0, 1), X(1, 1)), (X(2, 1), X(3, 1), W(1, 1))
        Ab, Bb = (W(0, *qb), X(0, *qb), ('P',)), (X(1, *qb), W(1, *qb))
        Cb = (X(2, *qb), X(3, *qb))
        w23, x1 = (W(2, *qr), W(3, *allq)), (('X', 1, 0, seq, allq),)
        zsrc[...] = jnp.zeros((8, _L), _U32)
        fetch_in((W(0, 0), ('Z',)), *q0, A1, B1)
        zero = jnp.zeros((_HALO, _L), _F32)
        for cp in range(ncp):
            for c in range(2):
                acc[cp, c, 0, _HALO + T:2 * _HALO + T, :] = zero
                acc[cp, c, 5, 0:_HALO, :] = zero
        arrive((W(0, 0), ('Z',)))
        run_now(wj(0, (0,)))
        arrive(q0[0])
        jit(xj(0, G(0), (0,), by_phase=True), S['n1'], S['r1'])
        kt([(0, 0)], (0,))
        if S['ramp'] == 2:
            fetch_in(Ab)
            arrive(q0[1])
            jit(xj(0, G(1) + G(2), (0,), by_phase=True), S['n3'], S['r2'])
            kt([(1, 0), (2, 0)], (0,))
            arrive(q0[2])
            jit(xj(0, G(3), (0,), by_phase=True), S['n1'], S['r1'])
            background(wj(1, (0,), by_phase=True), S['r1'])
            kt([(3, 0)], (0,))
            background([], S['r2'])
            kt([(i, 1) for i in range(4)], (0,), hooks={S['h0']: get(
                q0[3], lambda: wj(2, (0,), by_phase=True), S['ra'], (Bb, Cb))})
        else:
            arrive(q0[1])
            jit(xj(0, G(1), (0,), by_phase=True), S['n1'], S['r1'])
            kt([(1, 0)], (0,))
            fetch_in(Ab)
            arrive(q0[2])
            if S['ramp'] >= 5:
                jit(xj(0, G(2), (0,), by_phase=True), S['n1'], S['r1'])
                kt([(2, 0)], (0,))
                arrive(q0.pop(3))
                jit(xj(0, G(3), (0,), by_phase=True), S['n1'], S['r1'])
                if S['ramp'] == 6:
                    background(wj(1, (0,), by_phase=True), S['r1'])
                kt([(3, 0)], (0,))
            else:
                jit(xj(0, G(2) + G(3), (0,), by_phase=True), S['n3'], S['r2'])
                kt([(2, 0), (3, 0)], (0,))
            if S['ramp'] == 6:
                background([], S['r2'])
                kt([(i, 1) for i in range(4)], (0,), hooks={S['h0']: get(
                    q0[3], lambda: wj(2, (0,), by_phase=True), S['ra'], (Bb, Cb))})
            elif S['ramp'] == 3:
                fetch_in(Bb, Cb)
                arrive(q0[3])
                jit(wj(1, (0,), by_phase=True), S['n2'], S['r2'])
                background(wj(2, (0,), by_phase=True), S['ra'])
                kt([(i, 1) for i in range(4)], (0,))
            else:
                arrive(q0[3])
                jit(wj(1, (0,), by_phase=True), S['n2'], S['r2'])
                kt([(i, 1) for i in range(4)], (0,), hooks={S['h0']: get(
                    q0[4], lambda: wj(2, (0,), by_phase=True), S['ra'], (Bb, Cb))})
        kt([(i, 2) for i in range(4)], (0,), hooks={S['h1']: get(
            A1, lambda: wj(0, (1,), by_phase=True)
            + xj(0, G(0) + G(1), (1,), by_phase=S['bp'] & 1), S['ra'])})

        kt([(0, 0), (1, 0)], (1,), hooks={S['hb']: get(
            B1, lambda: xj(0, G(2) + G(3), (1,), by_phase=S['bp'] & 2)
            + wj(1, (1,), by_phase=True), S['ra'], (w23, x1))})
        kt([(2, 0), (3, 0)], (1,))
        kt([(i, 1) for i in range(4)], (1,), hooks={S['h2']: get(
            Ab, lambda: [j for ph in range(4) for j in
                         wj(0, qb, (ph,)) + xj(0, G(0), qb, (ph,))]
            if S['bp'] & 4 else xj(0, G(0), qb) + wj(0, qb, by_phase=True),
            S['r3'])})
        params()
        kt([(0, 0)], qb, hooks={S['hc']: get(
            Bb, lambda: xj(0, G(1), qb, by_phase=S['bp'] & 8)
            + wj(1, qb, by_phase=True), S['r7'])})
        kt([(1, 0)], qb)
        kt([(0, 1), (1, 1)], qb, hooks={S['h3']: get(
            Cb, lambda: xj(0, G(2), qb, by_phase=S['bp'] & 16) + xj(0, G(3), qb),
            S['r6'])})
        kt([(2, 0)], qb)
        kt([(3, 0)], qb)
        kt([(2, 1)], qb, hooks={S['h4']: get(
            w23, lambda: wj(2, qr, by_phase=True), S['r4'])})
        kt([(3, 1)], qb)
        q2 = qr
    else:
        q0 = {0: [(X(0, 0),), (X(1, 0),), (X(2, 0), X(3, 0)), (W(1, 0),)],
              1: [(X(0, 0),), (X(1, 0), X(2, 0)), (X(3, 0), W(1, 0))]}[S['ramp']]
        A1, B1 = (W(0, 1), X(0, 1), X(1, 1)), (X(2, 1), X(3, 1), W(1, 1))
        Ab, Bb = (W(0, *qb), X(0, *qb), ('P',)), (X(1, *qb), W(1, *qb))
        Cb = (X(2, *qb), X(3, *qb))
        w23, x1 = (W(2, *allq), W(3, *allq)), (('X', 1, 0, seq, allq),)
        fetch_in((W(0, 0),))
        zsrc[...] = jnp.zeros((8, _L), _U32)
        fetch_in((('Z',),), *q0, A1, B1, Ab)
        zero = jnp.zeros((_HALO, _L), _F32)
        for cp in range(ncp):
            for c in range(2):
                acc[cp, c, 0, _HALO + T:2 * _HALO + T, :] = zero
                acc[cp, c, 5, 0:_HALO, :] = zero

        hook_a1 = {S['h1']: get(
            A1, lambda: wj(0, (1,), by_phase=True)
            + xj(0, G(0) + G(1), (1,), by_phase=True), S['r3'])}
        arrive((W(0, 0),), (('Z',),))
        run_now(wj(0, (0,)))
        arrive(q0[0])
        jit(xj(0, G(0), (0,), by_phase=True), S['n1'], S['r1'])
        kt([(0, 0)], (0,))
        arrive(q0[1])
        if S['ramp'] == 0:
            jit(xj(0, G(1), (0,), by_phase=True), S['n1'], S['r1'])
            kt([(1, 0)], (0,))
            arrive(q0[2])
            fetch_in(Bb, Cb)
            jit(xj(0, G(2) + G(3), (0,), by_phase=True), S['n3'], S['r2'])
            kt([(2, 0), (3, 0)], (0,))
            arrive(q0[3])
            jit(wj(1, (0,), by_phase=True), S['n2'], S['r2'])
        else:
            jit(xj(0, G(1) + G(2), (0,), by_phase=True), S['n3'], S['r2'])
            kt([(1, 0), (2, 0)], (0,))
            arrive(q0[2])
            fetch_in(Bb, Cb)
            jit(xj(0, G(3), (0,), by_phase=True), S['n1'], S['r1'])
            background(wj(1, (0,), by_phase=True), S['r1'])
            kt([(3, 0)], (0,))
            background([], S['r2'])
        kt([(i, 1) for i in range(4)], (0,), hooks=hook_a1)
        kt([(0, 0), (1, 0)], (1,))
        arrive(B1)
        fetch_in(w23, x1)
        jit(xj(0, G(2) + G(3), (1,), by_phase=True), S['n3'], S['r2'])
        background(wj(1, (1,), by_phase=True), S['r2'])
        kt([(2, 0), (3, 0)], (1,))
        kt([(i, 1) for i in range(4)], (1,), hooks={S['h2']: get(
            Ab, lambda: [j for ph in range(4) for j in
                         wj(0, qb, (ph,)) + xj(0, G(0), qb, (ph,))], S['r3'])})
        params()
        kt([(0, 0)], qb)
        arrive(Bb)
        jit(xj(0, G(1), qb, by_phase=True), S['n4'], S['r7'])
        background(wj(1, qb, by_phase=True), S['r7'])
        kt([(1, 0)], qb)
        kt([(0, 1), (1, 1)], qb, hooks={S['h3']: get(
            Cb, lambda: xj(0, G(2), qb, by_phase=True) + xj(0, G(3), qb), S['r6'])})
        kt([(2, 0)], qb)
        kt([(3, 0)], qb)
        kt([(2, 1)], qb)
        kt([(3, 1)], qb, hooks={S['h4']: get(
            w23, lambda: wj(2, allq, by_phase=True), S['r4'])})
        q2 = allq
    if S['trunc']:
        kt([(0, 2), (1, 2)], q2)
        drain()
        arrive(x1)
        wait(o_copies)
        for n in range(24 if S['trunc'] == 2 else 0):
            for u in range(32):
                acc[3, 0, 1, 8:72, :] = jnp.dot(
                    lhs(u % 6, u % 7, 0, (0, 1), allq), rhs(1, u % 7, 0, allq),
                    preferred_element_type=_F32) + acc[3, 0, 1, 8:72, :]
            fetch_in((('Z',),))
            arrive((('Z',),))
        return
    kt([(i, 2) for i in range(4)], q2, hooks={4: lambda: background(
        wj(3, allq, by_phase=True), S['r4'])})
    kt([(i, 3) for i in range(4)], allq, hooks={S['h5']: get(
        x1, lambda: xj(1, G(0), allq), S['r4'])})

    col1 = [Col(1, cp, 480) for cp in range(ncp)]
    for i in range(4):
        if i < 3:
            background(xj(1, G(i + 1), allq), S['r5'], 4 * 2688 - 512)
        for cp in range(ncp):
            assert col0[cp].finished()
            if (i, cp) == (3, ncp - 1):
                col1[cp].out_rows = S['lastrows']
                bg.update(rate=S['rlast'], rep=S['rlast'])
            tiles([(col1[cp], i)], allq, two_phase=True,
                  split=S['split'] and (i, cp) == (3, ncp - 1))
    bg['tok'] = None
    drain()
    wait(o_copies)


@jax.jit
def pallas_standalone__batchnorm__prompt_kernel(
    x: jax.Array,
    w: jax.Array,
    mean: jax.Array,
    var: jax.Array,
    g: jax.Array,
    b: jax.Array,
):
    nb, seq, ch = x.shape
    T = seq // 4
    nct = ch // _L

    def kernel(*refs):
        _kernel(*refs, nb=nb, seq=seq, ch=ch)

    any_spec = pl.BlockSpec(memory_space=pl.ANY)
    return pl.pallas_call(
        kernel,
        out_shape=jax.ShapeDtypeStruct(x.shape, x.dtype),
        in_specs=[any_spec] * 6,
        out_specs=any_spec,
        scratch_shapes=[
            pltpu.VMEM((nb, nct, seq, _L), _BF16),
            pltpu.VMEM((nct, 3, ch, _L), _BF16),
            pltpu.VMEM((ch,), _BF16),
            pltpu.VMEM((ch,), _BF16),
            pltpu.VMEM((ch,), _BF16),
            pltpu.VMEM((ch,), _BF16),
            pltpu.VMEM((4 * nb, 6, 7, 32, ch // 2), _U32),
            pltpu.VMEM((nct // 2, 6, 7, ch // 4, _L), _U32),
            pltpu.VMEM((nct // 2, 2, 6, T + 2 * _HALO, _L), _F32),
            pltpu.VMEM((nb * nct, seq // 2, _L), _U32),
            pltpu.VMEM((3, nct, 8, _L), _F32),
            pltpu.VMEM((8, _L), _U32),
            pltpu.VMEM((8, _L), _U32),
            pltpu.SemaphoreType.DMA((10,)),
            pltpu.SemaphoreType.DMA((1,)),
        ],
        compiler_params=pltpu.CompilerParams(vmem_limit_bytes=110 * 1024 * 1024),
    )(x, w, mean, var, g, b)
```

```python
import jax
import jax.numpy as jnp
import jax.experimental.pallas as pl
import jax.experimental.pallas.tpu as pltpu

_A = 1.5
_B = 1.0 / _A
_A2 = _A * _A
_B2 = _B * _B
_C = _A2 + _B2
_LA = 1.0 / (2.0 * _A2 * (_A2 - _B2))
_LB = 1.0 / (2.0 * _B2 * (_A2 - _B2))
_GAM = 1.35
_EPS = 1e-5
_L = 128
_HALO = 8
_RG = 64
_POINTS = (0, 5, 1, 2, 3, 4)

_F32 = jnp.float32
_BF16 = jnp.bfloat16
_U32 = jnp.uint32

_TUNE = dict(
    r1=3.5, r2=3.3, ra=2.3, rb=2.6, r3=2.5, r7=2.2, r4=2.0, r8=1.8,
    r5=1.8, rep=1.8, rlast=2.8, n1=8, n2=8,
    h0=4, h1=2, h2=0, hc=2, h4=2, h5=3, h6=3,
    ehead=300, dem=128, lastrows=128)


def _kernel(x_hbm, w_hbm, mean_hbm, var_hbm, g_hbm, b_hbm, o_hbm,
            xb, wr, pb0, pb1, pb2, pb3, xs, ws, acc, ob, scsh, zsrc, zer,
            sem_i, sem_o, *, nb, seq, ch):
    assert nb == 2 and seq == 32 * _RG and ch == 8 * _L
    pbuf = (pb0, pb1, pb2, pb3)
    T = seq // 4
    nct = ch // _L
    ncp = nct // 2
    nq = nct // 2
    nblk = T // 8
    S = _TUNE

    free_sems = list(range(sem_i.shape[0]))
    inflight = {}

    def copies(name, sem):
        kind = name[0]
        if kind == 'X':
            _, b, r0, nr, qs = name
            return [pltpu.make_async_copy(
                x_hbm.at[b, pl.ds(r0, nr), pl.ds(ct * _L, _L)],
                xb.at[b, ct, pl.ds(r0, nr), :], sem)
                for ct in range(2 * qs[0], 2 * qs[-1] + 2)]
        if kind == 'W':
            _, cp, qs = name
            k0, nk = 2 * _L * qs[0], 2 * _L * len(qs)
            return [pltpu.make_async_copy(
                w_hbm.at[k, pl.ds(k0, nk), pl.ds(j * _L, _L)],
                wr.at[j, k, pl.ds(k0, nk), :], sem)
                for k in (2, 0, 1) for j in (2 * cp, 2 * cp + 1)]
        if kind == 'P':
            return [pltpu.make_async_copy(src, pbuf[i], sem) for i, src in
                    enumerate((mean_hbm, var_hbm, g_hbm, b_hbm))]
        return [pltpu.make_async_copy(zsrc, d, sem) for d in (
            zer, xs.at[4 * nb - 1, 5, 6, pl.ds(0, 8), pl.ds(0, _L)],
            ws.at[ncp - 1, 4, 6, pl.ds(0, 8), :])]

    def fetch_in(*groups):
        for names in groups:
            k = free_sems.pop(0)
            cs = [c for n in names for c in copies(n, sem_i.at[k])]
            inflight[names] = (k, cs)
            for c in cs:
                c.start()

    def arrive(*groups):
        for names in groups:
            k, cs = inflight.pop(names)
            wait(cs)
            free_sems.append(k)

    def wait(cs):
        bg['tok'] = None
        for c in cs:
            c.wait()

    o_copies = []

    def out_copy(b, j, r0, nr):
        return pltpu.make_async_copy(
            ob.at[b * nct + j, pl.ds(r0 // 2, nr // 2), :].bitcast(_BF16),
            o_hbm.at[b, pl.ds(r0, nr), pl.ds(j * _L, _L)], sem_o.at[0])

    def start_out(b, cp, r0, nr):
        for c in range(2):
            o_copies.append(out_copy(b, 2 * cp + c, r0, nr))
            o_copies[-1].start()

    keep = {}

    def tie(v, tok):
        if tok is None:
            return v
        if len(tok) == 2:
            tok.append({jnp.dtype(_F32): tok[0][tok[1]:tok[1] + 8]})
        if v.dtype not in tok[2]:
            tok[2][v.dtype] = pltpu.bitcast(tok[2][jnp.dtype(_F32)], v.dtype)
        t = tok[2][v.dtype]
        n = v.shape[0]
        if n not in keep:
            keep[n] = cat([zer[...]] * (n // 8)) == 0
        return jax.lax.select(keep[n], v, cat([t] * (n // 8)))

    sh16 = jnp.full((8, _L), 16, _U32)
    mk16 = jnp.full((8, _L), 0xFFFF0000, _U32)

    def unpackers(tok):
        sh, mk = cat([tie(sh16, tok)] * 2), cat([tie(mk16, tok)] * 2)
        return (lambda u: pltpu.bitcast(u << sh, _F32),
                lambda u: pltpu.bitcast(u & mk, _F32))

    def pack(lo, hi):
        return pltpu.pack_elementwise([lo, hi], packed_dtype=_BF16)

    def cat(vs, axis=0):
        return vs[0] if len(vs) == 1 else jnp.concatenate(vs, axis=axis)

    have = set()
    probe = [None]
    demand = []

    def x_job(b, g, q, h, phases):
        def words(half, ct, o):
            t = g * _RG + 32 * half + 16 * h
            xu = xb.at[b, ct, pl.ds(4 * t, 64), :].bitcast(_U32)
            return cat([xu[pl.ds(2 * par + o, 8, stride=4), :] for par in range(2)])

        blocks = [(half, ct) for half in range(2) for ct in (2 * q, 2 * q + 1)]
        for phase in phases:
            if phase < 2:
                lo, hi = unpackers((yield 27))
                if phase == 0:
                    outs = {0: [lo(words(*bl, 0)) for bl in blocks]}
                else:
                    outs = {5: [hi(words(*bl, 1)) for bl in blocks]}
            else:
                c = _A if phase == 2 else _B
                p = 2 * phase - 3
                outs = {p: [], p + 1: []}
                for bl in blocks:
                    lo, hi = unpackers((yield 42 if bl == blocks[-1] else 25))
                    we, wo = words(*bl, 0), words(*bl, 1)
                    e = lo(we) + (c * c) * lo(wo)
                    o = c * hi(we) + (c * c * c) * hi(wo)
                    outs[p].append(e + o)
                    outs[p + 1].append(e - o)
                    probe[0] = outs[p][-1]
            for p, (a11, a12, a21, a22) in outs.items():
                if phase >= 2 and p % 2 == 0:
                    tok = yield 22
                    a11, a22 = tie(a11, tok), tie(a22, tok)
                ss = (a11 - a22, a21 - a22, a11, a22, a11 - a12, a21 - a11,
                      a12 - a22)
                for i, s in enumerate(ss):
                    r = 16 * (g % 2) + 8 * h
                    xs[4 * b + g // 2, p, i, r:r + 8, q * _L:(q + 1) * _L] = pack(
                        s[0:8], s[8:16])
                have.add(('x', p, b, g, q, h))
                probe[0] = ss[6]

    def w_job(cp, q, kk, phases):
        def vals(tap, j, lo, hi):
            u = cat([wr.at[j, tap, pl.ds(ct * _L + 16 * kk, 16), :].bitcast(_U32)[...]
                     for ct in (2 * q, 2 * q + 1)])
            return cat([lo(u), hi(u)])

        j1, j2 = 2 * cp, 2 * cp + 1
        gh = 0.5 * _GAM
        for phase in phases:
            if phase < 2:
                lo, hi = unpackers((yield 34))
                tap = 2 if phase == 0 else 0
                p = 0 if phase == 0 else 5
                outs = {p: (gh * vals(tap, j1, lo, hi), vals(tap, j2, lo, hi))}
            else:
                c, lam = (_A, _LA) if phase == 2 else (_B, _LB)
                p = 2 * phase - 3
                uv = []
                for j, s in ((j1, gh * lam), (j2, lam)):
                    lo, hi = unpackers((yield 39))
                    e = s * vals(2, j, lo, hi) + (s * c * c) * vals(0, j, lo, hi)
                    o = (s * c) * vals(1, j, lo, hi)
                    uv.append((e + o, e - o))
                    probe[0] = uv[-1][0]
                outs = {p: (uv[0][0], uv[1][0]), p + 1: (uv[0][1], uv[1][1])}
            for p, (u, v) in outs.items():
                half = jnp.full((8, _L), 0.5, _F32)
                if phase >= 2:
                    half = tie(half, (yield 23))
                half = cat([half] * 2)
                sel = lambda a, n: cat(
                    [a[8 * n:8 * n + 8], a[16 + 8 * n:24 + 8 * n]])
                u1, u2, v1, v2 = sel(u, 0), sel(u, 1), sel(v, 0), sel(v, 1)
                t2 = half * v1 + u1
                t5 = half * v2 - u2
                t1 = t2 - t5
                ts = [t1, t2, v1 - t1, v2 + t1, t5]
                if phase >= 2:
                    ts += [v1, v2]
                for i, t in enumerate(ts):
                    r = 64 * q + 8 * kk
                    ws[cp, p, i, r:r + 8, :] = pack(t[0:8], t[8:16])
                have.add(('w', p, cp, q, kk))
                probe[0] = ts[3]

    def lhs(p, i, b, gs, qs):
        return xs[4 * b + gs[0] // 2, p, i, 16 * (gs[0] % 2):16 * (gs[-1] % 2 + 1),
                  qs[0] * _L:(qs[-1] + 1) * _L]

    def rhs(p, i, cp, qs):
        if p in (0, 5) and i >= 5:
            r = cat([wr.at[2 * cp + 1, 2 if p == 0 else 0,
                           pl.ds((2 * q + i - 5) * _L, _L), :].bitcast(_U32)[...]
                     for q in qs])
        else:
            r = ws[cp, p, i, 64 * qs[0]:64 * (qs[-1] + 1), :]
        return pltpu.bitcast(r, _BF16)

    def ep_job(acc, b, cp, blk, out=None):
        q = _HALO + 8 * blk
        ys = []
        for c in range(2):
            def ld(p, o=0, c=c):
                return acc[c, p, q + o:q + o + 8, :]

            m, mb = tie(ld(4), (yield 24)), ld(3)
            db = mb - m
            sb = mb + m
            ma, mna, z0, z5 = ld(1), ld(2), ld(0), ld(5)
            y0 = (_B * (((_A / _B) * db - ma) + mna) + z5) + ld(5, -1)
            t2 = (_A / _C) * ((ma - (_B / _A) * db) - mna) - z5
            z4 = ((ma - sb) + mna) + z0
            y3 = z4 + ld(0, 1)
            y1 = _A2 * (sb - z0) - _B2 * (z4 + sb)
            ys.append((y0, y1, t2, y3))
            probe[0] = y1
        for c in range(2):
            j = 2 * cp + c
            tok = yield 25
            sc, scc, sh = tie(scsh[0, j], tok), tie(scsh[1, j], tok), scsh[2, j]
            os_ = []
            for k in range(4):
                y = ys[0][k] - ys[1][k] if c == 0 else ys[0][k] + ys[1][k]
                h = y * (scc if k == 2 else sc) + sh
                os_.append(h * jnp.tanh(h) + h)
            probe[0] = os_[3]
            o_ = ob.at[b * nct + j]
            o_[pl.ds(16 * blk, 8, stride=2), :] = pack(os_[0], os_[1])
            o_[pl.ds(16 * blk + 1, 8, stride=2), :] = pack(os_[2], os_[3])
        if out:
            start_out(b, cp, *out)

    epq = []
    bg = dict(jobs=[], every=0, rate=2.0, budget=0.0, since=0, active=None,
              cost=0, tok=None, rep=S['rep'])

    def fetch(force=False):
        if bg['active'] is None:
            if bg['jobs'] and (force or bg['since'] >= bg['every']):
                bg['since'] = min(bg['since'] - bg['every'], 4 * bg['every'])
                bg['active'] = bg['jobs'].pop(0)
                bg['cap'] = 4.0
            elif epq:
                bg['active'] = epq.pop(0)
                bg['cap'] = bg['rep']
            else:
                return False
            bg['cost'] = next(bg['active'])
        return True

    def advance(tok, force=False):
        if fetch(force):
            try:
                bg['cost'] = bg['active'].send(tok)
            except StopIteration:
                bg['active'] = None

    def clock(tok, cycles):
        bg['since'] += cycles
        bg['tok'] = tok
        if not fetch():
            bg['budget'] = 0.0
            return
        bg['budget'] += min(bg['rate'], bg['cap']) * cycles
        if bg['budget'] >= bg['cost']:
            bg['budget'] = min(bg['budget'] - bg['cost'], 16.0)
            advance(tok)

    def burst(ops):
        vals = []
        while ops > 0 and fetch():
            ops -= bg['cost']
            advance(None)
            vals.append(probe[0])
        if S['dem']:
            demand[:] = [S['dem'], vals]

    def require(keys):
        while not all(k in have for k in keys):
            assert bg['active'] is not None or bg['jobs'], keys
            advance(bg['tok'], force=True)

    def drain():
        bg['every'] = 0
        while bg['active'] is not None or epq or bg['jobs']:
            advance(bg['tok'])

    def background(jobs, rate, span=0):
        bg['jobs'] += jobs
        every = span // max(len(bg['jobs']), 1)
        bg.update(every=every, rate=rate, since=every)

    def run_now(jobs):
        for j in jobs:
            for _ in j:
                pass

    def jit(jobs, n_eager, rate):
        run_now(jobs[:n_eager])
        background(jobs[n_eager:], rate)

    def xj(b, gs, qs, phases=(0, 1, 2, 3), by_phase=False):
        if by_phase:
            return [j for ph in phases for j in xj(b, gs, qs, (ph,))]
        return [x_job(b, g, q, h, phases) for g in gs for q in qs for h in range(2)]

    def wj(cp, qs, phases=(0, 1, 2, 3), by_phase=False):
        if by_phase:
            return [j for ph in phases for j in wj(cp, qs, (ph,))]
        return [w_job(cp, q, kk, phases) for q in qs for kk in range(8)]

    class Col:
        def __init__(self, b, cp, out_rows):
            self.b, self.cp, self.out_rows = b, cp, out_rows
            self.acc = acc.at[cp]
            self.todo = list(range(nblk))
            self.sent = 0
            self.jobs = []
            self.full = {p: set() for p in range(6)}
            self.kdone = {}

        def flush(self):
            f = self.full
            ready = [r for r in self.todo
                     if all(r in f[p] for p in range(6))
                     and (r + 1 == nblk or r + 1 in f[0])
                     and (r == 0 or r - 1 in f[5])]
            for r in ready:
                self.todo.remove(r)
                e = min(self.todo, default=nblk)
                out = None
                if e == nblk or 32 * (e - self.sent) >= self.out_rows:
                    out = (32 * self.sent, 32 * (e - self.sent))
                    self.sent = e
                self.jobs.append(ep_job(self.acc, self.b, self.cp, r, out))
                epq.append(self.jobs[-1])

        def finished(self):
            return not self.todo and not any(
                j in epq or j is bg['active'] for j in self.jobs)

    def tiles(subs, qs, two_phase=False, hooks=None, split=False):
        hooks = hooks or {}
        subs = [(c, (2 * i, 2 * i + 1)) for c, i in subs]
        fl = {(i not in c.kdone, c.kdone.get(i, 0) + len(qs) == nq) for c, i in subs}
        assert len(fl) == 1
        first, last = fl.pop()
        for c, i in subs:
            c.kdone[i] = c.kdone.get(i, 0) + len(qs)
        held = []

        def release():
            for k in range(0, held[0].shape[0], 8):
                for r in held:
                    clock([r, k], 2 * len(qs))
            held.clear()

        def prod(t, p, i):
            col, gs = t
            require([('x', p, col.b, g, q, h)
                     for g in gs for q in qs for h in range(2)]
                    + [('w', p, col.cp, q, kk) for q in qs for kk in range(8)])
            l = lhs(p, i, col.b, gs, qs)
            if demand:
                demand[0] -= 16 * len(qs)
                if demand[0] <= 0:
                    head = l[0:8, 0:_L]
                    for v in demand[1]:
                        head = tie(head, [v, 0])
                    row = cat([head, l[0:8, _L:]], axis=1) if len(qs) > 1 else head
                    l = cat([row, l[8:]])
                    demand.clear()
            r = jnp.dot(pltpu.bitcast(l, _BF16), rhs(p, i, col.cp, qs),
                        preferred_element_type=_F32)
            held.append(r)
            if len(held) * len(qs) >= 4:
                release()
            return r

        def put(t, p, half, c, v, init, final):
            col = t[0]
            for n, g in enumerate(t[1]):
                q = _HALO + g * _RG + 32 * half
                part = v[32 * n:32 * n + 32]
                if not init:
                    part = part + col.acc[c, p, q:q + 32, :]
                col.acc[c, p, q:q + 32, :] = part
                if final and last and c == 1:
                    col.full[p].update(range(8 * g + 4 * half, 8 * g + 4 * half + 4))

        def upper(t, p):
            p1 = prod(t, p, 0)
            c11 = p1 + prod(t, p, 6)
            p4 = prod(t, p, 3)
            c11 = c11 + p4
            p3 = prod(t, p, 2)
            c22 = p1 + p3
            p5 = prod(t, p, 4)
            put(t, p, 0, 0, c11 + p5, first, True)
            put(t, p, 0, 1, p3 - p5, first, True)
            if not two_phase:
                return p4, c22
            put(t, p, 1, 0, p4, first, False)
            put(t, p, 1, 1, c22, first, False)

        def lower(t, p, part=None):
            p6 = prod(t, p, 5)
            if part:
                p6 = p6 + part[1]
            p2 = prod(t, p, 1)
            put(t, p, 1, 0, p2 + part[0] if part else p2, first and part, True)
            put(t, p, 1, 1, p6 - p2, first and part, True)

        def flush():
            if held:
                release()
            for c, _ in subs:
                c.flush()

        if two_phase:
            for p in _POINTS:
                for t in subs:
                    upper(t, p)
            for part in ([[(c, (g,))] for c, gs in subs for g in gs]
                         if split else [subs]):
                flush()
                for p in _POINTS:
                    for t in part:
                        lower(t, p)
        else:
            for n, p in enumerate(_POINTS):
                if n in hooks:
                    flush()
                    hooks[n]()
                for t in subs:
                    lower(t, p, upper(t, p))
        flush()

    XR = 8 * _RG
    allq = tuple(range(nq))
    G = lambda i: (2 * i, 2 * i + 1)
    X = lambda i, *qs: ('X', 0, i * XR, XR, qs)
    W = lambda cp, *qs: ('W', cp, qs)

    col0 = [Col(0, cp, seq) for cp in range(ncp)]

    def params():
        mean, var, gam, bet = (
            pbuf[i][...].astype(_F32).reshape(1, ch) for i in range(4))
        s = gam * jax.lax.rsqrt(var + _EPS)
        col = jax.lax.broadcasted_iota(jnp.int32, (1, ch), 1)
        sm = jnp.where((col & _L) == 0, s * (1.0 / _GAM), s)
        for k, v in enumerate((0.5 * sm, (0.5 * _C) * sm, 0.5 * (bet - mean * s))):
            for j in range(nct):
                scsh[k, j] = jnp.broadcast_to(v[:, j * _L:(j + 1) * _L], (8, _L))

    def kt(subs, qs, hooks=None):
        tiles([(col0[cp], i) for i, cp in subs], qs, hooks=hooks)

    def get(group, jobs, rate, fetch=()):
        def f():
            fetch_in(*fetch)
            arrive(group)
            background(jobs(), rate)
            burst(S['ehead'])
        return f

    qb, qr = allq[2:], allq[1:]
    w0, w1, w23 = (W(0, 0), ('Z',)), (W(1, 0),), (W(2, 0), W(3, 0))
    c1 = (W(0, 1), X(0, 1), X(1, 1), X(2, 1), X(3, 1), W(1, 1))
    ca = (W(0, *qb), X(0, *qb), ('P',))
    cb = (X(1, *qb), X(2, *qb), W(1, *qb), X(3, *qb))
    wr23, x1 = (W(2, *qr), W(3, *qr)), (('X', 1, 0, seq, allq),)
    zsrc[...] = jnp.zeros((8, _L), _U32)
    fetch_in(w0, *[(X(i, 0),) for i in range(4)], w1, w23, c1)
    zero = jnp.zeros((_HALO, _L), _F32)
    for cp in range(ncp):
        for c in range(2):
            acc[cp, c, 0, _HALO + T:2 * _HALO + T, :] = zero
            acc[cp, c, 5, 0:_HALO, :] = zero

    arrive(w0)
    run_now(wj(0, (0,)))
    for i in range(4):
        if i == 2:
            fetch_in(ca)
        arrive((X(i, 0),))
        jit(xj(0, G(i), (0,), by_phase=True), S['n1'], S['r1'])
        kt([(i, 0)], (0,))
    arrive(w1)
    jit(wj(1, (0,), by_phase=True), S['n2'], S['r2'])
    kt([(i, 1) for i in range(4)], (0,), hooks={S['h0']: get(
        w23, lambda: wj(2, (0,), by_phase=True) + wj(3, (0,)), S['ra'], (cb,))})
    kt([(i, 2) for i in range(4)], (0,))
    kt([(i, 3) for i in range(4)], (0,), hooks={S['h1']: get(
        c1, lambda: wj(0, (1,), by_phase=True) + xj(0, range(8), (1,))
        + wj(1, (1,), by_phase=True), S['rb'], (wr23, x1))})
    kt([(0, 0), (1, 0)], (1,))
    kt([(2, 0), (3, 0)], (1,), hooks={S['h2']: get(
        ca, lambda: xj(0, G(0), qb) + wj(0, qb, by_phase=True), S['r3'])})
    kt([(i, 1) for i in range(4)], (1,))
    params()
    kt([(0, 0)], qb, hooks={S['hc']: get(
        cb, lambda: xj(0, G(1), qb, by_phase=True) + xj(0, G(2), qb)
        + xj(0, G(3), qb) + wj(1, qb, by_phase=True), S['r7'])})
    for i in range(1, 4):
        kt([(i, 0)], qb)
    kt([(i, 1) for i in range(4)], qb, hooks={S['h4']: get(
        wr23, lambda: wj(2, qr, by_phase=True), S['r4'])})
    kt([(i, 2) for i in range(4)], qr, hooks={S['h6']: lambda: background(
        wj(3, qr, by_phase=True), S['r8'])})
    kt([(i, 3) for i in range(4)], qr, hooks={S['h5']: get(
        x1, lambda: xj(1, G(0), allq), S['r8'])})

    col1 = [Col(1, cp, 480) for cp in range(ncp)]
    for i in range(4):
        if i < 3:
            background(xj(1, G(i + 1), allq), S['r5'], 4 * 2688 - 512)
        for cp in range(ncp):
            assert col0[cp].finished()
            if (i, cp) == (3, ncp - 1):
                col1[cp].out_rows = S['lastrows']
                bg.update(rate=S['rlast'], rep=S['rlast'])
            tiles([(col1[cp], i)], allq, two_phase=True,
                  split=(i, cp) == (3, ncp - 1))
    bg['tok'] = None
    drain()
    wait(o_copies)


@jax.jit
def pallas_standalone__batchnorm__prompt_kernel(
    x: jax.Array,
    w: jax.Array,
    mean: jax.Array,
    var: jax.Array,
    g: jax.Array,
    b: jax.Array,
):
    nb, seq, ch = x.shape
    T = seq // 4
    nct = ch // _L

    def kernel(*refs):
        _kernel(*refs, nb=nb, seq=seq, ch=ch)

    any_spec = pl.BlockSpec(memory_space=pl.ANY)
    return pl.pallas_call(
        kernel,
        out_shape=jax.ShapeDtypeStruct(x.shape, x.dtype),
        in_specs=[any_spec] * 6,
        out_specs=any_spec,
        scratch_shapes=[
            pltpu.VMEM((nb, nct, seq, _L), _BF16),
            pltpu.VMEM((nct, 3, ch, _L), _BF16),
            pltpu.VMEM((ch,), _BF16),
            pltpu.VMEM((ch,), _BF16),
            pltpu.VMEM((ch,), _BF16),
            pltpu.VMEM((ch,), _BF16),
            pltpu.VMEM((4 * nb, 6, 7, 32, ch // 2), _U32),
            pltpu.VMEM((nct // 2, 6, 7, ch // 4, _L), _U32),
            pltpu.VMEM((nct // 2, 2, 6, T + 2 * _HALO, _L), _F32),
            pltpu.VMEM((nb * nct, seq // 2, _L), _U32),
            pltpu.VMEM((3, nct, 8, _L), _F32),
            pltpu.VMEM((8, _L), _U32),
            pltpu.VMEM((8, _L), _U32),
            pltpu.SemaphoreType.DMA((8,)),
            pltpu.SemaphoreType.DMA((1,)),
        ],
        compiler_params=pltpu.CompilerParams(vmem_limit_bytes=110 * 1024 * 1024),
    )(x, w, mean, var, g, b)
```
